```python
import jax
import jax.numpy as jnp

def _softmax(x, axis=-1):
    return jax.nn.softmax(x, axis=axis)
def _gelu(x):
    return jax.nn.gelu(x, approximate=True)
def _silu(x):
    return jax.nn.silu(x)
def _sigmoid(x):
    return jax.nn.sigmoid(x)
def _layernorm(x, axis=-1, eps=1e-5):
    m = jnp.mean(x, axis=axis, keepdims=True)
    v = jnp.var(x, axis=axis, keepdims=True)
    return (x - m) / jnp.sqrt(v + eps)
def _scatter_add(tgt, idx, src, axis=0):
    return tgt.at[idx].add(src)
def _segment_sum(src, seg, n):
    return jax.ops.segment_sum(src, seg, n)
class _Rng:
    def __init__(self, key):
        self._k = key
    def _next(self):
        self._k, sub = jax.random.split(self._k)
        return sub
    def normal(self, shape):
        return jax.random.normal(self._next(), shape, dtype=jnp.bfloat16)
    def randint(self, lo, hi, shape):
        return jax.random.randint(self._next(), shape, lo, hi, dtype=jnp.int32)
    def uniform(self, shape, lo=0.0, hi=1.0):
        return jax.random.uniform(self._next(), shape, jnp.bfloat16, lo, hi)
    def permutation(self, n):
        return jax.random.permutation(self._next(), n)


kernel_name = 'interleave_layers__sliding_local_dilated__ssm_conv_s4__prompt'

def setup_inputs():
    _rng = _Rng(jax.random.key(int.from_bytes(__import__("os").urandom(4), "little")))
    _w = (lambda a: (lambda t: t.astype(jnp.bfloat16) if jnp.issubdtype(t.dtype, jnp.floating) else t)(jnp.asarray(a)))
    def _A_setup():
        B, S, D = 1, 2048, 512
        return {
            "x": _w((lambda *s: _rng.normal(s) * 0.05)(B, S, D)),
            "wqkv": _w((lambda *s: _rng.normal(s) * 0.05)(D, 3 * D)),
            "wo": _w((lambda *s: _rng.normal(s) * 0.05)(D, D)),
        }
    _A_in = _A_setup()

    def _B_setup():
        B, L, D, N = 1, 2048, 512, 128
        A_re = -jnp.exp((lambda *s: _rng.normal(s) * 0.05)(D, N))
        A_im = jnp.pi * (lambda *s: _rng.normal(s) * 0.05)(D, N)
        B_re = (lambda *s: _rng.normal(s) * 0.05)(D, N)
        B_im = (lambda *s: _rng.normal(s) * 0.05)(D, N)
        C_re = (lambda *s: _rng.normal(s) * 0.05)(D, N)
        C_im = (lambda *s: _rng.normal(s) * 0.05)(D, N)
        log_dt = (lambda *s: _rng.normal(s) * 0.05)(D) * 0.5 - 4.0
        Dskip = (lambda *s: _rng.normal(s) * 0.05)(D)
        return {
            "u": _w((lambda *s: _rng.normal(s) * 0.05)(B, L, D)),
            "A_re": _w(A_re),
            "A_im": _w(A_im),
            "B_re": _w(B_re),
            "B_im": _w(B_im),
            "C_re": _w(C_re),
            "C_im": _w(C_im),
            "log_dt": _w(log_dt),
            "Dskip": _w(Dskip),
        }
    _B_in = _B_setup()

    return {
        "A_x": _A_in["x"],
        "A_wqkv": _A_in["wqkv"],
        "A_wo": _A_in["wo"],
        "B_u": _B_in["u"],
        "B_A_re": _B_in["A_re"],
        "B_A_im": _B_in["A_im"],
        "B_B_re": _B_in["B_re"],
        "B_B_im": _B_in["B_im"],
        "B_C_re": _B_in["C_re"],
        "B_C_im": _B_in["C_im"],
        "B_log_dt": _B_in["log_dt"],
        "B_Dskip": _B_in["Dskip"],
    }

def reference(A_x, A_wqkv, A_wo, B_u, B_A_re, B_A_im, B_B_re, B_B_im, B_C_re, B_C_im, B_log_dt, B_Dskip):
    def _A_ref(x, wqkv, wo):
        B, S, D = x.shape
        H = 32; Dh = D // H
        W, dil = 8, 2
        qkv = (lambda x, *d: x.transpose(*d))((x @ wqkv).reshape(B, S, 3, H, Dh), 2, 0, 3, 1, 4)
        q, k, v = qkv[0], qkv[1], qkv[2]
        scale = Dh ** -0.5
        pos = jnp.arange(S)
        off = jnp.arange(W) * dil
        idx = pos[:, None] - off[None, :]
        mask = idx >= 0
        idx_c = jnp.where(mask, idx, 0).reshape(-1)
        kg = k[:, :, idx_c, :].reshape(B, H, S, W, Dh)
        vg = v[:, :, idx_c, :].reshape(B, H, S, W, Dh)
        logits = jnp.einsum("bhsd,bhswd->bhsw", q, kg) * scale
        logits = jnp.where(mask[None, None, :, :], logits, -1e9)
        attn = _softmax(logits, axis=-1)
        o = jnp.einsum("bhsw,bhswd->bhsd", attn, vg)
        return (lambda x, *d: x.transpose(*d))(o, 0, 2, 1, 3).reshape(B, S, D) @ wo

    def _B_ref(u, A_re, A_im, B_re, B_im, C_re, C_im, log_dt, Dskip):
        Bsz, L, D = u.shape
        dt = jnp.exp(log_dt)[:, None]
        A = A_re + 1j * A_im
        Bc = B_re + 1j * B_im
        Cc = C_re + 1j * C_im
        logdA = dt * A
        dB = dt * Bc
        l = (lambda x, dt: x.astype(dt))(jnp.arange(L), A_re.dtype)
        P = jnp.exp(logdA[:, :, None] * l[None, None, :])
        K = jnp.einsum("dn,dnl,dn->dl", Cc, P, dB).real
        L2 = 2 * L
        Kp = jnp.pad(K, ((0, 0), (0, L)))
        up = (lambda x, *d: x.transpose(*d))(u, 0, 2, 1)
        up = jnp.pad(up, ((0, 0), (0, 0), (0, L)))
        Kf = (lambda x, axes=(-2,-1): jnp.fft.rfft2(x.astype(jnp.float32), axes=axes))(Kp[:, None, :], axes=(-2, -1))
        Uf = (lambda x, axes=(-2,-1): jnp.fft.rfft2(x.astype(jnp.float32), axes=axes))(up[:, :, None, :], axes=(-2, -1))
        Yf = Uf * Kf[None, :, :, :]
        y = (lambda x, s, axes=(-2,-1): jnp.fft.irfft2(x, s=s, axes=axes).astype(jnp.bfloat16))(Yf, (1, L2), axes=(-2, -1))[:, :, 0, :L]
        y = (lambda x, *d: x.transpose(*d))(y, 0, 2, 1) + u * Dskip[None, None, :]
        return y

    x = A_x
    x = x + _A_ref(_layernorm(x, axis=-1), A_wqkv, A_wo)
    x = x + _B_ref(_layernorm(x, axis=-1), B_A_re, B_A_im, B_B_re, B_B_im, B_C_re, B_C_im, B_log_dt, B_Dskip)
    x = x + _A_ref(_layernorm(x, axis=-1), A_wqkv, A_wo)
    x = x + _B_ref(_layernorm(x, axis=-1), B_A_re, B_A_im, B_B_re, B_B_im, B_C_re, B_C_im, B_log_dt, B_Dskip)
    return x
```

```python
import numpy as np
import jax
import jax.numpy as jnp
from jax import lax
import jax.experimental.pallas as pl
import jax.experimental.pallas.tpu as pltpu

S, D, DH, WIN = 2048, 512, 16, 8
R = 16
LN = 128
CB = 64
NCB = D // CB
EPS = 1e-5
F32, BF16, U32 = jnp.float32, jnp.bfloat16, jnp.uint32
NT = (((1,), (1,)), ((), ()))


def _dft_matrices():
    lam = np.arange(LN, dtype=np.float64)[None, :, None]
    r = np.arange(R, dtype=np.float64)[:, None, None]
    f = np.arange(LN, dtype=np.float64)[None, None, :]
    th = 2.0 * np.pi * (f + 0.5) * (R * lam + r) / (2 * S)
    return np.concatenate([np.cos(th), -np.sin(th)], axis=-1).astype(BF16)


_M = _dft_matrices()


def _iota(shape, dim):
    return lax.broadcasted_iota(jnp.int32, shape, dim)


def _cmul(a, b):
    return (a[0] * b[0] - a[1] * b[1], a[0] * b[1] + a[1] * b[0])


def _csq(a):
    t = a[0] * a[1]
    return (a[0] * a[0] - a[1] * a[1], t + t)


def _radix4(a, b, c, d, sign):
    s0 = (a[0] + c[0], a[1] + c[1])
    d0 = (a[0] - c[0], a[1] - c[1])
    s1 = (b[0] + d[0], b[1] + d[1])
    d1 = (b[0] - d[0], b[1] - d[1])
    y0 = (s0[0] + s1[0], s0[1] + s1[1])
    y2 = (s0[0] - s1[0], s0[1] - s1[1])
    p = (d0[0] - d1[1], d0[1] + d1[0])
    m = (d0[0] + d1[1], d0[1] - d1[0])
    return (y0, p, y2, m) if sign > 0 else (y0, m, y2, p)


def _twiddle(a, k, sign):
    if k == 0:
        return a
    c = float(np.cos(2 * np.pi * k / 16))
    s = float(sign * np.sin(2 * np.pi * k / 16))
    if k == 4:
        return (-a[1], a[0]) if sign > 0 else (a[1], -a[0])
    if k == 2:
        if sign > 0:
            return ((a[0] - a[1]) * c, (a[0] + a[1]) * c)
        return ((a[0] + a[1]) * c, (a[1] - a[0]) * c)
    if k == 6:
        if sign > 0:
            return ((a[0] + a[1]) * c, (a[1] - a[0]) * c)
        return ((a[0] - a[1]) * c, (a[0] + a[1]) * c)
    return (a[0] * c - a[1] * s, a[0] * s + a[1] * c)


def _fft16_first(g):
    t = []
    for r0 in range(4):
        y = _radix4(g[r0], g[r0 + 4], g[r0 + 8], g[r0 + 12], -1)
        t.append([_twiddle(y[g0], r0 * g0, -1) for g0 in range(4)])
    return t


def _layernorm(x):
    m = jnp.sum(x, axis=0, keepdims=True) * (1.0 / D)
    xc = x - m
    v = jnp.sum(xc * xc, axis=0, keepdims=True) * (1.0 / D)
    return xc * lax.rsqrt(v + EPS)


def _kernel(x_hbm, wqkv_hbm, wo_hbm, are_hbm, aim_hbm, bre_hbm, bim_hbm, cre_hbm, cim_hbm,
            ldt_ref, dsk_ref, m_hbm, out_hbm,
            io, wraw, woraw, par, mm, X, XN, U, KV, Q, O, WT, WOT, KF, KT, G, HH, DT, DSK,
            SA, SB, KO, sems):
    pcp = [pltpu.make_async_copy(h, par.at[i], sems.at[i])
           for i, h in enumerate((are_hbm, aim_hbm, bre_hbm, bim_hbm, cre_hbm, cim_hbm))]
    mcp = pltpu.make_async_copy(m_hbm, mm, sems.at[6])
    xcp = [pltpu.make_async_copy(x_hbm.at[:, pl.ds(j * LN, LN)], io.at[j], sems.at[7 + j])
           for j in range(4)]
    wcp = pltpu.make_async_copy(wqkv_hbm, wraw, sems.at[11])
    wocp = pltpu.make_async_copy(wo_hbm, woraw, sems.at[12])
    for c in pcp + [mcp] + xcp + [wcp, wocp]:
        c.start()

    dt_row = jnp.exp(ldt_ref[...].astype(F32)).astype(BF16).astype(F32)
    ds_row = dsk_ref[...].astype(F32)
    for j in range(4):
        sl = slice(j * LN, (j + 1) * LN)
        DT[sl, :] = jnp.broadcast_to(dt_row[:, sl], (LN, LN)).T
        DSK[sl, :] = jnp.broadcast_to(ds_row[:, sl], (LN, LN)).T
    SB[...] = jnp.zeros(SB.shape, SB.dtype)
    for c in pcp:
        c.wait()

    lane = _iota((8, LN), 1)
    quarter = lane >> 5

    def kgen(J, carry):
        for s in range(4):
            row0 = pl.multiple_of(s * LN + J * 16, 16)
            p = [par[i, pl.ds(row0, 16), :].astype(F32) for i in range(6)]
            dt = DT[pl.ds(row0, 16), :]
            zr, zi = dt * p[0], dt * p[1]
            mag = jnp.exp(zr)
            e1 = (mag * jnp.cos(zi), mag * jnp.sin(zi))
            w = _cmul((p[4], p[5]), (dt * p[2], dt * p[3]))
            w = (w[0] * (1.0 / S), w[1] * (1.0 / S))
            pw = [e1]
            for _ in range(10):
                pw.append(_csq(pw[-1]))
            a = [w]
            for k in range(5):
                a += [_cmul(v, pw[4 + k]) for v in a]
            one = (jnp.ones_like(zr), jnp.zeros_like(zr))
            b = [one]
            for k in range(4):
                b += [pw[k]] + [_cmul(v, pw[k]) for v in b[1:]]
            b.append(pw[4])
            b += [pw[9]] + [_cmul(pw[9], b[i]) for i in (4, 8, 12, 16)]
            b += [pw[10]] + [_cmul(pw[10], b[i]) for i in (8, 16)]
            e1536 = _cmul(pw[10], pw[9])
            b += [e1536] + [_cmul(e1536, b[i]) for i in (8, 16)]
            for c in range(2):
                for i in range(16):
                    pair = [a[2 * i][c], a[2 * i + 1][c]]
                    SA[c, pl.ds(s * 16 + i, 16, stride=65), :] = pltpu.pack_elementwise(
                        pair, packed_dtype=BF16).astype(U32)
                for i in range(14):
                    pair = [b[2 * i][c], b[2 * i + 1][c]]
                    SB[c, pl.ds(s * 16 + i, 16, stride=65), :] = pltpu.pack_elementwise(
                        pair, packed_dtype=BF16).astype(U32)
        q32 = _iota((32, LN), 1) >> 5
        for m in range(16):
            o = [lax.dot_general(pltpu.bitcast(SB[c, pl.ds(m * 65, 64), :], BF16),
                                 pltpu.bitcast(SA[c, pl.ds(m * 65, 64), :], BF16),
                                 NT, preferred_element_type=F32) for c in range(2)]
            o = o[0] - o[1]
            KO[pl.ds(m * 33, 32), :] = jnp.where(
                q32 < 2, jnp.where(q32 == 0, o[0:32], o[32:64]),
                jnp.where(q32 == 2, o[64:96], o[96:128]))
        for h in range(2):
            kb = [KO[pl.ds(h * 8 * 33 + i, 8, stride=33), :] for i in range(28)]
            low = (lane & 31) < 16
            rnd = lambda r, st: int(np.round(r / st))
            q0 = [kb[r] if r % 2 == 0 else jnp.where(low, kb[r], kb[2 * rnd(r, 2)])
                  for r in range(R)]
            q1 = [pltpu.roll(v, 32, 1) for v in kb[17:22]]
            q2 = [pltpu.roll(v, 64, 1) for v in kb[22:25]]
            q3 = [pltpu.roll(v, 96, 1) for v in kb[25:28]]
            for s in range(4):
                q23 = [jnp.where(quarter == (s + 2) % 4, u, v) for u, v in zip(q2, q3)]
                rest = {}
                for r in range(R):
                    key = (rnd(r, 4), rnd(r, 8))
                    if key not in rest:
                        rest[key] = jnp.where(quarter == (s + 1) % 4, q1[key[0]], q23[key[1]])
                    row0 = pl.multiple_of(s * LN + J * 16 + h * 8, 8)
                    KT[r, pl.ds(row0, 8), :] = jnp.where(quarter == s, q0[r], rest[key])
        return carry

    lax.fori_loop(0, 8, kgen, 0)

    mcp.wait()

    for s in range(4):
        def kf(i, carry, s=s):
            row0 = pl.multiple_of(s * LN + i * CB, CB)
            for r in range(R):
                mr = mm[r]
                if s:
                    mr = jnp.concatenate([mr[LN - 32 * s:], mr[:LN - 32 * s]], axis=0)
                G[0, r] = jnp.dot(KT[r, pl.ds(row0, CB), :].astype(BF16), mr,
                                  preferred_element_type=F32)
            for h in range(CB // 8):
                g = [(G[0, r, h * 8:h * 8 + 8, :LN], G[0, r, h * 8:h * 8 + 8, LN:])
                     for r in range(R)]
                t = _fft16_first(g)
                for g0 in range(4):
                    y = _radix4(t[0][g0], t[1][g0], t[2][g0], t[3][g0], -1)
                    for g1 in range(4):
                        for c in range(2):
                            KF[2 * (4 * g0 + g1) + c, pl.ds(row0 + h * 8, 8), :] = y[g1][c]
            return carry
        lax.fori_loop(0, LN // CB, kf, 0)

    for j in range(4):
        xcp[j].wait()
    iow = io.bitcast(U32)

    def xin(j, carry):
        sl = pl.ds(pl.multiple_of(j * LN, LN), LN)
        for rho in range(8):
            t = iow[j, pl.ds(rho, LN, stride=8), :].T
            X[2 * rho, sl, :] = pltpu.bitcast(t << 16, F32)
            X[2 * rho + 1, sl, :] = pltpu.bitcast(t & np.uint32(0xFFFF0000), F32)
        return carry

    lax.fori_loop(0, 4, xin, 0)

    pr, pc = _iota((LN, LN), 0), _iota((LN, LN), 1)
    perm = jnp.where(pc == (pr & 7) * DH + (pr >> 3), 1.0, 0.0).astype(BF16)
    wcp.wait()
    for j in range(12):
        t = lax.dot_general(perm, wraw[:, j * LN:(j + 1) * LN], NT, preferred_element_type=F32)
        if j < 4:
            t = t * (DH ** -0.5)
        WT[j * LN:(j + 1) * LN, :] = t.astype(BF16)
    wocp.wait()
    for j in range(4):
        t = jnp.dot(perm, woraw[j * LN:(j + 1) * LN, :], preferred_element_type=F32)
        WOT[:, j * LN:(j + 1) * LN] = t.T.astype(BF16)

    def layer(l, carry):
        def phase1(r, carry):
            xn = _layernorm(X[r]).astype(BF16)
            XN[r] = xn
            kv = jnp.dot(WT[D:, :], xn, preferred_element_type=F32)
            KV[r + R] = kv
            KV[r] = pltpu.roll(kv, 1, 1)
            return carry

        lax.fori_loop(0, R, phase1, 0)

        def phase2(r, carry):
            Q[0] = jnp.dot(WT[:D, :], XN[r], preferred_element_type=F32)
            for j in range(4):
                lg = [None] * WIN
                for dh in range(DH):
                    row = j * LN + dh * 8
                    q = Q[0, row:row + 8, :]
                    for w in range(WIN):
                        t = q * KV[r + R - 2 * w, row:row + 8, :]
                        lg[w] = t if dh == 0 else lg[w] + t
                for w in range(1, WIN):
                    lg[w] = jnp.where(lane * R + (r - 2 * w) >= 0, lg[w], -1e9)
                mx = lg[0]
                for w in range(1, WIN):
                    mx = jnp.maximum(mx, lg[w])
                e = [jnp.exp(v - mx) for v in lg]
                den = e[0]
                for w in range(1, WIN):
                    den = den + e[w]
                inv = 1.0 / den
                e = [v * inv for v in e]
                for dh in range(0, DH, 2):
                    oo = []
                    for k in range(2):
                        row = D + j * LN + (dh + k) * 8
                        acc = None
                        for w in range(WIN):
                            t = e[w] * KV[r + R - 2 * w, row:row + 8, :]
                            acc = t if acc is None else acc + t
                        oo.append(acc)
                    row = j * LN + dh * 8
                    O[0, row:row + 16, :] = jnp.concatenate(oo, axis=0).astype(BF16)
            x = X[r] + jnp.dot(WOT[...], O[0], preferred_element_type=F32)
            u = _layernorm(x)
            U[r] = u.astype(BF16)
            X[r] = x + u * DSK[...]
            return carry

        lax.fori_loop(0, R, phase2, 0)

        def conv(i, carry):
            row0 = pl.multiple_of(i * CB, CB)
            for r in range(R):
                G[0, r] = jnp.dot(U[r, pl.ds(row0, CB), :], mm[r], preferred_element_type=F32)
            for h in range(CB // 8):
                hs = slice(h * 8, h * 8 + 8)
                g = [(G[0, r, hs, :LN], G[0, r, hs, LN:]) for r in range(R)]
                t = _fft16_first(g)
                v = [[None] * 4 for _ in range(4)]
                for g0 in range(4):
                    y = _radix4(t[0][g0], t[1][g0], t[2][g0], t[3][g0], -1)
                    y = [_cmul(y[g1], (KF[2 * (4 * g0 + g1), pl.ds(row0 + h * 8, 8), :],
                                       KF[2 * (4 * g0 + g1) + 1, pl.ds(row0 + h * 8, 8), :]))
                         for g1 in range(4)]
                    y = _radix4(*y, 1)
                    for r0 in range(4):
                        v[r0][g0] = _twiddle(y[r0], r0 * g0, 1)
                for r0 in range(4):
                    y = _radix4(*v[r0], 1)
                    for r1 in range(4):
                        HH[0, r0 + 4 * r1, hs, :LN] = y[r1][0]
                        HH[0, r0 + 4 * r1, hs, LN:] = y[r1][1]
            for r in range(R):
                y = lax.dot_general(HH[0, r].astype(BF16), mm[r], NT, preferred_element_type=F32)
                X[r, pl.ds(row0, CB), :] += y
            return carry

        lax.fori_loop(0, NCB, conv, 0)
        return carry

    lax.fori_loop(0, 2, layer, 0)

    ocp = [pltpu.make_async_copy(io.at[j], out_hbm.at[:, pl.ds(j * LN, LN)], sems.at[7 + j])
           for j in range(4)]
    for j in range(4):
        for rho in range(8):
            sl = slice(j * LN, (j + 1) * LN)
            w = pltpu.pack_elementwise([X[2 * rho, sl, :], X[2 * rho + 1, sl, :]],
                                       packed_dtype=BF16).astype(U32)
            iow[j, pl.ds(rho, LN, stride=8), :] = w.T
        ocp[j].start()
    for c in ocp:
        c.wait()


@jax.jit
def pallas_interleave_layers__sliding_local_dilated__ssm_conv_s4__prompt_kernel(
    A_x: jax.Array,
    A_wqkv: jax.Array,
    A_wo: jax.Array,
    B_u: jax.Array,
    B_A_re: jax.Array,
    B_A_im: jax.Array,
    B_B_re: jax.Array,
    B_B_im: jax.Array,
    B_C_re: jax.Array,
    B_C_im: jax.Array,
    B_log_dt: jax.Array,
    B_Dskip: jax.Array,
):
    del B_u
    hbm = pl.BlockSpec(memory_space=pl.ANY)
    vmem = pl.BlockSpec(memory_space=pltpu.VMEM)
    V = pltpu.VMEM
    out = pl.pallas_call(
        _kernel,
        out_shape=jax.ShapeDtypeStruct((S, D), BF16),
        in_specs=[hbm] * 9 + [vmem, vmem, hbm],
        out_specs=hbm,
        scratch_shapes=[
            V((4, S, LN), BF16),
            V((D, 3 * D), BF16),
            V((D, D), BF16),
            V((6, D, LN), BF16),
            V((R, LN, 2 * LN), BF16),
            V((R, D, LN), F32),
            V((R, D, LN), BF16),
            V((R, D, LN), BF16),
            V((2 * R, 2 * D, LN), F32),
            V((2, D, LN), F32),
            V((2, D, LN), BF16),
            V((3 * D, D), BF16),
            V((D, D), BF16),
            V((2 * R, D, LN), F32),
            V((R, D, LN), F32),
            V((2, R, CB, 2 * LN), F32),
            V((2, R, CB, 2 * LN), F32),
            V((D, LN), F32),
            V((D, LN), F32),
            V((2, 16 * 65, LN), U32),
            V((2, 16 * 65, LN), U32),
            V((16 * 33, LN), F32),
            pltpu.SemaphoreType.DMA((13,)),
        ],
        compiler_params=pltpu.CompilerParams(vmem_limit_bytes=100 * 1024 * 1024),
    )(A_x.reshape(S, D), A_wqkv, A_wo, B_A_re, B_A_im, B_B_re, B_B_im, B_C_re, B_C_im,
      B_log_dt.reshape(1, D), B_Dskip.reshape(1, D), _M)
    return out.reshape(1, S, D)
```

```python
import contextlib
import numpy as np
import jax
import jax.numpy as jnp
from jax import lax
import jax.experimental.pallas as pl
import jax.experimental.pallas.tpu as pltpu

S, D, DH, WIN = 2048, 512, 16, 8
R = 16
LN = 128
CB = 64
NCB = D // CB
EPS = 1e-5
F32, BF16, U32 = jnp.float32, jnp.bfloat16, jnp.uint32
NT = (((1,), (1,)), ((), ()))


def _dft_matrices():
    lam = np.arange(LN, dtype=np.float64)[None, :, None]
    r = np.arange(R, dtype=np.float64)[:, None, None]
    f = np.arange(LN, dtype=np.float64)[None, None, :]
    th = 2.0 * np.pi * (f + 0.5) * (R * lam + r) / (2 * S)
    m = np.stack([np.cos(th), -np.sin(th)], axis=1).astype(BF16).view(np.uint16).astype(np.uint32)
    return (m[:, :, 0::2] | (m[:, :, 1::2] << 16)).reshape(R * LN, LN)


_M = _dft_matrices()


SCOPES = False


def _scope(name):
    return jax.named_scope(name) if SCOPES else contextlib.nullcontext()


FLAGS = None
SKIP = NOB = ''
LO, NZ = 8, 16
B3 = ((0, 8, 0), (4, 12, 0), (9, 16, 4), (14, 16, 9), (16, 16, 14))
DO = 256
LAG, P4 = 0, 1
UN3 = 1
WROWS = 8 * D


class _Buf:
    def __init__(self, ref, base=0, size=None):
        if isinstance(base, int):
            self.ref, self.base = ref, base
        else:
            self.ref, self.base = ref.at[pl.ds(pl.multiple_of(base, 16), size), :], 0

    def ld(self, row, n):
        return self.ref[self.base + row:self.base + row + n, :]

    def st(self, row, v):
        self.ref[self.base + row:self.base + row + v.shape[0], :] = v.astype(self.ref.dtype)


def _weave(*stages):
    live = [[g, n, 0] for g, n in stages]
    while live:
        st = min(live, key=lambda t: t[2] / t[1])
        try:
            next(st[0])
            st[2] += 1
        except StopIteration:
            live.remove(st)


def _chain(*gens):
    for g in gens:
        yield from g


def _take(g, n):
    for _, _ in zip(range(n), g):
        yield


def _tree(op, v):
    while len(v) > 1:
        v = [op(v[i], v[i + 1]) for i in range(0, len(v), 2)]
    return v[0]


def _mult(i, n):
    return i if isinstance(i, int) else pl.multiple_of(i, n)


def _loop(lo, hi, body, unroll, force=False):
    n = hi - lo
    assert n % unroll == 0
    if n == unroll and not force:
        for i in range(lo, hi):
            body(i)
        return

    def outer(k, carry):
        for u in range(unroll):
            body(lo + k * unroll + u)
        return carry

    lax.fori_loop(0, n // unroll, outer, 0)


def _iota(shape, dim):
    return lax.broadcasted_iota(jnp.int32, shape, dim)


def _cmul(a, b):
    return (a[0] * b[0] - a[1] * b[1], a[0] * b[1] + a[1] * b[0])


def _csq(a):
    t = a[0] * a[1]
    return (a[0] * a[0] - a[1] * a[1], t + t)


def _radix4(a, b, c, d, sign):
    s0 = (a[0] + c[0], a[1] + c[1])
    d0 = (a[0] - c[0], a[1] - c[1])
    s1 = (b[0] + d[0], b[1] + d[1])
    d1 = (b[0] - d[0], b[1] - d[1])
    y0 = (s0[0] + s1[0], s0[1] + s1[1])
    y2 = (s0[0] - s1[0], s0[1] - s1[1])
    p = (d0[0] - d1[1], d0[1] + d1[0])
    m = (d0[0] + d1[1], d0[1] - d1[0])
    return (y0, p, y2, m) if sign > 0 else (y0, m, y2, p)


def _twiddle(a, k, sign):
    if k == 0:
        return a
    c = float(np.cos(2 * np.pi * k / 16))
    s = float(sign * np.sin(2 * np.pi * k / 16))
    if k == 4:
        return (-a[1], a[0]) if sign > 0 else (a[1], -a[0])
    if k == 2:
        if sign > 0:
            return ((a[0] - a[1]) * c, (a[0] + a[1]) * c)
        return ((a[0] + a[1]) * c, (a[1] - a[0]) * c)
    if k == 6:
        if sign > 0:
            return ((a[0] + a[1]) * c, (a[1] - a[0]) * c)
        return ((a[0] - a[1]) * c, (a[0] + a[1]) * c)
    return (a[0] * c - a[1] * s, a[0] * s + a[1] * c)


def _fft16_first(g):
    t = []
    for r0 in range(4):
        y = _radix4(g[r0], g[r0 + 4], g[r0 + 8], g[r0 + 12], -1)
        t.append([_twiddle(y[g0], r0 * g0, -1) for g0 in range(4)])
    return t


def _kernel(x_hbm, wqkv_hbm, wo_hbm, are_hbm, aim_hbm, bre_hbm, bim_hbm, cre_hbm, cim_hbm,
            ldt_ref, dsk_ref, m_hbm, out_hbm,
            io, wraw, woraw, par, mm, X, Y, KF, DSK, XN, U, W, Z, KVQ, O, G, T, HH,
            KT, G0, DT, SA, SB, KO, zero, sems):
    for k in range(R):
        zero[k] = 0

    def block(name):
        def deco(f):
            if SKIP and name in SKIP:
                return
            with _scope(name):
                f() if name in NOB else pl.when(zero[0] == 0)(f)
        return deco

    def opaque(r):
        return zero[r] if isinstance(r, int) else 0

    pcp = [pltpu.make_async_copy(h, par.at[i], sems.at[i])
           for i, h in enumerate((are_hbm, aim_hbm, bre_hbm, bim_hbm, cre_hbm, cim_hbm))]
    mcp = pltpu.make_async_copy(m_hbm, mm.at[pl.ds(0, R * LN), :], sems.at[6])
    xcp = [pltpu.make_async_copy(x_hbm.at[:, pl.ds(j * LN, LN)], io.at[j], sems.at[7 + j])
           for j in range(4)]
    wcp = pltpu.make_async_copy(wqkv_hbm, wraw, sems.at[11])
    wocp = pltpu.make_async_copy(wo_hbm, woraw, sems.at[12])
    for c in pcp + [mcp] + xcp + [wcp, wocp]:
        c.start()

    dt_row = jnp.exp(ldt_ref[...].astype(F32)).astype(BF16).astype(F32)
    ds_row = dsk_ref[...].astype(F32)
    for j in range(4):
        sl = slice(j * LN, (j + 1) * LN)
        DT[sl, :] = jnp.broadcast_to(dt_row[:, sl], (LN, LN)).T
        DSK[sl, :] = jnp.broadcast_to(ds_row[:, sl], (LN, LN)).T
    SB[...] = jnp.zeros(SB.shape, SB.dtype)
    with _scope('pwait'):
        for c in pcp:
            c.wait()

    lane = _iota((8, LN), 1)
    quarter = lane >> 5

    def kgen(J, carry):
        for s in range(4):
            row0 = pl.multiple_of(s * LN + J * 16, 16)
            p = [par[i, pl.ds(row0, 16), :].astype(F32) for i in range(6)]
            dt = DT[pl.ds(row0, 16), :]
            zr, zi = dt * p[0], dt * p[1]
            mag = jnp.exp(zr)
            e1 = (mag * jnp.cos(zi), mag * jnp.sin(zi))
            w = _cmul((p[4], p[5]), (dt * p[2], dt * p[3]))
            w = (w[0] * (1.0 / S), w[1] * (1.0 / S))
            pw = [e1]
            for _ in range(10):
                pw.append(_csq(pw[-1]))
            a = [w]
            for k in range(5):
                a += [_cmul(v, pw[4 + k]) for v in a]
            one = (jnp.ones_like(zr), jnp.zeros_like(zr))
            b = [one]
            for k in range(4):
                b += [pw[k]] + [_cmul(v, pw[k]) for v in b[1:]]
            b.append(pw[4])
            b += [pw[9]] + [_cmul(pw[9], b[i]) for i in (4, 8, 12, 16)]
            b += [pw[10]] + [_cmul(pw[10], b[i]) for i in (8, 16)]
            e1536 = _cmul(pw[10], pw[9])
            b += [e1536] + [_cmul(e1536, b[i]) for i in (8, 16)]
            for c in range(2):
                for i in range(16):
                    pair = [a[2 * i][c], a[2 * i + 1][c]]
                    SA[c, pl.ds(s * 16 + i, 16, stride=65), :] = pltpu.pack_elementwise(
                        pair, packed_dtype=BF16).astype(U32)
                for i in range(14):
                    pair = [b[2 * i][c], b[2 * i + 1][c]]
                    SB[c, pl.ds(s * 16 + i, 16, stride=65), :] = pltpu.pack_elementwise(
                        pair, packed_dtype=BF16).astype(U32)
        q32 = _iota((32, LN), 1) >> 5
        for m in range(16):
            o = [lax.dot_general(pltpu.bitcast(SB[c, pl.ds(m * 65, 64), :], BF16),
                                 pltpu.bitcast(SA[c, pl.ds(m * 65, 64), :], BF16),
                                 NT, preferred_element_type=F32) for c in range(2)]
            o = o[0] - o[1]
            KO[pl.ds(m * 33, 32), :] = jnp.where(
                q32 < 2, jnp.where(q32 == 0, o[0:32], o[32:64]),
                jnp.where(q32 == 2, o[64:96], o[96:128]))
        for h in range(2):
            kb = [KO[pl.ds(h * 8 * 33 + i, 8, stride=33), :] for i in range(28)]
            low = (lane & 31) < 16
            rnd = lambda r, st: int(np.round(r / st))
            q0 = [kb[r] if r % 2 == 0 else jnp.where(low, kb[r], kb[2 * rnd(r, 2)])
                  for r in range(R)]
            q1 = [pltpu.roll(v, 32, 1) for v in kb[17:22]]
            q2 = [pltpu.roll(v, 64, 1) for v in kb[22:25]]
            q3 = [pltpu.roll(v, 96, 1) for v in kb[25:28]]
            for s in range(4):
                q23 = [jnp.where(quarter == (s + 2) % 4, u, v) for u, v in zip(q2, q3)]
                rest = {}
                for r in range(R):
                    key = (rnd(r, 4), rnd(r, 8))
                    if key not in rest:
                        rest[key] = jnp.where(quarter == (s + 1) % 4, q1[key[0]], q23[key[1]])
                    row0 = pl.multiple_of(s * LN + J * 16 + h * 8, 8)
                    KT[r, pl.ds(row0, 8), :] = jnp.where(quarter == s, q0[r], rest[key])
        return carry

    @block("kgen")
    def _():
        lax.fori_loop(0, 8, kgen, 0)

    with _scope("mwait"):
        mcp.wait()

    for s in range(4):
        def kf(i, carry, s=s):
            row0 = pl.multiple_of(s * LN + i * CB, CB)
            for r in range(R):
                mr = jnp.concatenate([mm[r * LN:r * LN + 64, :], mm[r * LN + 64:(r + 1) * LN, :]], axis=1)
                if s:
                    mr = jnp.concatenate([mr[64 - 16 * s:], mr[:64 - 16 * s]], axis=0)
                mr = pltpu.bitcast(mr, BF16)
                G0[r] = jnp.dot(KT[r, pl.ds(row0, CB), :].astype(BF16), mr,
                                  preferred_element_type=F32)
            for h in range(CB // 8):
                g = [(G0[r, h * 8:h * 8 + 8, :LN], G0[r, h * 8:h * 8 + 8, LN:])
                     for r in range(R)]
                t = _fft16_first(g)
                for g0 in range(4):
                    y = _radix4(t[0][g0], t[1][g0], t[2][g0], t[3][g0], -1)
                    for g1 in range(4):
                        for c in range(2):
                            KF[pl.ds((2 * (4 * g0 + g1) + c) * D + row0 + h * 8, 8), :] = y[g1][c]
            return carry
        @block("kf")
        def _():
            lax.fori_loop(0, LN // CB, kf, 0)

    for j in range(4):
        with _scope("xwait"):
            xcp[j].wait()
    iow = io.bitcast(U32)

    def xin(j, carry):
        x = _Buf(X, j * LN, R * D - D + LN)
        for rho in range(8):
            t = iow[j, pl.ds(rho, LN, stride=8), :].T
            x.st(2 * rho * D, pltpu.bitcast(t << 16, F32))
            x.st((2 * rho + 1) * D, pltpu.bitcast(t & np.uint32(0xFFFF0000), F32))
        return carry

    with _scope("xin"):
        lax.fori_loop(0, 4, xin, 0)

    pr, pc = _iota((LN, LN), 0), _iota((LN, LN), 1)
    perm = jnp.where(pc == (pr & 7) * DH + (pr >> 3), 1.0, 0.0).astype(BF16)
    with _scope("wwait"):
        wcp.wait()
    for j in range(12):
        t = lax.dot_general(perm, wraw[:, j * LN:(j + 1) * LN], NT, preferred_element_type=F32)
        if j < 4:
            t = t * (DH ** -0.5)
        for k in range(4):
            _Buf(W).st((k * 4 * D + (3 * (j % 4) + (j // 4 + 2) % 3) * LN) // 2,
                       pltpu.bitcast(t[:, k * LN:(k + 1) * LN].astype(BF16), F32))
    wocp.wait()
    for j in range(4):
        t = jnp.dot(perm, woraw[j * LN:(j + 1) * LN, :], preferred_element_type=F32)
        _Buf(W).st((j * 4 * D + 3 * D) // 2, pltpu.bitcast(t.T.astype(BF16), F32))

    def colsum(f, step):
        acc = [f(c * 8) for c in range(4)]
        for i in range(4, D // 8):
            acc[i % 4] = acc[i % 4] + f(i * 8)
            if i % step == step - 1:
                yield
        s = jnp.sum((acc[0] + acc[1]) + (acc[2] + acc[3]), axis=0, keepdims=True)
        return jnp.broadcast_to(s * (1.0 / D), (8, LN))

    def ln_stats(ref, base):
        x = _Buf(ref, base + zero[0], D)
        m = yield from colsum(lambda c: x.ld(c, 8), 32)
        x = _Buf(ref, base + zero[1], D)
        v = yield from colsum(lambda c: jnp.square(x.ld(c, 8) - m), 8)
        return _Buf(ref, base + zero[2], D), m, lax.rsqrt(v + EPS)

    def ln1(r):
        x, m, rs = yield from ln_stats(X, r * D)
        for c in range(0, D, 16):
            t = [(x.ld(c + k, 8) - m) * rs for k in (0, 8)]
            _Buf(XN, r * D).st(c, jnp.concatenate(t, axis=0))
            if c % 64 == 48:
                yield

    def ln2(r):
        x, m, rs = yield from ln_stats(Z[order.index(r) % NZ], 0)
        dsk = _Buf(DSK, zero[r], D)
        for c in range(0, D, 16):
            t = []
            for k in (c, c + 8):
                v = x.ld(k, 8)
                t.append((v - m) * rs)
                _Buf(Y, r * D).st(k, v + t[-1] * dsk.ld(k, 8))
            _Buf(U, r * D).st(c, jnp.concatenate(t, axis=0))
            if c % 64 == 48:
                yield
                yield

    def wdot(c, n, rhs):
        lhs = jnp.concatenate(
            [pltpu.bitcast(W[(t * 4 * D + c) // 2:(t * 4 * D + c + n) // 2, :], BF16)
             for t in range(4)], axis=1)
        return jnp.dot(lhs, rhs.ld(0, D), preferred_element_type=F32)

    def qkvproj(j, r):
        b, i = _Buf(KVQ[j % 2][r % 2]), r // 2
        for c in range(3):
            t = wdot((3 * j + c) * LN, LN, _Buf(XN, r * D + zero[(r + c) % R], D))
            if c == 2:
                b.st((32 + i) * LN, t)
            else:
                b.st((2 * (8 + i) + c) * LN, t)
                if i:
                    b.st((2 * i + c) * LN, pltpu.roll(t, 1, 1))
            yield

    def core(j, r):
        b, i = _Buf(KVQ[j % 2][r % 2], zero[r], 40 * LN), r // 2
        lg = [None] * WIN
        for dh in range(DH):
            q = b.ld((32 + i) * LN + dh * 8, 8)
            for w in range(WIN):
                t = q * b.ld((8 + i - w) * 2 * LN + dh * 8, 8)
                lg[w] = t if dh == 0 else lg[w] + t
            if dh % 2:
                yield
        for w in range(i + 1, WIN):
            lg[w] = jnp.where(lane > 0, lg[w], -1e9)
        mx = _tree(jnp.maximum, lg)
        e = [jnp.exp(v - mx) for v in lg]
        inv = 1.0 / _tree(jnp.add, e)
        e = [v * inv for v in e]
        yield
        yield
        for dh in range(0, DH, 2):
            oo = []
            for k in (dh, dh + 1):
                acc = None
                for w in range(WIN):
                    t = e[w] * b.ld((8 + i - w) * 2 * LN + LN + k * 8, 8)
                    acc = t if acc is None else acc + t
                oo.append(acc)
            _Buf(O, r * D + j * LN).st(dh * 8, jnp.concatenate(oo, axis=0))
            yield

    def oproj(r):
        for c in range(0, D, DO):
            Z[order.index(r) % NZ][c:c + DO, :] = X[r * D + c:r * D + c + DO, :] + wdot(
                3 * D + c, DO, _Buf(O, r * D + zero[(r + c // DO) % R], D))
            yield

    def mat(r):
        return pltpu.bitcast(jnp.concatenate(
            [mm[2 * r * 64:(2 * r + 1) * 64, :], mm[(2 * r + 1) * 64:(2 * r + 2) * 64, :]], axis=1),
            BF16)

    def cmxu(fi, ii):
        res = []
        for r in order:
            if LAG and r >= LAG:
                _Buf(mm, R * LN + zero[0], 8).st(0, pltpu.bitcast(res[r - LAG], U32))
            if fi is not None:
                g = _Buf(G[fi % 2])
                t = jnp.dot(_Buf(U).ld(r * D + fi * CB, CB), mat(r), preferred_element_type=F32)
                g.st(2 * r * CB, t[:, :LN])
                g.st((2 * r + 1) * CB, t[:, LN:])
                yield
            if ii is not None:
                hh = _Buf(HH[ii % 2])
                lhs = jnp.concatenate([hh.ld(2 * r * CB, CB), hh.ld((2 * r + 1) * CB, CB)], axis=1)
                t = lax.dot_general(lhs, mat(r), NT, preferred_element_type=F32)
                _Buf(X).st(r * D + ii * CB, _Buf(Y).ld(r * D + ii * CB, CB) + t)
                yield
            res.append(t[:8, :LN])

    def cmid(i, slot):
        g, hh = _Buf(G[slot], zero[0], 2 * R * CB), _Buf(HH[slot])
        kf = _Buf(KF, i * CB, 2 * R * D - D + CB)
        tw = [_Buf(t) for t in T]
        tr = [_Buf(t, zero[1], 2 * R * CB) for t in T]

        def ld(b, k, h, n=8, stride=CB):
            return b.ld(2 * k * stride + h, n), b.ld((2 * k + 1) * stride + h, n)

        def st(b, k, h, v):
            b.st(2 * k * CB + h, v[0])
            b.st((2 * k + 1) * CB + h, v[1])

        for h in range(0, CB, 8):
            t = []
            for r0 in range(4):
                y = _radix4(*[ld(g, r, h) for r in range(r0, R, 4)], -1)
                t.append([_twiddle(y[g0], r0 * g0, -1) for g0 in range(4)])
                yield
            yield
            for g0 in range(4):
                y = _radix4(t[0][g0], t[1][g0], t[2][g0], t[3][g0], -1)
                yield
                y = [_cmul(y[g1], ld(kf, 4 * g0 + g1, h, 8, D)) for g1 in range(4)]
                yield
                y = _radix4(*y, 1)
                for r0 in range(4):
                    st(tw[h // 16 % 2], 4 * r0 + g0, h, _twiddle(y[r0], r0 * g0, 1))
                yield
                if g0 != 1:
                    yield
            if h % 16:
                for r0 in range(4):
                    y = _radix4(*[ld(tr[h // 16 % 2], 4 * r0 + g0, h - 8, 16) for g0 in range(4)], 1)
                    for r1 in range(4):
                        st(hh, r0 + 4 * r1, h - 8, y[r1])
                    yield
                    yield

    order = list(range(0, R, 2)) + list(range(1, R, 2))
    NCORE, NLN1, NLN2 = 18, 18, 26

    def layer(l, carry):
        @block("ph1")
        def _():
            for n, r in enumerate(order):
                _weave((qkvproj(0, r), 3), *([(ln1(order[n + 1]), NLN1 * 1.5)] if n + 1 < R else []))

        for j, lo, hi in ((1, 0, R), (2, 0, R), (3, 0, R // 2), (3, R // 2, R)):
            @block("ph2")
            def _():
                early = _chain(*[core(3, r) for r in order[:LO if lo else 0]])
                for r in order[lo:hi]:
                    _weave((qkvproj(j, r), 3), (core(j - 1, r), NCORE),
                           (_take(early, -(-LO * NCORE // 8)), LO * NCORE / 8 + 0.01))
                _weave((early, 1))

        for prev, cur in zip(B3, B3[1:]):
            @block("ph3")
            def _():
                w, c, n = (order[u:v] for u, v in zip(prev, cur))
                _weave((_chain(*map(oproj, w)), len(w) * D // DO),
                       (_chain(*[core(3, r) for r in c]), len(c) * NCORE + 0.01),
                       (_chain(*map(ln2, n)), len(n) * NLN2 + 0.01))

        for i in range(-1, NCB + 1):
            @block("conv")
            def _():
                fi, ii = i + 1 if i + 1 < NCB else None, i - 1 if i >= 1 else None
                _weave((cmxu(fi, ii), R * ((fi is not None) + (ii is not None)) * P4),
                       (cmid(i, i % 2) if 0 <= i < NCB else iter(()), 3 * CB),
                       *[(ln2(r), 2 * NLN2) for r in order[B3[-1][2]:] if i < 0])
                if i == NCB:
                    _weave((ln1(0), 1))

        return carry

    _weave((ln1(0), 1))
    with _scope("layers"):
        lax.fori_loop(0, 2, layer, 0)

    ocp = [pltpu.make_async_copy(io.at[j], out_hbm.at[:, pl.ds(j * LN, LN)], sems.at[7 + j])
           for j in range(4)]
    for j in range(4):
        for rho in range(8):
            x = _Buf(X, j * LN, R * D - D + LN)
            w = pltpu.pack_elementwise([x.ld(2 * rho * D, LN), x.ld((2 * rho + 1) * D, LN)],
                                       packed_dtype=BF16).astype(U32)
            iow[j, pl.ds(rho, LN, stride=8), :] = w.T
        ocp[j].start()
    for c in ocp:
        c.wait()


@jax.jit
def pallas_interleave_layers__sliding_local_dilated__ssm_conv_s4__prompt_kernel(
    A_x: jax.Array,
    A_wqkv: jax.Array,
    A_wo: jax.Array,
    B_u: jax.Array,
    B_A_re: jax.Array,
    B_A_im: jax.Array,
    B_B_re: jax.Array,
    B_B_im: jax.Array,
    B_C_re: jax.Array,
    B_C_im: jax.Array,
    B_log_dt: jax.Array,
    B_Dskip: jax.Array,
):
    del B_u
    hbm = pl.BlockSpec(memory_space=pl.ANY)
    vmem = pl.BlockSpec(memory_space=pltpu.VMEM)
    V = pltpu.VMEM
    out = pl.pallas_call(
        _kernel,
        out_shape=jax.ShapeDtypeStruct((S, D), BF16),
        in_specs=[hbm] * 9 + [vmem, vmem, hbm],
        out_specs=hbm,
        scratch_shapes=[
            V((4, S, LN), BF16),
            V((D, 3 * D), BF16),
            V((D, D), BF16),
            V((6, D, LN), BF16),
            V((R * LN + 8, LN), U32),
            V((R * D, LN), F32),
            V((R * D, LN), F32),
            V((2 * R * D, LN), F32),
            V((D, LN), F32),
            V((R * D, LN), BF16),
            V((R * D, LN), BF16),
            V((WROWS, LN), F32),
            [V((D, LN), F32)] * NZ,
            [[V((40 * LN, LN), F32)] * 2] * 2,
            V((R * D, LN), BF16),
            [V((2 * R * CB, LN), F32)] * 2,
            [V((2 * R * CB, LN), F32)] * 2,
            [V((2 * R * CB, LN), BF16)] * 2,
            V((R, D, LN), F32),
            V((R, CB, 2 * LN), F32),
            V((D, LN), F32),
            V((2, 16 * 65, LN), U32),
            V((2, 16 * 65, LN), U32),
            V((16 * 33, LN), F32),
            pltpu.SMEM((R,), jnp.int32),
            pltpu.SemaphoreType.DMA((13,)),
        ],
        compiler_params=pltpu.CompilerParams(vmem_limit_bytes=100 * 1024 * 1024, flags=FLAGS),
    )(A_x.reshape(S, D), A_wqkv, A_wo, B_A_re, B_A_im, B_B_re, B_B_im, B_C_re, B_C_im,
      B_log_dt.reshape(1, D), B_Dskip.reshape(1, D), _M)
    return out.reshape(1, S, D)
```

```python
import contextlib
import numpy as np
import jax
import jax.numpy as jnp
from jax import lax
import jax.experimental.pallas as pl
import jax.experimental.pallas.tpu as pltpu

S, D, DH, WIN = 2048, 512, 16, 8
R = 16
LN = 128
CB = 64
NCB = D // CB
EPS = 1e-5
F32, BF16, U32 = jnp.float32, jnp.bfloat16, jnp.uint32
NT = (((1,), (1,)), ((), ()))


def _dft_matrices():
    lam = np.arange(LN, dtype=np.float64)[None, :, None]
    r = np.arange(R, dtype=np.float64)[:, None, None]
    f = np.arange(LN, dtype=np.float64)[None, None, :]
    th = 2.0 * np.pi * (f + 0.5) * (R * lam + r) / (2 * S)
    m = np.stack([np.cos(th), -np.sin(th)], axis=1).astype(BF16).view(np.uint16).astype(np.uint32)
    return (m[:, :, 0::2] | (m[:, :, 1::2] << 16)).reshape(R * LN, LN)


_M = _dft_matrices()


SCOPES = False


def _scope(name):
    return jax.named_scope(name) if SCOPES else contextlib.nullcontext()


FLAGS = None
NK = 8
SKIP = NOB = ''
LO, NZ = 8, 16
B3 = ((0, 8, 0), (4, 12, 0), (9, 16, 4), (14, 16, 9), (16, 16, 14))
DO = 256
TS, WS, SS = LN, 2 * D, LN + 1


class _Buf:
    def __init__(self, ref, base=0, size=None):
        if isinstance(base, int):
            self.ref, self.base = ref, base
        else:
            self.ref, self.base = ref.at[pl.ds(pl.multiple_of(base, 16), size), :], 0

    def ld(self, row, n):
        return self.ref[self.base + row:self.base + row + n, :]

    def st(self, row, v):
        self.ref[self.base + row:self.base + row + v.shape[0], :] = v.astype(self.ref.dtype)


def _weave(*stages):
    live = [[g, n, 0] for g, n in stages]
    while live:
        st = min(live, key=lambda t: t[2] / t[1])
        try:
            next(st[0])
            st[2] += 1
        except StopIteration:
            live.remove(st)


def _chain(*gens):
    for g in gens:
        yield from g


def _take(g, n):
    for _, _ in zip(range(n), g):
        yield


def _tree(op, v):
    while len(v) > 1:
        v = [op(v[i], v[i + 1]) for i in range(0, len(v), 2)]
    return v[0]


def _mult(i, n):
    return i if isinstance(i, int) else pl.multiple_of(i, n)


def _loop(lo, hi, body, unroll, force=False):
    n = hi - lo
    assert n % unroll == 0
    if n == unroll and not force:
        for i in range(lo, hi):
            body(i)
        return

    def outer(k, carry):
        for u in range(unroll):
            body(lo + k * unroll + u)
        return carry

    lax.fori_loop(0, n // unroll, outer, 0)


def _iota(shape, dim):
    return lax.broadcasted_iota(jnp.int32, shape, dim)


def _cmul(a, b):
    return (a[0] * b[0] - a[1] * b[1], a[0] * b[1] + a[1] * b[0])


def _csq(a):
    t = a[0] * a[1]
    return (a[0] * a[0] - a[1] * a[1], t + t)


def _radix4(a, b, c, d, sign):
    s0 = (a[0] + c[0], a[1] + c[1])
    d0 = (a[0] - c[0], a[1] - c[1])
    s1 = (b[0] + d[0], b[1] + d[1])
    d1 = (b[0] - d[0], b[1] - d[1])
    y0 = (s0[0] + s1[0], s0[1] + s1[1])
    y2 = (s0[0] - s1[0], s0[1] - s1[1])
    p = (d0[0] - d1[1], d0[1] + d1[0])
    m = (d0[0] + d1[1], d0[1] - d1[0])
    return (y0, p, y2, m) if sign > 0 else (y0, m, y2, p)


def _twiddle(a, k, sign):
    if k == 0:
        return a
    c = float(np.cos(2 * np.pi * k / 16))
    s = float(sign * np.sin(2 * np.pi * k / 16))
    if k == 4:
        return (-a[1], a[0]) if sign > 0 else (a[1], -a[0])
    if k == 2:
        if sign > 0:
            return ((a[0] - a[1]) * c, (a[0] + a[1]) * c)
        return ((a[0] + a[1]) * c, (a[1] - a[0]) * c)
    if k == 6:
        if sign > 0:
            return ((a[0] + a[1]) * c, (a[1] - a[0]) * c)
        return ((a[0] - a[1]) * c, (a[0] + a[1]) * c)
    return (a[0] * c - a[1] * s, a[0] * s + a[1] * c)


def _kernel(x_hbm, wqkv_hbm, wo_hbm, are_hbm, aim_hbm, bre_hbm, bim_hbm, cre_hbm, cim_hbm,
            ldt_hbm, dsk_hbm, m_hbm, out_hbm, ldt_ref, dsk_ref,
            io, wraw, woraw, par, mm, X, Y, KF, DSK, XN, U, W, Z, KVQ, O, G, T, HH,
            KT, PF, E, DT, SA, SB, KO, zero, sems):
    for k in range(R):
        zero[k] = 0

    def block(name):
        def deco(f):
            if SKIP and name in SKIP:
                return
            with _scope(name):
                f() if name in NOB else pl.when(zero[0] == 0)(f)
        return deco

    def opaque(r):
        return zero[r] if isinstance(r, int) else 0

    pcp = [pltpu.make_async_copy(h, par.at[i], sems.at[i])
           for i, h in enumerate((are_hbm, aim_hbm, bre_hbm, bim_hbm, cre_hbm, cim_hbm))]
    mcp = pltpu.make_async_copy(m_hbm, mm, sems.at[6])
    xcp = [pltpu.make_async_copy(x_hbm.at[:, pl.ds(j * LN, LN)], io.at[j], sems.at[7 + j])
           for j in range(4)]
    wocp = pltpu.make_async_copy(wo_hbm, woraw, sems.at[11])
    wcp = [pltpu.make_async_copy(wqkv_hbm.at[:, pl.ds(j * LN, LN)], wraw.at[j], sems.at[12 + j])
           for j in range(12)]
    scp = [pltpu.make_async_copy(ldt_hbm, ldt_ref, sems.at[24]),
           pltpu.make_async_copy(dsk_hbm, dsk_ref, sems.at[25])]
    for c in scp + pcp + [mcp] + xcp + wcp + [wocp]:
        c.start()

    for sb in SB:
        for c in range(2):
            for row in range(32):
                o = row // 4 * SS + row % 4 * 32 + 28
                sb[c, o:o + 4, :] = jnp.zeros((4, LN), F32)

    for c in scp:
        c.wait()
    dt_row = jnp.exp(ldt_ref[...].astype(F32).reshape(1, D)).astype(BF16).astype(F32)
    ds_row = dsk_ref[...].astype(F32).reshape(1, D)
    for j in range(4):
        sl = slice(j * LN, (j + 1) * LN)
        DT[sl, :] = jnp.broadcast_to(dt_row[:, sl], (LN, LN)).T
        DSK[sl, :] = jnp.broadcast_to(ds_row[:, sl], (LN, LN)).T
    with _scope('pwait'):
        for c in pcp:
            c.wait()

    lane = _iota((8, LN), 1)

    def kpar(J, carry):
        rows = pl.ds(pl.multiple_of(J * 64, 64), 64)
        for i in range(6):
            PF[i, rows, :] = par[i, rows, :].astype(F32)
        return carry

    def kexp(J, slot):
        for s in range(4):
            rows = pl.ds(_mult(s * LN + J * 8, 8), 8)
            dt = DT[rows, :]
            zr, zi = dt * PF[0, rows, :], dt * PF[1, rows, :]
            mag = jnp.exp(zr)
            E[slot][0, s] = mag * jnp.cos(zi)
            yield
            E[slot][1, s] = mag * jnp.sin(zi)
            w = _cmul((PF[4, rows, :], PF[5, rows, :]), (dt * PF[2, rows, :], dt * PF[3, rows, :]))
            E[slot][2, s] = w[0] * (1.0 / S)
            E[slot][3, s] = w[1] * (1.0 / S)
            yield

    def kpow(J, slot):
        sa, sb = SA[slot], SB[slot]
        for s in range(4):
            def put(ref, i, v):
                ref[0, pl.ds(s * 32 + i, 8, stride=SS), :] = v[0]
                ref[1, pl.ds(s * 32 + i, 8, stride=SS), :] = v[1]

            p = (E[slot][0, s], E[slot][1, s])
            b = [(jnp.ones_like(p[0]), jnp.zeros_like(p[0]))]
            put(sb, 0, b[0])
            for k in range(4):
                for i in range(2 ** k):
                    b.append(_cmul(b[i], p) if i else p)
                    put(sb, len(b) - 1, b[-1])
                    yield
                p = _csq(p)
            put(sb, 16, p)
            b = {4: b[4], 8: b[8], 12: b[12], 16: p}
            w = (E[slot][2, s], E[slot][3, s])
            pw = []
            for k in range(5):
                pw.append(p)
                p = _csq(p)
                yield
            e512, e1024 = p, _csq(p)
            for o, st, e in ((17, 4, e512), (22, 8, e1024), (25, 8, _cmul(e512, e1024))):
                put(sb, o, e)
                for i in range(1, 16 // st + 1):
                    put(sb, o + i, _cmul(e, b[i * st]))
                    yield

            def tree(i, v, k):
                put(sa, i, v)
                yield
                for k2 in range(k):
                    yield from tree(i + 2 ** k2, _cmul(v, pw[k2]), k2)

            yield from tree(0, w, 5)

    def ksum(J, slot):
        sa, sb = SA[slot], SB[slot]
        q32 = _iota((32, LN), 1) >> 5
        for m in range(8):
            o = [lax.dot_general(sb[c, m * SS:m * SS + LN, :].astype(BF16),
                                 sa[c, m * SS:m * SS + LN, :].astype(BF16),
                                 NT, preferred_element_type=F32) for c in range(2)]
            o = o[0] - o[1]
            KO[slot][m * 33:m * 33 + 32, :] = jnp.where(
                q32 < 2, jnp.where(q32 == 0, o[0:32], o[32:64]),
                jnp.where(q32 == 2, o[64:96], o[96:128]))
            yield

    def kspread(J, slot):
        kb = lambda i: KO[slot][pl.ds(i, 8, stride=33), :]
        rnd = lambda r, st: int(np.round(r / st))
        quarter, low = lane >> 5, (lane & 31) < 16
        q1 = [pltpu.roll(kb(i), 32, 1) for i in range(17, 22)]
        q2 = [pltpu.roll(kb(i), 64, 1) for i in range(22, 25)]
        q3 = [pltpu.roll(kb(i), 96, 1) for i in range(25, 28)]
        for k8 in range(3):
            q23 = [jnp.where(quarter == (s + 2) % 4, q2[k8], q3[k8]) for s in range(4)]
            for k4 in range(5):
                rs = [r for r in range(R) if (rnd(r, 4), rnd(r, 8)) == (k4, k8)]
                rest = [jnp.where(quarter == (s + 1) % 4, q1[k4], q23[s]) for s in range(4) if rs]
                for r in rs:
                    q0 = kb(r) if r % 2 == 0 else jnp.where(low, kb(r), kb(2 * rnd(r, 2)))
                    for s in range(4):
                        KT[pl.ds(_mult(r * D + s * LN + J * 8, 8), 8), :] = jnp.where(
                            quarter == s, q0, rest[s])
                    yield

    def kstep(J, slot, e=True, a=True, b=True, c=True):
        @block("kgen")
        def _():
            _weave(*([(ksum(J, slot), NK)] if b else []),
                   *([(kpow(J + 1, 1 - slot), 4 * 60)] if a else []),
                   *([(kexp(jnp.minimum(J + 2, 15), slot), 8)] if e else []),
                   *([(kspread(J - 1, 1 - slot), 16)] if c else []))

    lax.fori_loop(0, D // 64, kpar, 0)
    kstep(-2, 0, a=False, b=False, c=False)
    kstep(-1, 1, b=False, c=False)
    kstep(0, 0, c=False)
    _loop(0, 7, lambda k: (kstep(2 * k + 1, 1), kstep(2 * k + 2, 0)), 1)
    kstep(15, 1, e=False, a=False)

    def ld(b, k, h, n=8, stride=CB):
        return b.ld(2 * k * stride + h, n), b.ld((2 * k + 1) * stride + h, n)

    def st(b, k, h, v, stride=CB):
        b.st(2 * k * stride + h, v[0])
        b.st((2 * k + 1) * stride + h, v[1])

    def kfwd(s, half):
        kt = _Buf(KT, s * LN + half * CB, R * D - D + CB)
        ms = [_Buf(mm, (p + 4 - s) % 4 * 16, R * LN - 48) for p in range(4)]
        for r in range(R):
            mr = jnp.concatenate(
                [jnp.concatenate([m.ld(r * LN + c * 64, 16) for m in ms], axis=0) for c in range(2)],
                axis=1)
            t = jnp.dot(kt.ld(r * D, CB).astype(BF16), pltpu.bitcast(mr, BF16),
                        preferred_element_type=F32)
            st(_Buf(G[half]), r, 0, (t[:, :LN], t[:, LN:]))
            yield

    def kfft(s, half):
        kf = _Buf(KF, s * LN + half * CB, 2 * R * D - D + CB)
        for h in range(0, CB, 8):
            t = []
            for r0 in range(4):
                y = _radix4(*[ld(_Buf(G[half]), r, h) for r in range(r0, R, 4)], -1)
                t.append([_twiddle(y[g0], r0 * g0, -1) for g0 in range(4)])
                yield
            for g0 in range(4):
                y = _radix4(t[0][g0], t[1][g0], t[2][g0], t[3][g0], -1)
                for g1 in range(4):
                    st(kf, 4 * g0 + g1, h, y[g1], D)
                yield

    iow = io.bitcast(U32)

    def xin(j, half):
        x = _Buf(X, j * LN, R * D - D + LN)
        for rho in range(4 * half, 4 * half + 4):
            t = iow[j, pl.ds(rho, LN, stride=8), :].T
            x.st(2 * rho * D, pltpu.bitcast(t << 16, F32))
            x.st((2 * rho + 1) * D, pltpu.bitcast(t & np.uint32(0xFFFF0000), F32))
            yield

    def wprep(j, half):
        pr, pc = _iota((LN, LN), 0), _iota((LN, LN), 1)
        perm = jnp.where(pc == (pr & 7) * DH + (pr >> 3), 1.0, 0.0).astype(BF16)
        w = _Buf(W, 3 * j * LN // 2, 3 * WS + 3 * LN // 2)
        for c in ((0, 1), (2,))[half]:
            t = lax.dot_general(perm, wraw[(c + 1) % 3 * 4 + j], NT, preferred_element_type=F32)
            if c == 2:
                t = t * (DH ** -0.5)
            for k in range(4):
                w.st(k * WS + c * LN // 2,
                     pltpu.bitcast(t[:, k * LN:(k + 1) * LN].astype(BF16), F32))
            yield
        if half:
            t = jnp.dot(perm, woraw[pl.ds(pl.multiple_of(j * LN, LN), LN), :],
                        preferred_element_type=F32)
            _Buf(W, j * WS + 3 * D // 2, D // 2).st(0, pltpu.bitcast(t.T.astype(BF16), F32))
            yield

    with _scope("mwait"):
        mcp.wait()

    @block("kf")
    def _():
        _weave((kspread(15, 1), 16), (kfwd(0, 0), 16))

    with _scope("xwait"):
        for c in xcp + wcp + [wocp]:
            c.wait()

    def prep(s):
        for half in range(2):
            @block("kf")
            def _():
                nxt = kfwd(jnp.minimum(s + 1, 3), 0) if half else kfwd(s, 1)
                _weave((nxt, 16), (kfft(s, half), 64), (xin(s, half), 4), (wprep(s, half), 2))

    _loop(0, 4, prep, 1)

    def colsum(f, step):
        acc = [f(c * 8) for c in range(4)]
        for i in range(4, D // 8):
            acc[i % 4] = acc[i % 4] + f(i * 8)
            if i % step == step - 1:
                yield
        s = jnp.sum((acc[0] + acc[1]) + (acc[2] + acc[3]), axis=0, keepdims=True)
        return jnp.broadcast_to(s * (1.0 / D), (8, LN))

    def ln_stats(ref, base):
        x = _Buf(ref, base + zero[0], D)
        m = yield from colsum(lambda c: x.ld(c, 8), 32)
        x = _Buf(ref, base + zero[1], D)
        v = yield from colsum(lambda c: jnp.square(x.ld(c, 8) - m), 8)
        return _Buf(ref, base + zero[2], D), m, lax.rsqrt(v + EPS)

    def ln1(r):
        x, m, rs = yield from ln_stats(X, r * D)
        for c in range(0, D, 16):
            t = [(x.ld(c + k, 8) - m) * rs for k in (0, 8)]
            _Buf(XN, r * D).st(c, jnp.concatenate(t, axis=0))
            if c % 64 == 48:
                yield

    def ln2(r):
        x, m, rs = yield from ln_stats(Z[order.index(r) % NZ], 0)
        dsk = _Buf(DSK, zero[r], D)
        for c in range(0, D, 16):
            t = []
            for k in (c, c + 8):
                v = x.ld(k, 8)
                t.append((v - m) * rs)
                _Buf(Y, r * D).st(k, v + t[-1] * dsk.ld(k, 8))
            _Buf(U, r * D).st(c, jnp.concatenate(t, axis=0))
            if c % 64 == 48:
                yield
                yield

    def wdot(c, n, rhs):
        lhs = jnp.concatenate(
            [pltpu.bitcast(W[t * WS + c // 2:t * WS + (c + n) // 2, :], BF16)
             for t in range(4)], axis=1)
        return jnp.dot(lhs, rhs.ld(0, D), preferred_element_type=F32)

    def qkvproj(j, r):
        b, i = _Buf(KVQ[j % 2][r % 2]), r // 2
        for c in range(3):
            t = wdot((3 * j + c) * LN, LN, _Buf(XN, r * D + zero[(r + c) % R], D))
            if c == 2:
                b.st((32 + i) * TS, t)
            else:
                b.st((16 * c + 8 + i) * TS, t)
                if i:
                    b.st((16 * c + i) * TS, pltpu.roll(t, 1, 1))
            yield

    def core(j, r):
        b, i = _Buf(KVQ[j % 2][r % 2], zero[r], 40 * TS), r // 2
        lg = [None] * WIN
        for dh in range(DH):
            q = b.ld((32 + i) * TS + dh * 8, 8)
            for w in range(WIN):
                t = q * b.ld((8 + i - w) * TS + dh * 8, 8)
                lg[w] = t if dh == 0 else lg[w] + t
            if dh % 2:
                yield
        for w in range(i + 1, WIN):
            lg[w] = jnp.where(lane > 0, lg[w], -1e9)
        mx = _tree(jnp.maximum, lg)
        e = [jnp.exp(v - mx) for v in lg]
        inv = 1.0 / _tree(jnp.add, e)
        e = [v * inv for v in e]
        yield
        yield
        for dh in range(0, DH, 2):
            oo = []
            for k in (dh, dh + 1):
                acc = None
                for w in range(WIN):
                    t = e[w] * b.ld((24 + i - w) * TS + k * 8, 8)
                    acc = t if acc is None else acc + t
                oo.append(acc)
            _Buf(O, r * D + j * LN).st(dh * 8, jnp.concatenate(oo, axis=0))
            yield

    def oproj(r):
        for c in range(0, D, DO):
            Z[order.index(r) % NZ][c:c + DO, :] = X[r * D + c:r * D + c + DO, :] + wdot(
                3 * D + c, DO, _Buf(O, r * D + zero[(r + c // DO) % R], D))
            yield

    def mat(r):
        return pltpu.bitcast(jnp.concatenate(
            [mm[2 * r * 64:(2 * r + 1) * 64, :], mm[(2 * r + 1) * 64:(2 * r + 2) * 64, :]], axis=1),
            BF16)

    def cmxu(fi, ii, slot):
        if fi is not None:
            u_ = _Buf(U, fi * CB, R * D - D + CB)
        if ii is not None:
            x, y = _Buf(X, ii * CB, R * D - D + CB), _Buf(Y, ii * CB, R * D - D + CB)
        for r in order:
            if fi is not None:
                t = jnp.dot(u_.ld(r * D, CB), mat(r), preferred_element_type=F32)
                st(_Buf(G[slot]), r, 0, (t[:, :LN], t[:, LN:]))
                yield
            if ii is not None:
                lhs = jnp.concatenate(ld(_Buf(HH[slot]), r, 0, CB), axis=1)
                t = lax.dot_general(lhs, mat(r), NT, preferred_element_type=F32)
                x.st(r * D, y.ld(r * D, CB) + t)
                yield

    def cmid(i, slot):
        g, hh = _Buf(G[slot], zero[0], 2 * R * CB), _Buf(HH[slot])
        kf = _Buf(KF, i * CB, 2 * R * D - D + CB)
        tw = [_Buf(t) for t in T]
        tr = [_Buf(t, zero[1], 2 * R * CB) for t in T]

        for h in range(0, CB, 8):
            t = []
            for r0 in range(4):
                y = _radix4(*[ld(g, r, h) for r in range(r0, R, 4)], -1)
                t.append([_twiddle(y[g0], r0 * g0, -1) for g0 in range(4)])
                yield
            yield
            for g0 in range(4):
                y = _radix4(t[0][g0], t[1][g0], t[2][g0], t[3][g0], -1)
                yield
                y = [_cmul(y[g1], ld(kf, 4 * g0 + g1, h, 8, D)) for g1 in range(4)]
                yield
                y = _radix4(*y, 1)
                for r0 in range(4):
                    st(tw[h // 16 % 2], 4 * r0 + g0, h, _twiddle(y[r0], r0 * g0, 1))
                yield
                if g0 != 1:
                    yield
            if h % 16:
                for r0 in range(4):
                    y = _radix4(*[ld(tr[h // 16 % 2], 4 * r0 + g0, h - 8, 16) for g0 in range(4)], 1)
                    for r1 in range(4):
                        st(hh, r0 + 4 * r1, h - 8, y[r1])
                    yield
                    yield

    def ocopy(j):
        return pltpu.make_async_copy(
            io.at[j], out_hbm.at[:, pl.ds(_mult(j * LN, LN), LN)], sems.at[7 + j])

    def xout(j):
        x = _Buf(X, j * LN, R * D - D + LN)
        for rho in range(8):
            lo, hi = (pltpu.bitcast(x.ld(r * D, LN).astype(BF16).astype(F32), U32)
                      for r in (2 * rho, 2 * rho + 1))
            iow[j, pl.ds(rho, LN, stride=8), :] = ((lo >> 16) | hi).T
        ocopy(j).start()

    order = list(range(0, R, 2)) + list(range(1, R, 2))
    NCORE, NLN1, NLN2 = 18, 18, 26

    def layer(l, carry):
        @block("ph1")
        def _():
            for n, r in enumerate(order):
                _weave((qkvproj(0, r), 3), *([(ln1(order[n + 1]), NLN1 * 1.5)] if n + 1 < R else []))

        for j, lo, hi in ((1, 0, R), (2, 0, R), (3, 0, R // 2), (3, R // 2, R)):
            @block("ph2")
            def _():
                early = _chain(*[core(3, r) for r in order[:LO if lo else 0]])
                for r in order[lo:hi]:
                    _weave((qkvproj(j, r), 3), (core(j - 1, r), NCORE),
                           (_take(early, -(-LO * NCORE // 8)), LO * NCORE / 8 + 0.01))
                _weave((early, 1))

        for prev, cur in zip(B3, B3[1:]):
            @block("ph3")
            def _():
                w, c, n = (order[u:v] for u, v in zip(prev, cur))
                _weave((_chain(*map(oproj, w)), len(w) * D // DO),
                       (_chain(*[core(3, r) for r in c]), len(c) * NCORE + 0.01),
                       (_chain(*map(ln2, n)), len(n) * NLN2 + 0.01))

        def cstep(i, slot, f=True, m=True, v=True):
            @block("conv")
            def _():
                _weave((cmxu(i + 1 if f else None, i - 1 if v else None, 1 - slot), R * (f + v)),
                       *([(cmid(i, slot), 3 * CB)] if m else []),
                       *[(ln2(r), 2 * NLN2) for r in order[B3[-1][2]:] if f and not m])
                if v and not m:
                    _weave((ln1(0), 1))

        cstep(-1, 1, m=False, v=False)
        cstep(0, 0, v=False)

        def cpair(k):
            cstep(2 * k + 1, 1)
            cstep(2 * k + 2, 0)
            pl.when(l == 1)(lambda: xout(k))

        _loop(0, NCB // 2 - 1, cpair, 1)
        cstep(NCB - 1, 1, f=False)
        cstep(NCB, 0, f=False, m=False)
        return carry

    _weave((ln1(0), 1))
    with _scope("layers"):
        lax.fori_loop(0, 2, layer, 0)
    xout(3)

    with _scope("owait"):
        for j in range(4):
            ocopy(j).wait()


@jax.jit
def pallas_interleave_layers__sliding_local_dilated__ssm_conv_s4__prompt_kernel(
    A_x: jax.Array,
    A_wqkv: jax.Array,
    A_wo: jax.Array,
    B_u: jax.Array,
    B_A_re: jax.Array,
    B_A_im: jax.Array,
    B_B_re: jax.Array,
    B_B_im: jax.Array,
    B_C_re: jax.Array,
    B_C_im: jax.Array,
    B_log_dt: jax.Array,
    B_Dskip: jax.Array,
):
    del B_u
    hbm = pl.BlockSpec(memory_space=pl.ANY)
    V = pltpu.VMEM
    out = pl.pallas_call(
        _kernel,
        out_shape=jax.ShapeDtypeStruct((S, D), BF16),
        in_specs=[hbm] * 12,
        out_specs=hbm,
        scratch_shapes=[
            V((D,), BF16), V((D,), BF16),
            V((4, S, LN), BF16),
            V((12, D, LN), BF16),
            V((D, D), BF16),
            V((6, D, LN), BF16),
            V((R * LN, LN), U32),
            V((R * D, LN), F32),
            V((R * D, LN), F32),
            V((2 * R * D, LN), F32),
            V((D, LN), F32),
            V((R * D, LN), BF16),
            V((R * D, LN), BF16),
            V((4 * WS, LN), F32),
            [V((D, LN), F32)] * NZ,
            [[V((40 * TS, LN), F32)] * 2] * 2,
            V((R * D, LN), BF16),
            [V((2 * R * CB, LN), F32)] * 2,
            [V((2 * R * CB, LN), F32)] * 2,
            [V((2 * R * CB, LN), BF16)] * 2,
            V((R * D, LN), F32),
            V((6, D, LN), F32),
            [V((4, 4, 8, LN), F32)] * 2,
            V((D, LN), F32),
            [V((2, 8 * SS, LN), F32)] * 2,
            [V((2, 8 * SS, LN), F32)] * 2,
            [V((8 * 33, LN), F32)] * 2,
            pltpu.SMEM((R,), jnp.int32),
            pltpu.SemaphoreType.DMA((26,)),
        ],
        compiler_params=pltpu.CompilerParams(vmem_limit_bytes=100 * 1024 * 1024, flags=FLAGS),
    )(A_x.reshape(S, D), A_wqkv, A_wo, B_A_re, B_A_im, B_B_re, B_B_im, B_C_re, B_C_im,
      B_log_dt, B_Dskip, _M)
    return out.reshape(1, S, D)
```

```python
import contextlib
import numpy as np
import jax
import jax.numpy as jnp
from jax import lax
import jax.experimental.pallas as pl
import jax.experimental.pallas.tpu as pltpu

S, D, DH, WIN = 2048, 512, 16, 8
R = 16
LN = 128
CB = 64
NCB = D // CB
EPS = 1e-5
F32, BF16, U32 = jnp.float32, jnp.bfloat16, jnp.uint32
NN, NT = (((1,), (0,)), ((), ())), (((1,), (1,)), ((), ()))


def _dft_matrices():
    lam = np.arange(LN, dtype=np.float64)[None, :, None]
    r = np.arange(R, dtype=np.float64)[:, None, None]
    f = np.arange(LN, dtype=np.float64)[None, None, :]
    th = 2.0 * np.pi * (f + 0.5) * (R * lam + r) / (2 * S)
    m = np.stack([np.cos(th), -np.sin(th)], axis=1).astype(BF16).view(np.uint16).astype(np.uint32)
    return (m[:, :, 0::2] | (m[:, :, 1::2] << 16)).reshape(R * LN, LN)


_M = _dft_matrices()


SCOPES = False


def _scope(name):
    return jax.named_scope(name) if SCOPES else contextlib.nullcontext()


FLAGS = None
SKIP = NOB = ''
LO = 6
KB = {1: (0, 1, 2), 2: (3, 4, 5), 3: (6, 7)}
B3 = ((0, 6, 0), (5, 11, 0), (10, 16, 5), (14, 16, 10), (16, 16, 14))
DO = 256
TS, WS, SS = LN, 2 * D, LN + 1


class _Buf:
    def __init__(self, ref, base=0, size=None):
        if isinstance(base, int):
            self.ref, self.base = ref, base
        else:
            self.ref, self.base = ref.at[pl.ds(pl.multiple_of(base, 16), size), :], 0

    def ld(self, row, n):
        return self.ref[self.base + row:self.base + row + n, :]

    def st(self, row, v):
        self.ref[self.base + row:self.base + row + v.shape[0], :] = v.astype(self.ref.dtype)


def _weave(*stages):
    live = [[g, n, 0] for g, n in stages]
    while live:
        st = min(live, key=lambda t: t[2] / t[1])
        try:
            next(st[0])
            st[2] += 1
        except StopIteration:
            live.remove(st)


def _chain(*gens):
    for g in gens:
        yield from g


def _take(g, n):
    for _, _ in zip(range(n), g):
        yield


def _tree(op, v):
    while len(v) > 1:
        v = [op(v[i], v[i + 1]) for i in range(0, len(v), 2)]
    return v[0]


def _mult(i, n):
    return i if isinstance(i, int) else pl.multiple_of(i, n)


def _loop(lo, hi, body, unroll, force=False):
    n = hi - lo
    assert n % unroll == 0
    if n == unroll and not force:
        for i in range(lo, hi):
            body(i)
        return

    def outer(k, carry):
        for u in range(unroll):
            body(lo + k * unroll + u)
        return carry

    lax.fori_loop(0, n // unroll, outer, 0)


def _iota(shape, dim):
    return lax.broadcasted_iota(jnp.int32, shape, dim)


def _cmul(a, b):
    return (a[0] * b[0] - a[1] * b[1], a[0] * b[1] + a[1] * b[0])


def _csq(a):
    t = a[0] * a[1]
    return (a[0] * a[0] - a[1] * a[1], t + t)


def _radix4(a, b, c, d, sign):
    s0 = (a[0] + c[0], a[1] + c[1])
    d0 = (a[0] - c[0], a[1] - c[1])
    s1 = (b[0] + d[0], b[1] + d[1])
    d1 = (b[0] - d[0], b[1] - d[1])
    y0 = (s0[0] + s1[0], s0[1] + s1[1])
    y2 = (s0[0] - s1[0], s0[1] - s1[1])
    p = (d0[0] - d1[1], d0[1] + d1[0])
    m = (d0[0] + d1[1], d0[1] - d1[0])
    return (y0, p, y2, m) if sign > 0 else (y0, m, y2, p)


def _twiddle(a, k, sign):
    if k == 0:
        return a
    c = float(np.cos(2 * np.pi * k / 16))
    s = float(sign * np.sin(2 * np.pi * k / 16))
    if k == 4:
        return (-a[1], a[0]) if sign > 0 else (a[1], -a[0])
    if k == 2:
        if sign > 0:
            return ((a[0] - a[1]) * c, (a[0] + a[1]) * c)
        return ((a[0] + a[1]) * c, (a[1] - a[0]) * c)
    if k == 6:
        if sign > 0:
            return ((a[0] + a[1]) * c, (a[1] - a[0]) * c)
        return ((a[0] - a[1]) * c, (a[0] + a[1]) * c)
    return (a[0] * c - a[1] * s, a[0] * s + a[1] * c)


def _kernel(x_hbm, wqkv_hbm, wo_hbm, are_hbm, aim_hbm, bre_hbm, bim_hbm, cre_hbm, cim_hbm,
            ldt_hbm, dsk_hbm, m_hbm, out_hbm, ldt_ref, dsk_ref,
            io, wraw, woraw, par, mm, X, KF, DSK, XN, U, W, Z, KVQ, O, G, HH,
            KT, GK, PF, E, DT, SA, SB, KO, zero, sems):
    for k in range(R):
        zero[k] = 0

    def block(name):
        def deco(f):
            if SKIP and name in SKIP:
                return
            with _scope(name):
                f() if name in NOB else pl.when(zero[0] == 0)(f)
        return deco

    def opaque(r):
        return zero[r] if isinstance(r, int) else 0

    pcp = [pltpu.make_async_copy(h, par.at[i], sems.at[i])
           for i, h in enumerate((are_hbm, aim_hbm, bre_hbm, bim_hbm, cre_hbm, cim_hbm))]
    mcp = pltpu.make_async_copy(m_hbm, mm, sems.at[6])
    xcp = [pltpu.make_async_copy(x_hbm.at[:, pl.ds(j * LN, LN)], io.at[j], sems.at[7 + j])
           for j in range(4)]
    wocp = pltpu.make_async_copy(wo_hbm, woraw, sems.at[11])
    wcp = [pltpu.make_async_copy(wqkv_hbm.at[:, pl.ds(j * LN, LN)], wraw.at[j], sems.at[12 + j])
           for j in range(12)]
    scp = [pltpu.make_async_copy(ldt_hbm, ldt_ref, sems.at[24]),
           pltpu.make_async_copy(dsk_hbm, dsk_ref, sems.at[25])]
    for c in scp + pcp + [mcp] + xcp + wcp + [wocp]:
        c.start()

    for sb in SB:
        for c in range(4):
            head = jnp.where(_iota((8, LN), 0) == 0, 1.0 - c % 2, 0.0)
            for row in range(32):
                o = row // 4 * SS + row % 4 * 32
                sb[c, o:o + 8, :] = head
                sb[c, o + 24:o + 32, :] = jnp.zeros((8, LN), F32)

    for c in scp:
        c.wait()
    dt_row = jnp.exp(ldt_ref[...].astype(F32).reshape(1, D)).astype(BF16).astype(F32)
    ds_row = dsk_ref[...].astype(F32).reshape(1, D)
    for j in range(4):
        sl = slice(j * LN, (j + 1) * LN)
        DT[sl, :] = jnp.broadcast_to(dt_row[:, sl], (LN, LN)).T
        DSK[sl, :] = jnp.broadcast_to(ds_row[:, sl], (LN, LN)).T
    with _scope('pwait'):
        for c in pcp:
            c.wait()

    lane = _iota((8, LN), 1)

    def kpar(J, carry):
        rows = pl.ds(pl.multiple_of(J * 64, 64), 64)
        for i in range(6):
            PF[i, rows, :] = par[i, rows, :].astype(F32)
        return carry

    def kexp(J, slot):
        for s in range(8):
            rows = pl.ds(_mult(J * CB + s * 8, 8), 8)
            dt = DT[rows, :]
            zr, zi = dt * PF[0, rows, :], dt * PF[1, rows, :]
            mag = jnp.exp(zr)
            E[slot][0, s] = mag * jnp.cos(zi)
            yield
            E[slot][1, s] = mag * jnp.sin(zi)
            w = _cmul((PF[4, rows, :], PF[5, rows, :]), (dt * PF[2, rows, :], dt * PF[3, rows, :]))
            E[slot][2, s] = w[0] * (1.0 / S)
            E[slot][3, s] = w[1] * (1.0 / S)
            yield

    def kpow(J, slot):
        sa, sb = SA[slot], SB[slot]
        for s in range(8):
            def put(ref, i, v):
                for c in range(2):
                    ref[s // 4 * 2 + c, pl.ds(s % 4 * 32 + i, 8, stride=SS), :] = v[c]

            p = (E[slot][0, s], E[slot][1, s])
            b = [None]
            for k in range(4):
                for i in range(2 ** k):
                    b.append(_cmul(b[i], p) if i else p)
                    put(sb, len(b) - 1, b[-1])
                    yield
                p = _csq(p)
            put(sb, 16, p)
            b = {4: b[4], 8: b[8], 12: b[12], 16: p}
            w = (E[slot][2, s], E[slot][3, s])
            pw = []
            for k in range(5):
                pw.append(p)
                p = _csq(p)
                yield
            e512, e1024 = p, _csq(p)
            for o, st, e in ((17, 4, e512), (22, 8, e1024), (25, 8, _cmul(e512, e1024))):
                put(sb, o, e)
                for i in range(1, 16 // st + 1):
                    put(sb, o + i, _cmul(e, b[i * st]))
                    yield

            def tree(i, v, k):
                put(sa, i, v)
                yield
                for k2 in range(k):
                    yield from tree(i + 2 ** k2, _cmul(v, pw[k2]), k2)

            yield from tree(0, w, 5)

    def ksum(J, slot):
        sa, sb = SA[slot], SB[slot]
        q32 = _iota((32, LN), 1) >> 5
        for hm in range(16):
            h, m = divmod(hm, 8)
            o = [lax.dot_general(sb[2 * h + c, m * SS:m * SS + LN, :],
                                 sa[2 * h + c, m * SS:m * SS + LN, :],
                                 NT, preferred_element_type=F32) for c in range(2)]
            o = o[0] - o[1]
            KO[slot][h, m * 33:m * 33 + 32, :] = jnp.where(
                q32 < 2, jnp.where(q32 == 0, o[0:32], o[32:64]),
                jnp.where(q32 == 2, o[64:96], o[96:128]))
            yield

    def kspread(J, slot, h):
        kb = lambda i: KO[slot][h, pl.ds(i, 8, stride=33), :]
        rnd = lambda r, st: int(np.round(r / st))
        quarter, low = lane >> 5, (lane & 31) < 16
        q1 = [pltpu.roll(kb(i), 32, 1) for i in range(17, 22)]
        q2 = [pltpu.roll(kb(i), 64, 1) for i in range(22, 25)]
        q3 = [pltpu.roll(kb(i), 96, 1) for i in range(25, 28)]
        for k8 in range(3):
            q23 = [jnp.where(quarter == (s + 2) % 4, q2[k8], q3[k8]) for s in range(4)]
            for k4 in range(5):
                rs = [r for r in range(R) if (rnd(r, 4), rnd(r, 8)) == (k4, k8)]
                rest = [jnp.where(quarter == (s + 1) % 4, q1[k4], q23[s]) for s in range(4) if rs]
                for r in rs:
                    q0 = kb(r) if r % 2 == 0 else jnp.where(low, kb(r), kb(2 * rnd(r, 2)))
                    for s in range(4):
                        t = jnp.where(quarter == s, q0, rest[s])
                        if s:
                            t = pltpu.roll(t, LN - 32 * s, 1)
                        if r == 0:
                            ds = DSK[pl.ds(_mult(J * CB + h * 32 + s * 8, 8), 8), :] * (1.0 / S)
                            t = t + jnp.where(lane == 0, ds, 0.0)
                        _Buf(KT[slot]).st(r * CB + h * 32 + s * 8, t)
                    yield

    def ld(b, k, h, n=8, stride=CB):
        return b.ld(2 * k * stride + h, n), b.ld((2 * k + 1) * stride + h, n)

    def st(b, k, h, v, stride=CB):
        b.st(2 * k * stride + h, v[0])
        b.st((2 * k + 1) * stride + h, v[1])

    def mat(r):
        return pltpu.bitcast(jnp.concatenate(ld(_Buf(mm), r, 0, 64, 64), axis=1), BF16)

    def kfwd(i, slot):
        g = _Buf(GK, i * 2 * R * CB, 2 * R * CB)
        for r in range(R):
            t = lax.dot_general(_Buf(KT[slot]).ld(r * CB, CB), mat(r), NN, preferred_element_type=F32)
            st(g, r, 0, (t[:, :LN], t[:, LN:]))
            yield

    def kfft(i):
        kf = _Buf(KF, i * CB, 2 * R * D - D + CB)
        for h in range(0, CB, 8):
            t = []
            for r0 in range(4):
                y = _radix4(*[ld(_Buf(GK, i * 2 * R * CB), r, h) for r in range(r0, R, 4)], -1)
                t.append([_twiddle(y[g0], r0 * g0, -1) for g0 in range(4)])
                yield
            for g0 in range(4):
                y = _radix4(t[0][g0], t[1][g0], t[2][g0], t[3][g0], -1)
                for g1 in range(4):
                    st(kf, 4 * g0 + g1, h, y[g1], D)
                yield

    iow = io.bitcast(U32)

    def xin(j):
        x = _Buf(X, j * LN)
        for rho in range(8):
            t = iow[j, pl.ds(rho, LN, stride=8), :].T
            x.st(2 * rho * D, pltpu.bitcast(t << 16, F32))
            x.st((2 * rho + 1) * D, pltpu.bitcast(t & np.uint32(0xFFFF0000), F32))
            yield

    def wprep(j):
        pr, pc = _iota((LN, LN), 0), _iota((LN, LN), 1)
        perm = jnp.where(pc == (pr & 7) * DH + (pr >> 3), 1.0, 0.0).astype(BF16)
        for c in range(3):
            t = lax.dot_general(perm, wraw[(c + 1) % 3 * 4 + j], NT, preferred_element_type=F32)
            if c == 2:
                t = t * (DH ** -0.5)
            for k in range(4):
                _Buf(W).st(k * WS + (3 * j + c) * LN // 2,
                           pltpu.bitcast(t[:, k * LN:(k + 1) * LN].astype(BF16), F32))
            yield
        t = jnp.dot(perm, woraw[j * LN:(j + 1) * LN, :], preferred_element_type=F32)
        _Buf(W).st(j * WS + 3 * D // 2, pltpu.bitcast(t.T.astype(BF16), F32))
        yield

    def kstep(J, ref):
        @block("kgen")
        def _():
            slot, m, v = ref % 2, [], []
            if 0 <= ref < NCB:
                m.append(ksum(J, slot))
            if 0 <= ref - 2:
                m.append(kfwd(J - 2, slot))
            if m:
                v.append((_chain(*m), 16 * len(m)))
            if 0 <= ref - 1 < NCB:
                v.append((_chain(*[kspread(J - 1, 1 - slot, h) for h in range(2)]), 32))
            if 0 <= ref + 1 < NCB:
                v.append((kpow(J + 1, 1 - slot), 8 * 59))
            if ref + 2 < NCB:
                v.append((kexp(J + 2, slot), 16))
            if ref >= NCB:
                js = (2 * (ref - NCB), 2 * (ref - NCB) + 1)
                v += [(_chain(*map(xin, js)), 16), (_chain(*map(wprep, js)), 8)]
            _weave(*v)

    lax.fori_loop(0, D // 64, kpar, 0)
    for J in range(-2, 2):
        kstep(J, J)
    with _scope("mwait"):
        mcp.wait()
    _loop(1, 3, lambda k: (kstep(2 * k, 2), kstep(2 * k + 1, 3)), 1)
    for J in range(6, 10):
        if J == NCB:
            with _scope("xwait"):
                for c in xcp + wcp + [wocp]:
                    c.wait()
        kstep(J, J)

    def colsum(f, step):
        acc = [f(c * 8) for c in range(4)]
        for i in range(4, D // 8):
            acc[i % 4] = acc[i % 4] + f(i * 8)
            if i % step == step - 1:
                yield
        s = jnp.sum((acc[0] + acc[1]) + (acc[2] + acc[3]), axis=0, keepdims=True)
        return jnp.broadcast_to(s * (1.0 / D), (8, LN))

    def ln_stats(ref, base):
        x = _Buf(ref, base + zero[0], D)
        m = yield from colsum(lambda c: x.ld(c, 8), 32)
        x = _Buf(ref, base + zero[1], D)
        v = yield from colsum(lambda c: jnp.square(x.ld(c, 8) - m), 8)
        return _Buf(ref, base + zero[2], D), m, lax.rsqrt(v + EPS)

    def ln(ref, base, out, r):
        x, m, rs = yield from ln_stats(ref, base)
        for c in range(0, D, 16):
            t = [(x.ld(c + k, 8) - m) * rs for k in (0, 8)]
            _Buf(out, r * D).st(c, jnp.concatenate(t, axis=0))
            if c % 64 == 48:
                yield

    def ln1(r):
        return ln(X, r * D, XN, r)

    def ln2(r):
        return ln(Z[r], 0, U, r)

    def wdot(c, n, rhs):
        lhs = jnp.concatenate(
            [pltpu.bitcast(W[t * WS + c // 2:t * WS + (c + n) // 2, :], BF16)
             for t in range(4)], axis=1)
        return jnp.dot(lhs, rhs.ld(0, D), preferred_element_type=F32)

    def qkvproj(j, r):
        b, i = _Buf(KVQ[j % 2][r % 2]), r // 2
        for c in range(3):
            t = wdot((3 * j + c) * LN, LN, _Buf(XN, r * D + zero[(r + c) % R], D))
            if c == 2:
                b.st((32 + i) * TS, t)
            else:
                b.st((16 * c + 8 + i) * TS, t)
                if i:
                    b.st((16 * c + i) * TS, pltpu.roll(t, 1, 1))
            yield

    def core(j, r):
        b, i = _Buf(KVQ[j % 2][r % 2], zero[r], 40 * TS), r // 2
        lg = [None] * WIN
        for dh in range(DH):
            q = b.ld((32 + i) * TS + dh * 8, 8)
            for w in range(WIN):
                t = q * b.ld((8 + i - w) * TS + dh * 8, 8)
                lg[w] = t if dh == 0 else lg[w] + t
            if dh % 2:
                yield
        for w in range(i + 1, WIN):
            lg[w] = jnp.where(lane > 0, lg[w], -1e9)
        mx = _tree(jnp.maximum, lg)
        e = [jnp.exp(v - mx) for v in lg]
        inv = 1.0 / _tree(jnp.add, e)
        e = [v * inv for v in e]
        yield
        yield
        for dh in range(0, DH, 2):
            oo = []
            for k in (dh, dh + 1):
                acc = None
                for w in range(WIN):
                    t = e[w] * b.ld((24 + i - w) * TS + k * 8, 8)
                    acc = t if acc is None else acc + t
                oo.append(acc)
            _Buf(O, r * D + j * LN).st(dh * 8, jnp.concatenate(oo, axis=0))
            yield

    def oproj(r):
        for c in range(0, D, DO):
            Z[r][c:c + DO, :] = X[r * D + c:r * D + c + DO, :] + wdot(
                3 * D + c, DO, _Buf(O, r * D + zero[(r + c // DO) % R], D))
            yield

    def cmxu(fi, ii, slot):
        if fi is not None:
            u_ = _Buf(U, fi * CB, R * D - D + CB)
        if ii is not None:
            x = _Buf(X, ii * CB, R * D - D + CB)
        for r in order:
            if fi is not None:
                t = lax.dot_general(u_.ld(r * D, CB), mat(r), NN, preferred_element_type=F32)
                st(_Buf(G[slot]), r, 0, (t[:, :LN], t[:, LN:]))
                yield
            if ii is not None:
                lhs = jnp.concatenate(ld(_Buf(HH[slot]), r, 0, CB), axis=1)
                t = lax.dot_general(lhs, mat(r), NT, preferred_element_type=F32)
                x.st(r * D, _Buf(Z[r], ii * CB, CB).ld(0, CB) + t)
                yield

    def cmid(i, slot):
        g, hh = _Buf(G[slot], zero[0], 2 * R * CB), _Buf(HH[slot])
        kf = _Buf(KF, i * CB, 2 * R * D - D + CB)

        for h in range(0, CB, 8):
            t, v = [], []
            for r0 in range(4):
                y = _radix4(*[ld(g, r, h) for r in range(r0, R, 4)], -1)
                t.append([_twiddle(y[g0], r0 * g0, -1) for g0 in range(4)])
                yield
            yield
            for g0 in range(4):
                y = _radix4(t[0][g0], t[1][g0], t[2][g0], t[3][g0], -1)
                yield
                y = [_cmul(y[g1], ld(kf, 4 * g0 + g1, h, 8, D)) for g1 in range(4)]
                yield
                y = _radix4(*y, 1)
                v.append([_twiddle(y[r0], r0 * g0, 1) for r0 in range(4)])
                yield
                if g0 != 1:
                    yield
            for r0 in range(4):
                y = _radix4(*[v[g0][r0] for g0 in range(4)], 1)
                for r1 in range(4):
                    st(hh, r0 + 4 * r1, h, y[r1])
                yield

    def ocopy(j):
        return pltpu.make_async_copy(
            io.at[j], out_hbm.at[:, pl.ds(_mult(j * LN, LN), LN)], sems.at[7 + j])

    def xout(j):
        x = _Buf(X, j * LN, R * D - D + LN)
        for rho in range(8):
            lo, hi = (pltpu.bitcast(x.ld(r * D, LN).astype(BF16).astype(F32), U32)
                      for r in (2 * rho, 2 * rho + 1))
            iow[j, pl.ds(rho, LN, stride=8), :] = ((lo >> 16) | hi).T
        ocopy(j).start()

    order = list(range(0, R, 2)) + list(range(1, R, 2))
    NCORE, NLN1, NLN2 = 18, 18, 18

    def layer(l, carry):
        @block("ph1")
        def _():
            for n, r in enumerate(order):
                _weave((qkvproj(0, r), 3), *([(ln1(order[n + 1]), NLN1 * 1.5)] if n + 1 < R else []))

        for j, lo, hi in ((1, 0, R), (2, 0, R), (3, 0, R // 2), (3, R // 2, R)):
            @block("ph2")
            def _():
                early = _chain(*[core(3, r) for r in order[:LO if lo else 0]])
                kf = _chain(*map(kfft, KB[j] if not lo else ()))
                for r in order[lo:hi]:
                    _weave((qkvproj(j, r), 3), (core(j - 1, r), NCORE),
                           (_take(early, -(-LO * NCORE // 8)), LO * NCORE / 8 + 0.01),
                           (_take(kf, len(KB[j]) * 64 // (hi - lo)), len(KB[j]) * 64 / (hi - lo)))
                _weave((early, 1))

        for prev, cur in zip(B3, B3[1:]):
            @block("ph3")
            def _():
                w, c, n = (order[u:v] for u, v in zip(prev, cur))
                _weave((_chain(*map(oproj, w)), len(w) * D // DO),
                       (_chain(*[core(3, r) for r in c]), len(c) * NCORE + 0.01),
                       (_chain(*map(ln2, n)), len(n) * NLN2 + 0.01))

        def cstep(i, slot, f=True, m=True, v=True):
            @block("conv")
            def _():
                _weave((cmxu(i + 1 if f else None, i - 1 if v else None, 1 - slot), R * (f + v)),
                       *([(cmid(i, slot), 3 * CB)] if m else []),
                       *[(ln2(r), 2 * NLN2) for r in order[B3[-1][2]:] if f and not m])
                if v and not m:
                    _weave((ln1(0), 1))

        cstep(-1, 1, m=False, v=False)
        cstep(0, 0, v=False)

        def cpair(k):
            cstep(2 * k + 1, 1)
            cstep(2 * k + 2, 0)
            pl.when(l == 1)(lambda: xout(k))

        _loop(0, NCB // 2 - 1, cpair, 1)
        cstep(NCB - 1, 1, f=False)
        cstep(NCB, 0, f=False, m=False)
        return carry

    _weave((ln1(0), 1))
    with _scope("layers"):
        lax.fori_loop(0, 2, layer, 0)
    xout(3)

    with _scope("owait"):
        for j in range(4):
            ocopy(j).wait()


@jax.jit
def pallas_interleave_layers__sliding_local_dilated__ssm_conv_s4__prompt_kernel(
    A_x: jax.Array,
    A_wqkv: jax.Array,
    A_wo: jax.Array,
    B_u: jax.Array,
    B_A_re: jax.Array,
    B_A_im: jax.Array,
    B_B_re: jax.Array,
    B_B_im: jax.Array,
    B_C_re: jax.Array,
    B_C_im: jax.Array,
    B_log_dt: jax.Array,
    B_Dskip: jax.Array,
):
    del B_u
    hbm = pl.BlockSpec(memory_space=pl.ANY)
    V = pltpu.VMEM
    out = pl.pallas_call(
        _kernel,
        out_shape=jax.ShapeDtypeStruct((S, D), BF16),
        in_specs=[hbm] * 12,
        out_specs=hbm,
        scratch_shapes=[
            V((D,), BF16), V((D,), BF16),
            V((4, S, LN), BF16),
            V((12, D, LN), BF16),
            V((D, D), BF16),
            V((6, D, LN), BF16),
            V((R * LN, LN), U32),
            V((R * D, LN), F32),
            V((2 * R * D, LN), F32),
            V((D, LN), F32),
            V((R * D, LN), BF16),
            V((R * D, LN), F32),
            V((4 * WS, LN), F32),
            [V((D, LN), F32)] * R,
            [[V((40 * TS, LN), F32)] * 2] * 2,
            V((R * D, LN), BF16),
            [V((2 * R * CB, LN), F32)] * 2,
            [V((2 * R * CB, LN), F32)] * 2,
            [V((R * CB, LN), F32)] * 2,
            V((2 * R * D, LN), F32),
            V((6, D, LN), F32),
            [V((4, 8, 8, LN), F32)] * 2,
            V((D, LN), F32),
            [V((4, 8 * SS, LN), F32)] * 2,
            [V((4, 8 * SS, LN), F32)] * 2,
            [V((2, 8 * 33, LN), F32)] * 2,
            pltpu.SMEM((R,), jnp.int32),
            pltpu.SemaphoreType.DMA((26,)),
        ],
        compiler_params=pltpu.CompilerParams(vmem_limit_bytes=100 * 1024 * 1024, flags=FLAGS),
    )(A_x.reshape(S, D), A_wqkv, A_wo, B_A_re, B_A_im, B_B_re, B_B_im, B_C_re, B_C_im,
      B_log_dt, B_Dskip, _M)
    return out.reshape(1, S, D)
```

```python
import contextlib
import numpy as np
import jax
import jax.numpy as jnp
from jax import lax
import jax.experimental.pallas as pl
import jax.experimental.pallas.tpu as pltpu

S, D, DH, WIN = 2048, 512, 16, 8
R = 16
LN = 128
CB = 64
NCB = D // CB
EPS = 1e-5
F32, BF16, U32 = jnp.float32, jnp.bfloat16, jnp.uint32
NN, NT = (((1,), (0,)), ((), ())), (((1,), (1,)), ((), ()))


def _dft_matrices():
    lam = np.arange(LN, dtype=np.float64)[None, :, None]
    r = np.arange(R, dtype=np.float64)[:, None, None]
    f = np.arange(LN, dtype=np.float64)[None, None, :]
    th = 2.0 * np.pi * (f + 0.5) * (R * lam + r) / (2 * S)
    m = np.stack([np.cos(th), -np.sin(th)], axis=1).astype(BF16).view(np.uint16).astype(np.uint32)
    return (m[:, :, 0::2] | (m[:, :, 1::2] << 16)).reshape(R * LN, LN)


_M = _dft_matrices()


SCOPES = False


def _scope(name):
    return jax.named_scope(name) if SCOPES else contextlib.nullcontext()


FLAGS = None
SKIP = NOB = ''
LO = 6
KW = 0.9
KB = {1: (0, 1, 2), 2: (3, 4, 5), 3: (6, 7)}
B3 = ((0, 6, 0), (5, 11, 0), (10, 16, 5), (14, 16, 10), (16, 16, 14))
DO = 256
TS, WS, SS = LN, 2 * D, LN + 1


class _Buf:
    def __init__(self, ref, base=0, size=None):
        if isinstance(base, int):
            self.ref, self.base = ref, base
        else:
            self.ref, self.base = ref.at[pl.ds(pl.multiple_of(base, 16), size), :], 0

    def ld(self, row, n):
        return self.ref[self.base + row:self.base + row + n, :]

    def st(self, row, v):
        self.ref[self.base + row:self.base + row + v.shape[0], :] = v.astype(self.ref.dtype)


def _weave(*stages):
    live = [[g, n, 0] for g, n in stages]
    while live:
        st = min(live, key=lambda t: t[2] / t[1])
        try:
            next(st[0])
            st[2] += 1
        except StopIteration:
            live.remove(st)


def _chain(*gens):
    for g in gens:
        yield from g


def _take(g, n):
    for _, _ in zip(range(n), g):
        yield


def _tree(op, v):
    while len(v) > 1:
        v = [op(v[i], v[i + 1]) for i in range(0, len(v), 2)]
    return v[0]


def _mult(i, n):
    return i if isinstance(i, int) else pl.multiple_of(i, n)


def _loop(lo, hi, body, unroll, force=False):
    n = hi - lo
    assert n % unroll == 0
    if n == unroll and not force:
        for i in range(lo, hi):
            body(i)
        return

    def outer(k, carry):
        for u in range(unroll):
            body(lo + k * unroll + u)
        return carry

    lax.fori_loop(0, n // unroll, outer, 0)


def _iota(shape, dim):
    return lax.broadcasted_iota(jnp.int32, shape, dim)


def _cmul(a, b):
    return (a[0] * b[0] - a[1] * b[1], a[0] * b[1] + a[1] * b[0])


def _csq(a):
    t = a[0] * a[1]
    return (a[0] * a[0] - a[1] * a[1], t + t)


def _radix4(a, b, c, d, sign):
    s0 = (a[0] + c[0], a[1] + c[1])
    d0 = (a[0] - c[0], a[1] - c[1])
    s1 = (b[0] + d[0], b[1] + d[1])
    d1 = (b[0] - d[0], b[1] - d[1])
    y0 = (s0[0] + s1[0], s0[1] + s1[1])
    y2 = (s0[0] - s1[0], s0[1] - s1[1])
    p = (d0[0] - d1[1], d0[1] + d1[0])
    m = (d0[0] + d1[1], d0[1] - d1[0])
    return (y0, p, y2, m) if sign > 0 else (y0, m, y2, p)


def _twiddle(a, k, sign):
    if k == 0:
        return a
    c = float(np.cos(2 * np.pi * k / 16))
    s = float(sign * np.sin(2 * np.pi * k / 16))
    if k == 4:
        return (-a[1], a[0]) if sign > 0 else (a[1], -a[0])
    if k == 2:
        if sign > 0:
            return ((a[0] - a[1]) * c, (a[0] + a[1]) * c)
        return ((a[0] + a[1]) * c, (a[1] - a[0]) * c)
    if k == 6:
        if sign > 0:
            return ((a[0] + a[1]) * c, (a[1] - a[0]) * c)
        return ((a[0] - a[1]) * c, (a[0] + a[1]) * c)
    return (a[0] * c - a[1] * s, a[0] * s + a[1] * c)


def _kernel(x_hbm, wqkv_hbm, wo_hbm, are_hbm, aim_hbm, bre_hbm, bim_hbm, cre_hbm, cim_hbm,
            ldt_hbm, dsk_hbm, m_hbm, out_hbm, ldt_ref, dsk_ref,
            io, wraw, woraw, par, mm, X, KF, DSK, XN, U, W, Z, KVQ, O, G, HH,
            KT, GK, PF, E, DT, SA, SB, KO, zero, sems):
    for k in range(R):
        zero[k] = 0

    def block(name):
        def deco(f):
            if SKIP and name in SKIP:
                return
            with _scope(name):
                f() if name in NOB else pl.when(zero[0] == 0)(f)
        return deco

    def opaque(r):
        return zero[r] if isinstance(r, int) else 0

    pcp = [pltpu.make_async_copy(h, par.at[i], sems.at[i])
           for i, h in enumerate((are_hbm, aim_hbm, bre_hbm, bim_hbm, cre_hbm, cim_hbm))]
    mcp = pltpu.make_async_copy(m_hbm, mm, sems.at[6])
    xcp = [pltpu.make_async_copy(x_hbm.at[:, pl.ds(j * LN, LN)], io.at[j], sems.at[7 + j])
           for j in range(4)]
    wocp = pltpu.make_async_copy(wo_hbm, woraw, sems.at[11])
    wcp = [pltpu.make_async_copy(wqkv_hbm.at[:, pl.ds(j * LN, LN)], wraw.at[j], sems.at[12 + j])
           for j in range(12)]
    scp = [pltpu.make_async_copy(ldt_hbm, ldt_ref, sems.at[24]),
           pltpu.make_async_copy(dsk_hbm, dsk_ref, sems.at[25])]
    for c in scp + pcp:
        c.start()

    for sb in SB:
        for c in range(4):
            head = jnp.where(_iota((8, LN), 0) == 0, 1.0 - c % 2, 0.0)
            for row in range(32):
                o = row // 4 * SS + row % 4 * 32
                sb[c, o:o + 8, :] = head
                sb[c, o + 24:o + 32, :] = jnp.zeros((8, LN), F32)

    for c in scp:
        c.wait()
    dt_row = jnp.exp(ldt_ref[...].astype(F32).reshape(1, D)).astype(BF16).astype(F32)
    ds_row = dsk_ref[...].astype(F32).reshape(1, D)
    for j in range(4):
        sl = slice(j * LN, (j + 1) * LN)
        DT[sl, :] = jnp.broadcast_to(dt_row[:, sl], (LN, LN)).T
        DSK[sl, :] = jnp.broadcast_to(ds_row[:, sl], (LN, LN)).T
    with _scope('pwait'):
        for c in pcp:
            c.wait()
    for c in [mcp] + xcp + wcp + [wocp]:
        c.start()

    lane = _iota((8, LN), 1)

    def kpar(J, carry):
        rows = pl.ds(pl.multiple_of(J * 64, 64), 64)
        for i in range(6):
            PF[i, rows, :] = par[i, rows, :].astype(F32)
        return carry

    def kexp(J, slot):
        for s in range(8):
            rows = pl.ds(_mult(J * CB + s * 8, 8), 8)
            dt = DT[rows, :]
            zr, zi = dt * PF[0, rows, :], dt * PF[1, rows, :]
            mag = jnp.exp(zr)
            E[slot][0, s] = mag * jnp.cos(zi)
            yield
            E[slot][1, s] = mag * jnp.sin(zi)
            w = _cmul((PF[4, rows, :], PF[5, rows, :]), (dt * PF[2, rows, :], dt * PF[3, rows, :]))
            E[slot][2, s] = w[0] * (1.0 / S)
            E[slot][3, s] = w[1] * (1.0 / S)
            yield

    def kpow(J, slot):
        sa, sb = SA[slot], SB[slot]
        for s in range(8):
            def put(ref, i, v):
                for c in range(2):
                    ref[s // 4 * 2 + c, pl.ds(s % 4 * 32 + i, 8, stride=SS), :] = v[c]

            p = (E[slot][0, s], E[slot][1, s])
            b = [None]
            for k in range(4):
                for i in range(2 ** k):
                    b.append(_cmul(b[i], p) if i else p)
                    put(sb, len(b) - 1, b[-1])
                    yield
                p = _csq(p)
            put(sb, 16, p)
            b = {4: b[4], 8: b[8], 12: b[12], 16: p}
            w = (E[slot][2, s], E[slot][3, s])
            pw = []
            for k in range(5):
                pw.append(p)
                p = _csq(p)
                yield
            e512, e1024 = p, _csq(p)
            for o, st, e in ((17, 4, e512), (22, 8, e1024), (25, 8, _cmul(e512, e1024))):
                put(sb, o, e)
                for i in range(1, 16 // st + 1):
                    put(sb, o + i, _cmul(e, b[i * st]))
                    yield

            def tree(i, v, k):
                put(sa, i, v)
                yield
                for k2 in range(k):
                    yield from tree(i + 2 ** k2, _cmul(v, pw[k2]), k2)

            yield from tree(0, w, 5)

    def ksum(J, slot):
        sa, sb = SA[slot], SB[slot]
        q32 = _iota((32, LN), 1) >> 5
        for hm in range(16):
            h, m = divmod(hm, 8)
            o = [lax.dot_general(sb[2 * h + c, m * SS:m * SS + LN, :],
                                 sa[2 * h + c, m * SS:m * SS + LN, :],
                                 NT, preferred_element_type=F32) for c in range(2)]
            o = o[0] - o[1]
            KO[slot][h, m * 33:m * 33 + 32, :] = jnp.where(
                q32 < 2, jnp.where(q32 == 0, o[0:32], o[32:64]),
                jnp.where(q32 == 2, o[64:96], o[96:128]))
            yield

    def kspread(J, slot, h):
        kb = lambda i: KO[slot][h, pl.ds(i, 8, stride=33), :]
        rnd = lambda r, st: int(np.round(r / st))
        quarter, low = lane >> 5, (lane & 31) < 16
        q1 = [pltpu.roll(kb(i), 32, 1) for i in range(17, 22)]
        q2 = [pltpu.roll(kb(i), 64, 1) for i in range(22, 25)]
        q3 = [pltpu.roll(kb(i), 96, 1) for i in range(25, 28)]
        for k8 in range(3):
            q23 = [jnp.where(quarter == (s + 2) % 4, q2[k8], q3[k8]) for s in range(4)]
            for k4 in range(5):
                rs = [r for r in range(R) if (rnd(r, 4), rnd(r, 8)) == (k4, k8)]
                rest = [jnp.where(quarter == (s + 1) % 4, q1[k4], q23[s]) for s in range(4) if rs]
                for r in rs:
                    q0 = kb(r) if r % 2 == 0 else jnp.where(low, kb(r), kb(2 * rnd(r, 2)))
                    for s in range(4):
                        t = jnp.where(quarter == s, q0, rest[s])
                        if s:
                            t = pltpu.roll(t, LN - 32 * s, 1)
                        if r == 0:
                            ds = DSK[pl.ds(_mult(J * CB + h * 32 + s * 8, 8), 8), :] * (1.0 / S)
                            t = t + jnp.where(lane == 0, ds, 0.0)
                        _Buf(KT[slot]).st(r * CB + h * 32 + s * 8, t)
                    yield

    def ld(b, k, h, n=8, stride=CB):
        return b.ld(2 * k * stride + h, n), b.ld((2 * k + 1) * stride + h, n)

    def st(b, k, h, v, stride=CB):
        b.st(2 * k * stride + h, v[0])
        b.st((2 * k + 1) * stride + h, v[1])

    def mat(r):
        return pltpu.bitcast(jnp.concatenate(ld(_Buf(mm), r, 0, 64, 64), axis=1), BF16)

    def kfwd(i, slot):
        g = _Buf(GK, i * 2 * R * CB, 2 * R * CB)
        for r in range(R):
            t = lax.dot_general(_Buf(KT[slot]).ld(r * CB, CB), mat(r), NN, preferred_element_type=F32)
            st(g, r, 0, (t[:, :LN], t[:, LN:]))
            yield

    def kfft(i):
        kf = _Buf(KF, i * CB, 2 * R * D - D + CB)
        for h in range(0, CB, 8):
            t = []
            for r0 in range(4):
                y = _radix4(*[ld(_Buf(GK, i * 2 * R * CB), r, h) for r in range(r0, R, 4)], -1)
                t.append([_twiddle(y[g0], r0 * g0, -1) for g0 in range(4)])
                yield
            for g0 in range(4):
                y = _radix4(t[0][g0], t[1][g0], t[2][g0], t[3][g0], -1)
                for g1 in range(4):
                    st(kf, 4 * g0 + g1, h, y[g1], D)
                yield

    iow = io.bitcast(U32)

    def xin(j):
        x = _Buf(X, j * LN)
        for rho in range(8):
            t = iow[j, pl.ds(rho, LN, stride=8), :].T
            x.st(2 * rho * D, pltpu.bitcast(t << 16, F32))
            x.st((2 * rho + 1) * D, pltpu.bitcast(t & np.uint32(0xFFFF0000), F32))
            yield

    def wprep(j):
        pr, pc = _iota((LN, LN), 0), _iota((LN, LN), 1)
        perm = jnp.where(pc == (pr & 7) * DH + (pr >> 3), 1.0, 0.0).astype(BF16)
        for c in range(3):
            t = lax.dot_general(perm, wraw[(c + 1) % 3 * 4 + j], NT, preferred_element_type=F32)
            if c == 2:
                t = t * (DH ** -0.5)
            for k in range(4):
                _Buf(W).st(k * WS + (3 * j + c) * LN // 2,
                           pltpu.bitcast(t[:, k * LN:(k + 1) * LN].astype(BF16), F32))
            yield
        t = jnp.dot(perm, woraw[j * LN:(j + 1) * LN, :], preferred_element_type=F32)
        _Buf(W).st(j * WS + 3 * D // 2, pltpu.bitcast(t.T.astype(BF16), F32))
        yield

    def kstep(J, ref):
        @block("kgen")
        def _():
            slot, m, v = ref % 2, [], []
            if 0 <= ref < NCB:
                m.append(ksum(J, slot))
            if 0 <= ref - 2:
                m.append(kfwd(J - 2, slot))
            v = [(g, 16 * KW) for g in m]
            if 0 <= ref - 1 < NCB:
                v.append((_chain(*[kspread(J - 1, 1 - slot, h) for h in range(2)]), 32))
            if 0 <= ref + 1 < NCB:
                v.append((kpow(J + 1, 1 - slot), 8 * 59))
            if ref + 2 < NCB:
                v.append((kexp(J + 2, slot), 16))
            if ref >= NCB:
                js = (2 * (ref - NCB), 2 * (ref - NCB) + 1)
                v += [(_chain(*map(xin, js)), 16), (_chain(*map(wprep, js)), 8)]
            _weave(*v)

    lax.fori_loop(0, D // 64, kpar, 0)
    for J in range(-2, 2):
        kstep(J, J)
    with _scope("mwait"):
        mcp.wait()
    _loop(1, 3, lambda k: (kstep(2 * k, 2), kstep(2 * k + 1, 3)), 1)
    for J in range(6, 10):
        if J == NCB:
            with _scope("xwait"):
                for c in xcp + wcp + [wocp]:
                    c.wait()
        kstep(J, J)

    def colsum(f, step):
        acc = [f(c * 8) for c in range(4)]
        for i in range(4, D // 8):
            acc[i % 4] = acc[i % 4] + f(i * 8)
            if i % step == step - 1:
                yield
        s = jnp.sum((acc[0] + acc[1]) + (acc[2] + acc[3]), axis=0, keepdims=True)
        return jnp.broadcast_to(s * (1.0 / D), (8, LN))

    def ln_stats(ref, base):
        x = _Buf(ref, base + zero[0], D)
        m = yield from colsum(lambda c: x.ld(c, 8), 32)
        x = _Buf(ref, base + zero[1], D)
        v = yield from colsum(lambda c: jnp.square(x.ld(c, 8) - m), 8)
        return _Buf(ref, base + zero[2], D), m, lax.rsqrt(v + EPS)

    def ln(ref, base, out, r):
        x, m, rs = yield from ln_stats(ref, base)
        for c in range(0, D, 16):
            t = [(x.ld(c + k, 8) - m) * rs for k in (0, 8)]
            _Buf(out, r * D).st(c, jnp.concatenate(t, axis=0))
            if c % 64 == 48:
                yield

    def ln1(r):
        return ln(X, r * D, XN, r)

    def ln2(r):
        return ln(Z[r], 0, U, r)

    def wdot(c, n, rhs):
        lhs = jnp.concatenate(
            [pltpu.bitcast(W[t * WS + c // 2:t * WS + (c + n) // 2, :], BF16)
             for t in range(4)], axis=1)
        return jnp.dot(lhs, rhs.ld(0, D), preferred_element_type=F32)

    def qkvproj(j, r):
        b, i = _Buf(KVQ[j % 2][r % 2]), r // 2
        for c in range(3):
            t = wdot((3 * j + c) * LN, LN, _Buf(XN, r * D + zero[(r + c) % R], D))
            if c == 2:
                b.st((32 + i) * TS, t)
            else:
                b.st((16 * c + 8 + i) * TS, t)
                if i:
                    b.st((16 * c + i) * TS, pltpu.roll(t, 1, 1))
            yield

    def core(j, r):
        b, i = _Buf(KVQ[j % 2][r % 2], zero[r], 40 * TS), r // 2
        lg = [None] * WIN
        for dh in range(DH):
            q = b.ld((32 + i) * TS + dh * 8, 8)
            for w in range(WIN):
                t = q * b.ld((8 + i - w) * TS + dh * 8, 8)
                lg[w] = t if dh == 0 else lg[w] + t
            if dh % 2:
                yield
        for w in range(i + 1, WIN):
            lg[w] = jnp.where(lane > 0, lg[w], -1e9)
        mx = _tree(jnp.maximum, lg)
        e = [jnp.exp(v - mx) for v in lg]
        inv = 1.0 / _tree(jnp.add, e)
        e = [v * inv for v in e]
        yield
        yield
        for dh in range(0, DH, 2):
            oo = []
            for k in (dh, dh + 1):
                acc = None
                for w in range(WIN):
                    t = e[w] * b.ld((24 + i - w) * TS + k * 8, 8)
                    acc = t if acc is None else acc + t
                oo.append(acc)
            _Buf(O, r * D + j * LN).st(dh * 8, jnp.concatenate(oo, axis=0))
            yield

    def oproj(r):
        for c in range(0, D, DO):
            Z[r][c:c + DO, :] = X[r * D + c:r * D + c + DO, :] + wdot(
                3 * D + c, DO, _Buf(O, r * D + zero[(r + c // DO) % R], D))
            yield

    def cmxu(fi, ii, slot):
        if fi is not None:
            u_ = _Buf(U, fi * CB, R * D - D + CB)
        if ii is not None:
            x = _Buf(X, ii * CB, R * D - D + CB)
        for r in order:
            if fi is not None:
                t = lax.dot_general(u_.ld(r * D, CB), mat(r), NN, preferred_element_type=F32)
                st(_Buf(G[slot]), r, 0, (t[:, :LN], t[:, LN:]))
                yield
            if ii is not None:
                lhs = jnp.concatenate(ld(_Buf(HH[slot]), r, 0, CB), axis=1)
                t = lax.dot_general(lhs, mat(r), NT, preferred_element_type=F32)
                x.st(r * D, _Buf(Z[r], ii * CB, CB).ld(0, CB) + t)
                yield

    def cmid(i, slot):
        g, hh = _Buf(G[slot], zero[0], 2 * R * CB), _Buf(HH[slot])
        kf = _Buf(KF, i * CB, 2 * R * D - D + CB)

        for h in range(0, CB, 8):
            t, v = [], []
            for r0 in range(4):
                y = _radix4(*[ld(g, r, h) for r in range(r0, R, 4)], -1)
                t.append([_twiddle(y[g0], r0 * g0, -1) for g0 in range(4)])
                yield
            yield
            for g0 in range(4):
                y = _radix4(t[0][g0], t[1][g0], t[2][g0], t[3][g0], -1)
                yield
                y = [_cmul(y[g1], ld(kf, 4 * g0 + g1, h, 8, D)) for g1 in range(4)]
                yield
                y = _radix4(*y, 1)
                v.append([_twiddle(y[r0], r0 * g0, 1) for r0 in range(4)])
                yield
                if g0 != 1:
                    yield
            for r0 in range(4):
                y = _radix4(*[v[g0][r0] for g0 in range(4)], 1)
                for r1 in range(4):
                    st(hh, r0 + 4 * r1, h, y[r1])
                yield

    def ocopy(j):
        return pltpu.make_async_copy(
            io.at[j], out_hbm.at[:, pl.ds(_mult(j * LN, LN), LN)], sems.at[7 + j])

    def xout(j):
        x = _Buf(X, j * LN, R * D - D + LN)
        for rho in range(8):
            lo, hi = (pltpu.bitcast(x.ld(r * D, LN).astype(BF16).astype(F32), U32)
                      for r in (2 * rho, 2 * rho + 1))
            iow[j, pl.ds(rho, LN, stride=8), :] = ((lo >> 16) | hi).T
        ocopy(j).start()

    order = list(range(0, R, 2)) + list(range(1, R, 2))
    NCORE, NLN1, NLN2 = 18, 18, 18

    def layer(l, carry):
        @block("ph1")
        def _():
            for n, r in enumerate(order):
                _weave((qkvproj(0, r), 3), *([(ln1(order[n + 1]), NLN1 * 1.5)] if n + 1 < R else []))

        for j, lo, hi in ((1, 0, R), (2, 0, R), (3, 0, R // 2), (3, R // 2, R)):
            @block("ph2")
            def _():
                early = _chain(*[core(3, r) for r in order[:LO if lo else 0]])
                kf = _chain(*map(kfft, KB[j] if not lo else ()))
                for r in order[lo:hi]:
                    _weave((qkvproj(j, r), 3), (core(j - 1, r), NCORE),
                           (_take(early, -(-LO * NCORE // 8)), LO * NCORE / 8 + 0.01),
                           (_take(kf, len(KB[j]) * 64 // (hi - lo)), len(KB[j]) * 64 / (hi - lo)))
                _weave((early, 1))

        for prev, cur in zip(B3, B3[1:]):
            @block("ph3")
            def _():
                w, c, n = (order[u:v] for u, v in zip(prev, cur))
                _weave((_chain(*map(oproj, w)), len(w) * D // DO),
                       (_chain(*[core(3, r) for r in c]), len(c) * NCORE + 0.01),
                       (_chain(*map(ln2, n)), len(n) * NLN2 + 0.01))

        def cstep(i, slot, f=True, m=True, v=True):
            @block("conv")
            def _():
                _weave((cmxu(i + 1 if f else None, i - 1 if v else None, 1 - slot), R * (f + v)),
                       *([(cmid(i, slot), 3 * CB)] if m else []),
                       *[(ln2(r), 2 * NLN2) for r in order[B3[-1][2]:] if f and not m])
                if v and not m:
                    _weave((ln1(0), 1))

        cstep(-1, 1, m=False, v=False)
        cstep(0, 0, v=False)

        def cpair(k):
            cstep(2 * k + 1, 1)
            cstep(2 * k + 2, 0)
            pl.when(l == 1)(lambda: xout(k))

        _loop(0, NCB // 2 - 1, cpair, 1)
        cstep(NCB - 1, 1, f=False)
        cstep(NCB, 0, f=False, m=False)
        return carry

    _weave((ln1(0), 1))
    with _scope("layers"):
        lax.fori_loop(0, 2, layer, 0)
    xout(3)

    with _scope("owait"):
        for j in range(4):
            ocopy(j).wait()


@jax.jit
def pallas_interleave_layers__sliding_local_dilated__ssm_conv_s4__prompt_kernel(
    A_x: jax.Array,
    A_wqkv: jax.Array,
    A_wo: jax.Array,
    B_u: jax.Array,
    B_A_re: jax.Array,
    B_A_im: jax.Array,
    B_B_re: jax.Array,
    B_B_im: jax.Array,
    B_C_re: jax.Array,
    B_C_im: jax.Array,
    B_log_dt: jax.Array,
    B_Dskip: jax.Array,
):
    del B_u
    hbm = pl.BlockSpec(memory_space=pl.ANY)
    V = pltpu.VMEM
    out = pl.pallas_call(
        _kernel,
        out_shape=jax.ShapeDtypeStruct((S, D), BF16),
        in_specs=[hbm] * 12,
        out_specs=hbm,
        scratch_shapes=[
            V((D,), BF16), V((D,), BF16),
            V((4, S, LN), BF16),
            V((12, D, LN), BF16),
            V((D, D), BF16),
            V((6, D, LN), BF16),
            V((R * LN, LN), U32),
            V((R * D, LN), F32),
            V((2 * R * D, LN), F32),
            V((D, LN), F32),
            V((R * D, LN), BF16),
            V((R * D, LN), F32),
            V((4 * WS, LN), F32),
            [V((D, LN), F32)] * R,
            [[V((40 * TS, LN), F32)] * 2] * 2,
            V((R * D, LN), BF16),
            [V((2 * R * CB, LN), F32)] * 2,
            [V((2 * R * CB, LN), F32)] * 2,
            [V((R * CB, LN), F32)] * 2,
            V((2 * R * D, LN), F32),
            V((6, D, LN), F32),
            [V((4, 8, 8, LN), F32)] * 2,
            V((D, LN), F32),
            [V((4, 8 * SS, LN), F32)] * 2,
            [V((4, 8 * SS, LN), F32)] * 2,
            [V((2, 8 * 33, LN), F32)] * 2,
            pltpu.SMEM((R,), jnp.int32),
            pltpu.SemaphoreType.DMA((26,)),
        ],
        compiler_params=pltpu.CompilerParams(vmem_limit_bytes=100 * 1024 * 1024, flags=FLAGS),
    )(A_x.reshape(S, D), A_wqkv, A_wo, B_A_re, B_A_im, B_B_re, B_B_im, B_C_re, B_C_im,
      B_log_dt, B_Dskip, _M)
    return out.reshape(1, S, D)
```

```python
import contextlib
import numpy as np
import jax
import jax.numpy as jnp
from jax import lax
import jax.experimental.pallas as pl
import jax.experimental.pallas.tpu as pltpu

S, D, DH, WIN = 2048, 512, 16, 8
R = 16
LN = 128
CB = 64
NCB = D // CB
EPS = 1e-5
F32, BF16, U32 = jnp.float32, jnp.bfloat16, jnp.uint32
NN, NT = (((1,), (0,)), ((), ())), (((1,), (1,)), ((), ()))


def _dft_matrices():
    lam = np.arange(LN, dtype=np.float64)[None, :, None]
    r = np.arange(R, dtype=np.float64)[:, None, None]
    f = np.arange(LN, dtype=np.float64)[None, None, :]
    th = 2.0 * np.pi * (f + 0.5) * (R * lam + r) / (2 * S)
    m = np.stack([np.cos(th), -np.sin(th)], axis=1).astype(BF16).view(np.uint16).astype(np.uint32)
    return (m[:, :, 0::2] | (m[:, :, 1::2] << 16)).reshape(R * LN, LN)


_M = _dft_matrices()


SCOPES = False


def _scope(name):
    return jax.named_scope(name) if SCOPES else contextlib.nullcontext()


FLAGS = None
SKIP = NOB = ''
LO = 6
KW = 0.9
KB = {1: (0, 1, 2), 2: (3, 4, 5), 3: (6, 7)}
B3 = ((0, 6, 0), (5, 11, 0), (10, 16, 5), (14, 16, 10), (16, 16, 14))
DO = 256
TS, WS = LN, 2 * D


class _Buf:
    def __init__(self, ref, base=0, size=None):
        if isinstance(base, int):
            self.ref, self.base = ref, base
        else:
            self.ref, self.base = ref.at[pl.ds(pl.multiple_of(base, 16), size), :], 0

    def ld(self, row, n):
        return self.ref[self.base + row:self.base + row + n, :]

    def st(self, row, v):
        self.ref[self.base + row:self.base + row + v.shape[0], :] = v.astype(self.ref.dtype)


def _weave(*stages):
    live = [[g, n, 0] for g, n in stages]
    while live:
        st = min(live, key=lambda t: t[2] / t[1])
        try:
            next(st[0])
            st[2] += 1
        except StopIteration:
            live.remove(st)


def _chain(*gens):
    for g in gens:
        yield from g


def _take(g, n):
    for _, _ in zip(range(n), g):
        yield


def _tree(op, v):
    while len(v) > 1:
        v = [op(v[i], v[i + 1]) for i in range(0, len(v), 2)]
    return v[0]


def _mult(i, n):
    return i if isinstance(i, int) else pl.multiple_of(i, n)


def _loop(lo, hi, body, unroll, force=False):
    n = hi - lo
    assert n % unroll == 0
    if n == unroll and not force:
        for i in range(lo, hi):
            body(i)
        return

    def outer(k, carry):
        for u in range(unroll):
            body(lo + k * unroll + u)
        return carry

    lax.fori_loop(0, n // unroll, outer, 0)


def _iota(shape, dim):
    return lax.broadcasted_iota(jnp.int32, shape, dim)


def _cmul(a, b):
    return (a[0] * b[0] - a[1] * b[1], a[0] * b[1] + a[1] * b[0])


def _csq(a):
    t = a[0] * a[1]
    return (a[0] * a[0] - a[1] * a[1], t + t)


def _radix4(a, b, c, d, sign):
    s0 = (a[0] + c[0], a[1] + c[1])
    d0 = (a[0] - c[0], a[1] - c[1])
    s1 = (b[0] + d[0], b[1] + d[1])
    d1 = (b[0] - d[0], b[1] - d[1])
    y0 = (s0[0] + s1[0], s0[1] + s1[1])
    y2 = (s0[0] - s1[0], s0[1] - s1[1])
    p = (d0[0] - d1[1], d0[1] + d1[0])
    m = (d0[0] + d1[1], d0[1] - d1[0])
    return (y0, p, y2, m) if sign > 0 else (y0, m, y2, p)


def _twiddle(a, k, sign):
    if k == 0:
        return a
    c = float(np.cos(2 * np.pi * k / 16))
    s = float(sign * np.sin(2 * np.pi * k / 16))
    if k == 4:
        return (-a[1], a[0]) if sign > 0 else (a[1], -a[0])
    if k == 2:
        if sign > 0:
            return ((a[0] - a[1]) * c, (a[0] + a[1]) * c)
        return ((a[0] + a[1]) * c, (a[1] - a[0]) * c)
    if k == 6:
        if sign > 0:
            return ((a[0] + a[1]) * c, (a[1] - a[0]) * c)
        return ((a[0] - a[1]) * c, (a[0] + a[1]) * c)
    return (a[0] * c - a[1] * s, a[0] * s + a[1] * c)


def _kernel(x_hbm, wqkv_hbm, wo_hbm, are_hbm, aim_hbm, bre_hbm, bim_hbm, cre_hbm, cim_hbm,
            ldt_hbm, dsk_hbm, m_hbm, out_hbm, ldt_ref, dsk_ref,
            io, wraw, woraw, par, mm, X, KF, DSK, XN, U, W, Z, KVQ, O, G, HH,
            KT, GK, PF, E, DT, ZK, SA, SB, KO, zero, sems):
    for k in range(R):
        zero[k] = 0

    def block(name):
        def deco(f):
            if SKIP and name in SKIP:
                return
            with _scope(name):
                f() if name in NOB else pl.when(zero[0] == 0)(f)
        return deco

    def opaque(r):
        return zero[r] if isinstance(r, int) else 0

    pcp = [pltpu.make_async_copy(h, par.at[i], sems.at[i])
           for i, h in enumerate((are_hbm, aim_hbm, bre_hbm, bim_hbm, cre_hbm, cim_hbm))]
    mcp = pltpu.make_async_copy(m_hbm, mm, sems.at[6])
    xcp = [pltpu.make_async_copy(x_hbm.at[:, pl.ds(j * LN, LN)], io.at[j], sems.at[7 + j])
           for j in range(4)]
    wocp = pltpu.make_async_copy(wo_hbm, woraw, sems.at[11])
    wcp = [pltpu.make_async_copy(wqkv_hbm.at[:, pl.ds(j * LN, LN)], wraw.at[j], sems.at[12 + j])
           for j in range(12)]
    scp = [pltpu.make_async_copy(ldt_hbm, ldt_ref, sems.at[24]),
           pltpu.make_async_copy(dsk_hbm, dsk_ref, sems.at[25])]
    for c in scp + pcp:
        c.start()

    for c in scp:
        c.wait()
    dt_row = jnp.exp(ldt_ref[...].astype(F32).reshape(1, D)).astype(BF16).astype(F32)
    ds_row = dsk_ref[...].astype(F32).reshape(1, D)
    for j in range(4):
        sl = slice(j * LN, (j + 1) * LN)
        DT[sl, :] = jnp.broadcast_to(dt_row[:, sl], (LN, LN)).T
        DSK[sl, :] = jnp.broadcast_to(ds_row[:, sl], (LN, LN)).T
    with _scope('pwait'):
        for c in pcp:
            c.wait()
    for c in [mcp] + xcp + wcp + [wocp]:
        c.start()

    lane = _iota((8, LN), 1)

    def kpar(J, carry):
        rows = pl.ds(pl.multiple_of(J * 64, 64), 64)
        for i in range(6):
            PF[i, rows, :] = par[i, rows, :].astype(F32)
        return carry

    def kexp(J, slot):
        for s in range(8):
            rows = pl.ds(_mult(J * CB + s * 8, 8), 8)
            dt = DT[rows, :]
            zr, zi = dt * PF[0, rows, :], dt * PF[1, rows, :]
            mag = jnp.exp(zr)
            E[slot][0, s] = mag * jnp.cos(zi)
            yield
            E[slot][1, s] = mag * jnp.sin(zi)
            w = _cmul((PF[4, rows, :], PF[5, rows, :]), (dt * PF[2, rows, :], dt * PF[3, rows, :]))
            E[slot][2, s] = w[0] * (1.0 / S)
            E[slot][3, s] = w[1] * (1.0 / S)
            ZK[rows, :] = (jnp.sum(w[0], axis=1, keepdims=True) + DSK[rows, :]) * (1.0 / S)
            yield

    def kpow(J, slot):
        sa, sb = SA[slot], SB[slot]
        for s in range(8):
            def put(ref, i, v):
                n = (ref.shape[1] // 8 - 1) // 4
                for c in range(2):
                    ref[s // 4 * 2 + c, pl.ds(s % 4 * n + i, 8, stride=4 * n + 1), :] = v[c]

            p = (E[slot][0, s], E[slot][1, s])
            b = [None]
            for k in range(4):
                for i in range(2 ** k):
                    b.append(_cmul(b[i], p) if i else p)
                    put(sb, len(b) - 2, b[-1])
                    yield
                p = _csq(p)
            put(sb, 15, p)
            b = {4: b[4], 8: b[8], 12: b[12], 16: p}
            w = (E[slot][2, s], E[slot][3, s])
            pw = []
            for k in range(5):
                pw.append(p)
                p = _csq(p)
                yield
            e512, e1024 = p, _csq(p)
            for o, st, e in ((15, 4, e512), (19, 8, e1024), (21, 8, _cmul(e512, e1024))):
                for i in range(1, 16 // st + 1):
                    put(sb, o + i, _cmul(e, b[i * st]))
                    yield

            def tree(i, v, k):
                put(sa, i, v)
                yield
                for k2 in range(k):
                    yield from tree(i + 2 ** k2, _cmul(v, pw[k2]), k2)

            yield from tree(0, w, 5)

    def ksum(J, slot):
        sa, sb = SA[slot], SB[slot]
        q = _iota((24, LN), 1) >> 5
        for hm in range(16):
            h, m = divmod(hm, 8)
            o = [lax.dot_general(sb[2 * h + c, m * 97:m * 97 + 96, :],
                                 sa[2 * h + c, m * 129:m * 129 + LN, :],
                                 NT, preferred_element_type=F32) for c in range(2)]
            o = o[0] - o[1]
            KO[slot][h, m * 25:m * 25 + 24, :] = jnp.where(
                q < 2, jnp.where(q == 0, o[0:24], o[24:48]), jnp.where(q == 2, o[48:72], o[72:96]))
            yield

    def kspread(J, slot, h):
        kb = lambda i: KO[slot][h, pl.ds(i, 8, stride=25), :]
        rnd = lambda r, st: int(np.round(r / st))
        quarter = lane >> 5
        q1 = [None] + [pltpu.roll(kb(i), 32, 1) for i in range(16, 20)]
        q2 = [None] + [pltpu.roll(kb(i), 64, 1) for i in range(20, 22)]
        q3 = [None] + [pltpu.roll(kb(i), 96, 1) for i in range(22, 24)]
        k0, q23, rest = [], {}, {}
        for r in (16,) + tuple(range(R)):
            k2, k4, k8 = rnd(r, 2), rnd(r, 4), rnd(r, 8)
            if r:
                q0 = kb(r - 1)
                if r % 2 and k2:
                    q0 = jnp.where((lane & 31) < 16, q0, kb(2 * k2 - 1))
            for s in range(4):
                row = pl.ds(_mult(J * CB + h * 32 + s * 8, 8), 8)
                if r:
                    t = q0
                    if k8 and (k8, s) not in q23:
                        q23[k8, s] = jnp.where(quarter == (s + 2) % 4, q2[k8], q3[k8])
                    if k4:
                        if (k4, k8, s) not in rest:
                            rest[k4, k8, s] = jnp.where(
                                quarter == (s + 1) % 4, q1[k4], q23[k8, s]) if k8 else q1[k4]
                        t = jnp.where(quarter == s, t, rest[k4, k8, s])
                    if s or r == 16:
                        t = pltpu.roll(t, (LN - 32 * s + (r == 16)) % LN, 1)
                    if not k8:
                        t = jnp.where(lane < (64 if k4 else 32 if k2 else 16), t, k0[s])
                else:
                    t = jnp.where(lane == 0, ZK[row, :], k0[s])
                if r == 16:
                    k0.append(t)
                else:
                    _Buf(KT[slot]).st(r * CB + h * 32 + s * 8, t)
            yield

    def ld(b, k, h, n=8, stride=CB):
        return b.ld(2 * k * stride + h, n), b.ld((2 * k + 1) * stride + h, n)

    def st(b, k, h, v, stride=CB):
        b.st(2 * k * stride + h, v[0])
        b.st((2 * k + 1) * stride + h, v[1])

    def mat(r):
        return pltpu.bitcast(jnp.concatenate(ld(_Buf(mm), r, 0, 64, 64), axis=1), BF16)

    def kfwd(i, slot):
        g = _Buf(GK, i * 2 * R * CB, 2 * R * CB)
        for r in range(R):
            t = lax.dot_general(_Buf(KT[slot]).ld(r * CB, CB), mat(r), NN, preferred_element_type=F32)
            st(g, r, 0, (t[:, :LN], t[:, LN:]))
            yield

    def kfft(i):
        kf = _Buf(KF, i * CB, 2 * R * D - D + CB)
        for h in range(0, CB, 8):
            t = []
            for r0 in range(4):
                y = _radix4(*[ld(_Buf(GK, i * 2 * R * CB), r, h) for r in range(r0, R, 4)], -1)
                t.append([_twiddle(y[g0], r0 * g0, -1) for g0 in range(4)])
                yield
            for g0 in range(4):
                y = _radix4(t[0][g0], t[1][g0], t[2][g0], t[3][g0], -1)
                for g1 in range(4):
                    st(kf, 4 * g0 + g1, h, y[g1], D)
                yield

    iow = io.bitcast(U32)

    def xin(j):
        x = _Buf(X, j * LN)
        for rho in range(8):
            t = iow[j, pl.ds(rho, LN, stride=8), :].T
            x.st(2 * rho * D, pltpu.bitcast(t << 16, F32))
            x.st((2 * rho + 1) * D, pltpu.bitcast(t & np.uint32(0xFFFF0000), F32))
            yield

    def wprep(j):
        pr, pc = _iota((LN, LN), 0), _iota((LN, LN), 1)
        perm = jnp.where(pc == (pr & 7) * DH + (pr >> 3), 1.0, 0.0).astype(BF16)
        for c in range(3):
            t = lax.dot_general(perm, wraw[(c + 1) % 3 * 4 + j], NT, preferred_element_type=F32)
            if c == 2:
                t = t * (DH ** -0.5)
            for k in range(4):
                _Buf(W).st(k * WS + (3 * j + c) * LN // 2,
                           pltpu.bitcast(t[:, k * LN:(k + 1) * LN].astype(BF16), F32))
            yield
        t = jnp.dot(perm, woraw[j * LN:(j + 1) * LN, :], preferred_element_type=F32)
        _Buf(W).st(j * WS + 3 * D // 2, pltpu.bitcast(t.T.astype(BF16), F32))
        yield

    def kstep(J, ref):
        @block("kgen")
        def _():
            slot, m, v = ref % 2, [], []
            if 0 <= ref < NCB:
                m.append(ksum(J, slot))
            if 0 <= ref - 2:
                m.append(kfwd(J - 2, slot))
            v = [(g, 16 * KW) for g in m]
            if 0 <= ref - 1 < NCB:
                v.append((_chain(*[kspread(J - 1, 1 - slot, h) for h in range(2)]), 34))
            if 0 <= ref + 1 < NCB:
                v.append((kpow(J + 1, 1 - slot), 8 * 60))
            if ref + 2 < NCB:
                v.append((kexp(J + 2, slot), 16))
            if ref >= NCB:
                js = (2 * (ref - NCB), 2 * (ref - NCB) + 1)
                v += [(_chain(*map(xin, js)), 16), (_chain(*map(wprep, js)), 8)]
            _weave(*v)

    lax.fori_loop(0, D // 64, kpar, 0)
    for J in range(-2, 2):
        kstep(J, J)
    with _scope("mwait"):
        mcp.wait()
    _loop(1, 3, lambda k: (kstep(2 * k, 2), kstep(2 * k + 1, 3)), 1)
    for J in range(6, 10):
        if J == NCB:
            with _scope("xwait"):
                for c in xcp + wcp + [wocp]:
                    c.wait()
        kstep(J, J)

    def colsum(f, step):
        acc = [f(c * 8) for c in range(4)]
        for i in range(4, D // 8):
            acc[i % 4] = acc[i % 4] + f(i * 8)
            if i % step == step - 1:
                yield
        s = jnp.sum((acc[0] + acc[1]) + (acc[2] + acc[3]), axis=0, keepdims=True)
        return jnp.broadcast_to(s * (1.0 / D), (8, LN))

    def ln_stats(ref, base):
        x = _Buf(ref, base + zero[0], D)
        m = yield from colsum(lambda c: x.ld(c, 8), 32)
        x = _Buf(ref, base + zero[1], D)
        v = yield from colsum(lambda c: jnp.square(x.ld(c, 8) - m), 8)
        return _Buf(ref, base + zero[2], D), m, lax.rsqrt(v + EPS)

    def ln(ref, base, out, r):
        x, m, rs = yield from ln_stats(ref, base)
        for c in range(0, D, 16):
            t = [(x.ld(c + k, 8) - m) * rs for k in (0, 8)]
            _Buf(out, r * D).st(c, jnp.concatenate(t, axis=0))
            if c % 64 == 48:
                yield

    def ln1(r):
        return ln(X, r * D, XN, r)

    def ln2(r):
        return ln(Z[r], 0, U, r)

    def wdot(c, n, rhs):
        lhs = jnp.concatenate(
            [pltpu.bitcast(W[t * WS + c // 2:t * WS + (c + n) // 2, :], BF16)
             for t in range(4)], axis=1)
        return jnp.dot(lhs, rhs.ld(0, D), preferred_element_type=F32)

    def qkvproj(j, r):
        b, i = _Buf(KVQ[j % 2][r % 2]), r // 2
        for c in range(3):
            t = wdot((3 * j + c) * LN, LN, _Buf(XN, r * D + zero[(r + c) % R], D))
            if c == 2:
                b.st((32 + i) * TS, t)
            else:
                b.st((16 * c + 8 + i) * TS, t)
                if i:
                    b.st((16 * c + i) * TS, pltpu.roll(t, 1, 1))
            yield

    def core(j, r):
        b, i = _Buf(KVQ[j % 2][r % 2], zero[r], 40 * TS), r // 2
        lg = [None] * WIN
        for dh in range(DH):
            q = b.ld((32 + i) * TS + dh * 8, 8)
            for w in range(WIN):
                t = q * b.ld((8 + i - w) * TS + dh * 8, 8)
                lg[w] = t if dh == 0 else lg[w] + t
            if dh % 2:
                yield
        for w in range(i + 1, WIN):
            lg[w] = jnp.where(lane > 0, lg[w], -1e9)
        mx = _tree(jnp.maximum, lg)
        e = [jnp.exp(v - mx) for v in lg]
        inv = 1.0 / _tree(jnp.add, e)
        e = [v * inv for v in e]
        yield
        yield
        for dh in range(0, DH, 2):
            oo = []
            for k in (dh, dh + 1):
                acc = None
                for w in range(WIN):
                    t = e[w] * b.ld((24 + i - w) * TS + k * 8, 8)
                    acc = t if acc is None else acc + t
                oo.append(acc)
            _Buf(O, r * D + j * LN).st(dh * 8, jnp.concatenate(oo, axis=0))
            yield

    def oproj(r):
        for c in range(0, D, DO):
            Z[r][c:c + DO, :] = X[r * D + c:r * D + c + DO, :] + wdot(
                3 * D + c, DO, _Buf(O, r * D + zero[(r + c // DO) % R], D))
            yield

    def cmxu(fi, ii, slot):
        if fi is not None:
            u_ = _Buf(U, fi * CB, R * D - D + CB)
        if ii is not None:
            x = _Buf(X, ii * CB, R * D - D + CB)
        for r in order:
            if fi is not None:
                t = lax.dot_general(u_.ld(r * D, CB), mat(r), NN, preferred_element_type=F32)
                st(_Buf(G[slot]), r, 0, (t[:, :LN], t[:, LN:]))
                yield
            if ii is not None:
                lhs = jnp.concatenate(ld(_Buf(HH[slot]), r, 0, CB), axis=1)
                t = lax.dot_general(lhs, mat(r), NT, preferred_element_type=F32)
                x.st(r * D, _Buf(Z[r], ii * CB, CB).ld(0, CB) + t)
                yield

    def cmid(i, slot):
        g, hh = _Buf(G[slot], zero[0], 2 * R * CB), _Buf(HH[slot])
        kf = _Buf(KF, i * CB, 2 * R * D - D + CB)

        for h in range(0, CB, 8):
            t, v = [], []
            for r0 in range(4):
                y = _radix4(*[ld(g, r, h) for r in range(r0, R, 4)], -1)
                t.append([_twiddle(y[g0], r0 * g0, -1) for g0 in range(4)])
                yield
            yield
            for g0 in range(4):
                y = _radix4(t[0][g0], t[1][g0], t[2][g0], t[3][g0], -1)
                yield
                y = [_cmul(y[g1], ld(kf, 4 * g0 + g1, h, 8, D)) for g1 in range(4)]
                yield
                y = _radix4(*y, 1)
                v.append([_twiddle(y[r0], r0 * g0, 1) for r0 in range(4)])
                yield
                if g0 != 1:
                    yield
            for r0 in range(4):
                y = _radix4(*[v[g0][r0] for g0 in range(4)], 1)
                for r1 in range(4):
                    st(hh, r0 + 4 * r1, h, y[r1])
                yield

    def ocopy(j):
        return pltpu.make_async_copy(
            io.at[j], out_hbm.at[:, pl.ds(_mult(j * LN, LN), LN)], sems.at[7 + j])

    def xout(j):
        x = _Buf(X, j * LN, R * D - D + LN)
        for rho in range(8):
            lo, hi = (pltpu.bitcast(x.ld(r * D, LN).astype(BF16).astype(F32), U32)
                      for r in (2 * rho, 2 * rho + 1))
            iow[j, pl.ds(rho, LN, stride=8), :] = ((lo >> 16) | hi).T
        ocopy(j).start()

    order = list(range(0, R, 2)) + list(range(1, R, 2))
    NCORE, NLN1, NLN2 = 18, 18, 18

    def layer(l, carry):
        @block("ph1")
        def _():
            for n, r in enumerate(order):
                _weave((qkvproj(0, r), 3), *([(ln1(order[n + 1]), NLN1 * 1.5)] if n + 1 < R else []))

        for j, lo, hi in ((1, 0, R), (2, 0, R), (3, 0, R // 2), (3, R // 2, R)):
            @block("ph2")
            def _():
                early = _chain(*[core(3, r) for r in order[:LO if lo else 0]])
                kf = _chain(*map(kfft, KB[j] if not lo else ()))
                for r in order[lo:hi]:
                    _weave((qkvproj(j, r), 3), (core(j - 1, r), NCORE),
                           (_take(early, -(-LO * NCORE // 8)), LO * NCORE / 8 + 0.01),
                           (_take(kf, len(KB[j]) * 64 // (hi - lo)), len(KB[j]) * 64 / (hi - lo)))
                _weave((early, 1))

        for prev, cur in zip(B3, B3[1:]):
            @block("ph3")
            def _():
                w, c, n = (order[u:v] for u, v in zip(prev, cur))
                _weave((_chain(*map(oproj, w)), len(w) * D // DO),
                       (_chain(*[core(3, r) for r in c]), len(c) * NCORE + 0.01),
                       (_chain(*map(ln2, n)), len(n) * NLN2 + 0.01))

        def cstep(i, slot, f=True, m=True, v=True):
            @block("conv")
            def _():
                _weave((cmxu(i + 1 if f else None, i - 1 if v else None, 1 - slot), R * (f + v)),
                       *([(cmid(i, slot), 3 * CB)] if m else []),
                       *[(ln2(r), 2 * NLN2) for r in order[B3[-1][2]:] if f and not m])
                if v and not m:
                    _weave((ln1(0), 1))

        cstep(-1, 1, m=False, v=False)
        cstep(0, 0, v=False)

        def cpair(k):
            cstep(2 * k + 1, 1)
            cstep(2 * k + 2, 0)
            pl.when(l == 1)(lambda: xout(k))

        _loop(0, NCB // 2 - 1, cpair, 1)
        cstep(NCB - 1, 1, f=False)
        cstep(NCB, 0, f=False, m=False)
        return carry

    _weave((ln1(0), 1))
    with _scope("layers"):
        lax.fori_loop(0, 2, layer, 0)
    xout(3)

    with _scope("owait"):
        for j in range(4):
            ocopy(j).wait()


@jax.jit
def pallas_interleave_layers__sliding_local_dilated__ssm_conv_s4__prompt_kernel(
    A_x: jax.Array,
    A_wqkv: jax.Array,
    A_wo: jax.Array,
    B_u: jax.Array,
    B_A_re: jax.Array,
    B_A_im: jax.Array,
    B_B_re: jax.Array,
    B_B_im: jax.Array,
    B_C_re: jax.Array,
    B_C_im: jax.Array,
    B_log_dt: jax.Array,
    B_Dskip: jax.Array,
):
    del B_u
    hbm = pl.BlockSpec(memory_space=pl.ANY)
    V = pltpu.VMEM
    out = pl.pallas_call(
        _kernel,
        out_shape=jax.ShapeDtypeStruct((S, D), BF16),
        in_specs=[hbm] * 12,
        out_specs=hbm,
        scratch_shapes=[
            V((D,), BF16), V((D,), BF16),
            V((4, S, LN), BF16),
            V((12, D, LN), BF16),
            V((D, D), BF16),
            V((6, D, LN), BF16),
            V((R * LN, LN), U32),
            V((R * D, LN), F32),
            V((2 * R * D, LN), F32),
            V((D, LN), F32),
            V((R * D, LN), BF16),
            V((R * D, LN), F32),
            V((4 * WS, LN), F32),
            [V((D, LN), F32)] * R,
            [[V((40 * TS, LN), F32)] * 2] * 2,
            V((R * D, LN), BF16),
            [V((2 * R * CB, LN), F32)] * 2,
            [V((2 * R * CB, LN), F32)] * 2,
            [V((R * CB, LN), F32)] * 2,
            V((2 * R * D, LN), F32),
            V((6, D, LN), F32),
            [V((4, 8, 8, LN), F32)] * 2,
            V((D, LN), F32),
            V((D, LN), F32),
            [V((4, 8 * 129, LN), F32)] * 2,
            [V((4, 8 * 97, LN), F32)] * 2,
            [V((2, 8 * 25, LN), F32)] * 2,
            pltpu.SMEM((R,), jnp.int32),
            pltpu.SemaphoreType.DMA((26,)),
        ],
        compiler_params=pltpu.CompilerParams(vmem_limit_bytes=100 * 1024 * 1024, flags=FLAGS),
    )(A_x.reshape(S, D), A_wqkv, A_wo, B_A_re, B_A_im, B_B_re, B_B_im, B_C_re, B_C_im,
      B_log_dt, B_Dskip, _M)
    return out.reshape(1, S, D)
```

```python
import contextlib
import numpy as np
import jax
import jax.numpy as jnp
from jax import lax
import jax.experimental.pallas as pl
import jax.experimental.pallas.tpu as pltpu

S, D, DH, WIN = 2048, 512, 16, 8
R = 16
LN = 128
CB = 64
NCB = D // CB
EPS = 1e-5
F32, BF16, U32 = jnp.float32, jnp.bfloat16, jnp.uint32
NN, NT = (((1,), (0,)), ((), ())), (((1,), (1,)), ((), ()))


def _dft_matrices():
    lam = np.arange(LN, dtype=np.float64)[None, :, None]
    r = np.arange(R, dtype=np.float64)[:, None, None]
    f = np.arange(LN, dtype=np.float64)[None, None, :]
    th = 2.0 * np.pi * (f + 0.5) * (R * lam + r) / (2 * S)
    m = np.stack([np.cos(th), -np.sin(th)], axis=1).astype(BF16).view(np.uint16).astype(np.uint32)
    return (m[:, :, 0::2] | (m[:, :, 1::2] << 16)).reshape(R * LN, LN)


_M = _dft_matrices()


SCOPES = False


def _scope(name):
    return jax.named_scope(name) if SCOPES else contextlib.nullcontext()


FLAGS = None
SKIP = NOB = ''
LO, NO = 6, 1
KW = 1
KB, L1 = (0, 3, 3, 1, 0, 1, 0, 0, 0), 1
B3 = ((0, 6, 0), (5, 11, 0), (10, 16, 5), (14, 16, 10), (16, 16, 14))
DO = 256
TS, WS = LN, 2 * D


class _Buf:
    def __init__(self, ref, base=0, size=None):
        if isinstance(base, int):
            self.ref, self.base = ref, base
        else:
            self.ref, self.base = ref.at[pl.ds(pl.multiple_of(base, 16), size), :], 0

    def ld(self, row, n):
        return self.ref[self.base + row:self.base + row + n, :]

    def st(self, row, v):
        self.ref[self.base + row:self.base + row + v.shape[0], :] = v.astype(self.ref.dtype)


def _weave(*stages):
    live = [[g, n, 0] for g, n in stages]
    while live:
        st = min(live, key=lambda t: t[2] / t[1])
        try:
            next(st[0])
            st[2] += 1
        except StopIteration:
            live.remove(st)


def _chain(*gens):
    for g in gens:
        yield from g


def _take(g, n):
    for _, _ in zip(range(n), g):
        yield


def _tree(op, v):
    while len(v) > 1:
        v = [op(v[i], v[i + 1]) for i in range(0, len(v), 2)]
    return v[0]


def _mult(i, n):
    return i if isinstance(i, int) else pl.multiple_of(i, n)


def _loop(lo, hi, body, unroll, force=False):
    n = hi - lo
    assert n % unroll == 0
    if n == unroll and not force:
        for i in range(lo, hi):
            body(i)
        return

    def outer(k, carry):
        for u in range(unroll):
            body(lo + k * unroll + u)
        return carry

    lax.fori_loop(0, n // unroll, outer, 0)


def _iota(shape, dim):
    return lax.broadcasted_iota(jnp.int32, shape, dim)


def _cmul(a, b):
    return (a[0] * b[0] - a[1] * b[1], a[0] * b[1] + a[1] * b[0])


def _csq(a):
    t = a[0] * a[1]
    return (a[0] * a[0] - a[1] * a[1], t + t)


def _radix4(a, b, c, d, sign):
    s0 = (a[0] + c[0], a[1] + c[1])
    d0 = (a[0] - c[0], a[1] - c[1])
    s1 = (b[0] + d[0], b[1] + d[1])
    d1 = (b[0] - d[0], b[1] - d[1])
    y0 = (s0[0] + s1[0], s0[1] + s1[1])
    y2 = (s0[0] - s1[0], s0[1] - s1[1])
    p = (d0[0] - d1[1], d0[1] + d1[0])
    m = (d0[0] + d1[1], d0[1] - d1[0])
    return (y0, p, y2, m) if sign > 0 else (y0, m, y2, p)


def _twiddle(a, k, sign):
    if k == 0:
        return a
    c = float(np.cos(2 * np.pi * k / 16))
    s = float(sign * np.sin(2 * np.pi * k / 16))
    if k == 4:
        return (-a[1], a[0]) if sign > 0 else (a[1], -a[0])
    if k == 2:
        if sign > 0:
            return ((a[0] - a[1]) * c, (a[0] + a[1]) * c)
        return ((a[0] + a[1]) * c, (a[1] - a[0]) * c)
    if k == 6:
        if sign > 0:
            return ((a[0] + a[1]) * c, (a[1] - a[0]) * c)
        return ((a[0] - a[1]) * c, (a[0] + a[1]) * c)
    return (a[0] * c - a[1] * s, a[0] * s + a[1] * c)


def _kernel(x_hbm, wqkv_hbm, wo_hbm, are_hbm, aim_hbm, bre_hbm, bim_hbm, cre_hbm, cim_hbm,
            ldt_hbm, dsk_hbm, m_hbm, out_hbm, ldt_ref, dsk_ref,
            io, wraw, woraw, par, mm, X, KF, DSK, XN, U, W, Z, KVQ, O, G, HH,
            KT, GK, PF, E, DT, ZK, SA, SB, KO, zero, sems):
    for k in range(R):
        zero[k] = 0

    def block(name):
        def deco(f):
            if SKIP and name in SKIP:
                return
            with _scope(name):
                f() if name in NOB else pl.when(zero[0] == 0)(f)
        return deco

    def opaque(r):
        return zero[r] if isinstance(r, int) else 0

    pcp = [pltpu.make_async_copy(h, par.at[i], sems.at[i])
           for i, h in enumerate((are_hbm, aim_hbm, bre_hbm, bim_hbm, cre_hbm, cim_hbm))]
    mcp = pltpu.make_async_copy(m_hbm, mm, sems.at[6])
    xcp = [pltpu.make_async_copy(x_hbm.at[:, pl.ds(j * LN, LN)], io.at[j], sems.at[7 + j])
           for j in range(4)]
    wocp = pltpu.make_async_copy(wo_hbm, woraw, sems.at[11])
    wcp = [pltpu.make_async_copy(wqkv_hbm.at[:, pl.ds(j * LN, LN)], wraw.at[j], sems.at[12 + j])
           for j in range(12)]
    scp = [pltpu.make_async_copy(ldt_hbm, ldt_ref, sems.at[24]),
           pltpu.make_async_copy(dsk_hbm, dsk_ref, sems.at[25])]
    for c in scp + pcp:
        c.start()

    for c in scp:
        c.wait()
    dt_row = jnp.exp(ldt_ref[...].astype(F32).reshape(1, D)).astype(BF16).astype(F32)
    ds_row = dsk_ref[...].astype(F32).reshape(1, D)
    for j in range(4):
        sl = slice(j * LN, (j + 1) * LN)
        DT[sl, :] = jnp.broadcast_to(dt_row[:, sl], (LN, LN)).T
        DSK[sl, :] = jnp.broadcast_to(ds_row[:, sl], (LN, LN)).T
    with _scope('pwait'):
        for c in pcp:
            c.wait()
    for c in [mcp] + xcp + wcp + [wocp]:
        c.start()

    lane = _iota((8, LN), 1)

    def kpar(J, carry):
        rows = pl.ds(pl.multiple_of(J * 64, 64), 64)
        for i in range(6):
            PF[i, rows, :] = par[i, rows, :].astype(F32)
        return carry

    def kexp(J, slot):
        for s in range(8):
            rows = pl.ds(_mult(J * CB + s * 8, 8), 8)
            dt = DT[rows, :]
            zr, zi = dt * PF[0, rows, :], dt * PF[1, rows, :]
            mag = jnp.exp(zr)
            E[slot][0, s] = mag * jnp.cos(zi)
            yield
            E[slot][1, s] = mag * jnp.sin(zi)
            w = _cmul((PF[4, rows, :], PF[5, rows, :]), (dt * PF[2, rows, :], dt * PF[3, rows, :]))
            E[slot][2, s] = w[0] * (1.0 / S)
            E[slot][3, s] = w[1] * (1.0 / S)
            ZK[rows, :] = (jnp.sum(w[0], axis=1, keepdims=True) + DSK[rows, :]) * (1.0 / S)
            yield

    def kpow(J, slot):
        sa, sb = SA[slot], SB[slot]
        for s in range(8):
            def put(ref, i, v):
                n = (ref.shape[1] // 8 - 1) // 4
                for c in range(2):
                    ref[s // 4 * 2 + c, pl.ds(s % 4 * n + i, 8, stride=4 * n + 1), :] = v[c]

            p = (E[slot][0, s], E[slot][1, s])
            b = [None]
            for k in range(4):
                for i in range(2 ** k):
                    b.append(_cmul(b[i], p) if i else p)
                    put(sb, len(b) - 2, b[-1])
                    yield
                p = _csq(p)
            put(sb, 15, p)
            b = {4: b[4], 8: b[8], 12: b[12], 16: p}
            w = (E[slot][2, s], E[slot][3, s])
            pw = []
            for k in range(5):
                pw.append(p)
                p = _csq(p)
                yield
            e512, e1024 = p, _csq(p)
            for o, st, e in ((15, 4, e512), (19, 8, e1024), (21, 8, _cmul(e512, e1024))):
                for i in range(1, 16 // st + 1):
                    put(sb, o + i, _cmul(e, b[i * st]))
                    yield

            def tree(i, v, k):
                put(sa, i, v)
                yield
                for k2 in range(k):
                    yield from tree(i + 2 ** k2, _cmul(v, pw[k2]), k2)

            yield from tree(0, w, 5)

    def ksum(J, slot):
        sa, sb = SA[slot], SB[slot]
        q = _iota((24, LN), 1) >> 5
        for hm in range(16):
            h, m = divmod(hm, 8)
            o = [lax.dot_general(sb[2 * h + c, m * 97:m * 97 + 96, :],
                                 sa[2 * h + c, m * 129:m * 129 + LN, :],
                                 NT, preferred_element_type=F32) for c in range(2)]
            o = o[0] - o[1]
            KO[slot][h, m * 25:m * 25 + 24, :] = jnp.where(
                q < 2, jnp.where(q == 0, o[0:24], o[24:48]), jnp.where(q == 2, o[48:72], o[72:96]))
            yield

    def kspread(J, slot, h):
        kb = lambda i: KO[slot][h, pl.ds(i, 8, stride=25), :]
        rnd = lambda r, st: int(np.round(r / st))
        quarter = lane >> 5
        q1 = [None] + [pltpu.roll(kb(i), 32, 1) for i in range(16, 20)]
        q2 = [None] + [pltpu.roll(kb(i), 64, 1) for i in range(20, 22)]
        q3 = [None] + [pltpu.roll(kb(i), 96, 1) for i in range(22, 24)]
        k0, q23, rest = [], {}, {}
        for r in (16,) + tuple(range(R)):
            k2, k4, k8 = rnd(r, 2), rnd(r, 4), rnd(r, 8)
            if r:
                q0 = kb(r - 1)
                if r % 2 and k2:
                    q0 = jnp.where((lane & 31) < 16, q0, kb(2 * k2 - 1))
            for s in range(4):
                row = pl.ds(_mult(J * CB + h * 32 + s * 8, 8), 8)
                if r:
                    t = q0
                    if k8 and (k8, s) not in q23:
                        q23[k8, s] = jnp.where(quarter == (s + 2) % 4, q2[k8], q3[k8])
                    if k4:
                        if (k4, k8, s) not in rest:
                            rest[k4, k8, s] = jnp.where(
                                quarter == (s + 1) % 4, q1[k4], q23[k8, s]) if k8 else q1[k4]
                        t = jnp.where(quarter == s, t, rest[k4, k8, s])
                    if s or r == 16:
                        t = pltpu.roll(t, (LN - 32 * s + (r == 16)) % LN, 1)
                    if not k8:
                        t = jnp.where(lane < (64 if k4 else 32 if k2 else 16), t, k0[s])
                else:
                    t = jnp.where(lane == 0, ZK[row, :], k0[s])
                if r == 16:
                    k0.append(t)
                else:
                    _Buf(KT[slot]).st(r * CB + h * 32 + s * 8, t)
            yield

    def ld(b, k, h, n=8, stride=CB):
        return b.ld(2 * k * stride + h, n), b.ld((2 * k + 1) * stride + h, n)

    def st(b, k, h, v, stride=CB):
        b.st(2 * k * stride + h, v[0])
        b.st((2 * k + 1) * stride + h, v[1])

    def mat(r):
        return pltpu.bitcast(jnp.concatenate(ld(_Buf(mm), r, 0, 64, 64), axis=1), BF16)

    def kfwd(i, slot):
        g = _Buf(GK, i * 2 * R * CB, 2 * R * CB)
        for r in range(R):
            t = lax.dot_general(_Buf(KT[slot]).ld(r * CB, CB), mat(r), NN, preferred_element_type=F32)
            st(g, r, 0, (t[:, :LN], t[:, LN:]))
            yield

    def kfft(i):
        kf = _Buf(KF, i * CB, 2 * R * D - D + CB)
        for h in range(0, CB, 8):
            t = []
            for r0 in range(4):
                y = _radix4(*[ld(_Buf(GK, i * 2 * R * CB), r, h) for r in range(r0, R, 4)], -1)
                t.append([_twiddle(y[g0], r0 * g0, -1) for g0 in range(4)])
                yield
            for g0 in range(4):
                y = _radix4(t[0][g0], t[1][g0], t[2][g0], t[3][g0], -1)
                for g1 in range(4):
                    st(kf, 4 * g0 + g1, h, y[g1], D)
                yield

    iow = io.bitcast(U32)

    def xin(j):
        x = _Buf(X, j * LN)
        for rho in range(8):
            t = iow[j, pl.ds(rho, LN, stride=8), :].T
            x.st(2 * rho * D, pltpu.bitcast(t << 16, F32))
            x.st((2 * rho + 1) * D, pltpu.bitcast(t & np.uint32(0xFFFF0000), F32))
            yield

    def wprep(j):
        pr, pc = _iota((LN, LN), 0), _iota((LN, LN), 1)
        perm = jnp.where(pc == (pr & 7) * DH + (pr >> 3), 1.0, 0.0).astype(BF16)
        for c in range(3):
            t = lax.dot_general(perm, wraw[(c + 1) % 3 * 4 + j], NT, preferred_element_type=F32)
            if c == 2:
                t = t * (DH ** -0.5)
            for k in range(4):
                _Buf(W).st(k * WS + (3 * j + c) * LN // 2,
                           pltpu.bitcast(t[:, k * LN:(k + 1) * LN].astype(BF16), F32))
            yield
        t = jnp.dot(perm, woraw[j * LN:(j + 1) * LN, :], preferred_element_type=F32)
        _Buf(W).st(j * WS + 3 * D // 2, pltpu.bitcast(t.T.astype(BF16), F32))
        yield

    def kstep(J, ref):
        @block("kgen")
        def _():
            slot, m, v = ref % 2, [], []
            if 0 <= ref < NCB:
                m.append(ksum(J, slot))
            if 0 <= ref - 2:
                m.append(kfwd(J - 2, slot))
            v = [(g, 16 * KW) for g in m]
            if 0 <= ref - 1 < NCB:
                v.append((_chain(*[kspread(J - 1, 1 - slot, h) for h in range(2)]), 34))
            if 0 <= ref + 1 < NCB:
                v.append((kpow(J + 1, 1 - slot), 8 * 60))
            if ref + 2 < NCB:
                v.append((kexp(J + 2, slot), 16))
            if ref >= NCB:
                js = (2 * (ref - NCB), 2 * (ref - NCB) + 1)
                v += [(_chain(*map(xin, js)), 16), (_chain(*map(wprep, js)), 8)]
            _weave(*v)

    lax.fori_loop(0, D // 64, kpar, 0)
    for J in range(-2, 2):
        kstep(J, J)
    with _scope("mwait"):
        mcp.wait()
    _loop(1, 3, lambda k: (kstep(2 * k, 2), kstep(2 * k + 1, 3)), 1)
    for J in range(6, 10):
        if J == NCB:
            with _scope("xwait"):
                for c in xcp + wcp + [wocp]:
                    c.wait()
        kstep(J, J)

    def colsum(f, step):
        acc = [f(c * 8) for c in range(4)]
        for i in range(4, D // 8):
            acc[i % 4] = acc[i % 4] + f(i * 8)
            if i % step == step - 1:
                yield
        s = jnp.sum((acc[0] + acc[1]) + (acc[2] + acc[3]), axis=0, keepdims=True)
        return jnp.broadcast_to(s * (1.0 / D), (8, LN))

    def ln_stats(ref, base):
        x = _Buf(ref, base + zero[0], D)
        m = yield from colsum(lambda c: x.ld(c, 8), 32)
        x = _Buf(ref, base + zero[1], D)
        v = yield from colsum(lambda c: jnp.square(x.ld(c, 8) - m), 8)
        return _Buf(ref, base + zero[2], D), m, lax.rsqrt(v + EPS)

    def ln(ref, base, out, r):
        x, m, rs = yield from ln_stats(ref, base)
        for c in range(0, D, 16):
            t = [(x.ld(c + k, 8) - m) * rs for k in (0, 8)]
            _Buf(out, r * D).st(c, jnp.concatenate(t, axis=0))
            if c % 64 == 48:
                yield

    def ln1(r):
        return ln(X, r * D, XN, r)

    def ln2(r):
        return ln(Z[r], 0, U, r)

    def wdot(c, n, rhs):
        lhs = jnp.concatenate(
            [pltpu.bitcast(W[t * WS + c // 2:t * WS + (c + n) // 2, :], BF16)
             for t in range(4)], axis=1)
        return jnp.dot(lhs, rhs.ld(0, D), preferred_element_type=F32)

    def qkvproj(j, r):
        b, i = _Buf(KVQ[j % 2][r % 2]), r // 2
        for c in range(3):
            t = wdot((3 * j + c) * LN, LN, _Buf(XN, r * D + zero[(r + c) % R], D))
            if c == 2:
                b.st((32 + i) * TS, t)
            else:
                b.st((16 * c + 8 + i) * TS, t)
                if i:
                    b.st((16 * c + i) * TS, pltpu.roll(t, 1, 1))
            yield

    def core(j, r):
        b, i = _Buf(KVQ[j % 2][r % 2], zero[r], 40 * TS), r // 2
        lg = [None] * WIN
        for dh in range(DH):
            q = b.ld((32 + i) * TS + dh * 8, 8)
            for w in range(WIN):
                t = q * b.ld((8 + i - w) * TS + dh * 8, 8)
                lg[w] = t if dh == 0 else lg[w] + t
            if dh % 2:
                yield
        for w in range(i + 1, WIN):
            lg[w] = jnp.where(lane > 0, lg[w], -1e9)
        mx = _tree(jnp.maximum, lg)
        e = [jnp.exp(v - mx) for v in lg]
        inv = 1.0 / _tree(jnp.add, e)
        e = [v * inv for v in e]
        yield
        yield
        for dh in range(0, DH, 2):
            oo = []
            for k in (dh, dh + 1):
                acc = None
                for w in range(WIN):
                    t = e[w] * b.ld((24 + i - w) * TS + k * 8, 8)
                    acc = t if acc is None else acc + t
                oo.append(acc)
            _Buf(O, r * D + j * LN).st(dh * 8, jnp.concatenate(oo, axis=0))
            yield

    def oproj(r):
        for c in range(0, D, DO):
            Z[r][c:c + DO, :] = X[r * D + c:r * D + c + DO, :] + wdot(
                3 * D + c, DO, _Buf(O, r * D + zero[(r + c // DO) % R], D))
            yield

    def cmxu(fi, ii, slot, rs):
        if fi is not None:
            u_ = _Buf(U, fi * CB, R * D - D + CB)
        if ii is not None:
            x = _Buf(X, ii * CB, R * D - D + CB)
        for r in rs:
            if fi is not None:
                t = lax.dot_general(u_.ld(r * D, CB), mat(r), NN, preferred_element_type=F32)
                st(_Buf(G[slot]), r, 0, (t[:, :LN], t[:, LN:]))
                yield
            if ii is not None:
                lhs = jnp.concatenate(ld(_Buf(HH[slot]), r, 0, CB), axis=1)
                t = lax.dot_general(lhs, mat(r), NT, preferred_element_type=F32)
                x.st(r * D, _Buf(Z[r], ii * CB, CB).ld(0, CB) + t)
                yield

    def cmid(i, slot):
        g, hh = _Buf(G[slot], zero[0], 2 * R * CB), _Buf(HH[slot])
        kf = _Buf(KF, i * CB, 2 * R * D - D + CB)

        for h in range(0, CB, 8):
            t, v = [], []
            for r0 in range(4):
                y = _radix4(*[ld(g, r, h) for r in range(r0, R, 4)], -1)
                t.append([_twiddle(y[g0], r0 * g0, -1) for g0 in range(4)])
                yield
            yield
            for g0 in range(4):
                y = _radix4(t[0][g0], t[1][g0], t[2][g0], t[3][g0], -1)
                yield
                y = [_cmul(y[g1], ld(kf, 4 * g0 + g1, h, 8, D)) for g1 in range(4)]
                yield
                y = _radix4(*y, 1)
                v.append([_twiddle(y[r0], r0 * g0, 1) for r0 in range(4)])
                yield
                if g0 != 1:
                    yield
            for r0 in range(4):
                y = _radix4(*[v[g0][r0] for g0 in range(4)], 1)
                for r1 in range(4):
                    st(hh, r0 + 4 * r1, h, y[r1])
                yield

    def ocopy(j):
        n = S // NO
        return [pltpu.make_async_copy(
            io.at[j, pl.ds(k * n, n), :],
            out_hbm.at[pl.ds(k * n, n), pl.ds(_mult(j * LN, LN), LN)], sems.at[NO * j + k])
            for k in range(NO)]

    def xout(j):
        x = _Buf(X, j * LN, R * D - D + LN)
        for rho in range(8):
            lo, hi = (pltpu.bitcast(x.ld(r * D, LN).astype(BF16).astype(F32), U32)
                      for r in (2 * rho, 2 * rho + 1))
            iow[j, pl.ds(rho, LN, stride=8), :] = ((lo >> 16) | hi).T
            yield
        for c in ocopy(j):
            c.start()

    order = list(range(0, R, 2)) + list(range(1, R, 2))
    NCORE, NLN1, NLN2 = 18, 18, 18

    def layer(l, carry):
        def spectra(b):
            ids = range(sum(KB[:b]), sum(KB[:b + 1]))
            return _chain(*map(kfft, ids)), 64 * len(ids) + 0.01

        @block("ph1")
        def _():
            _weave((_chain(*[qkvproj(0, r) for r in order]), 3 * R),
                   (_chain(*map(ln1, order[1:])), NLN1 * (R + L1)), spectra(0))

        for b, (j, lo, hi) in enumerate(((1, 0, R), (2, 0, R), (3, 0, R // 2), (3, R // 2, R))):
            @block("ph2")
            def _():
                early = _chain(*[core(3, r) for r in order[:LO if lo else 0]])
                kf, nk = spectra(1 + b)
                nk = int(nk) // (hi - lo)
                for r in order[lo:hi]:
                    _weave((qkvproj(j, r), 3), (core(j - 1, r), NCORE),
                           (_take(early, -(-LO * NCORE // 8)), LO * NCORE / 8),
                           (_take(kf, nk), nk + 0.01))

        for b, (prev, cur) in enumerate(zip(B3, B3[1:])):
            @block("ph3")
            def _():
                w, c, n = (order[u:v] for u, v in zip(prev, cur))
                _weave((_chain(*map(oproj, w)), len(w) * D // DO),
                       (_chain(*[core(3, r) for r in c]), len(c) * NCORE + 0.01),
                       (_chain(*map(ln2, n)), len(n) * NLN2 + 0.01), spectra(5 + b))

        def cstep(i, slot, f=True, m=True, v=True):
            @block("conv")
            def _():
                _weave((cmxu(i + 1 if f else None, i - 1 if v else None, 1 - slot, order), R * (f + v)),
                       *([(cmid(i, slot), 3 * CB)] if m else []),
                       *[(ln2(r), 2 * NLN2) for r in order[B3[-1][2]:] if f and not m])

        cstep(-1, 1, m=False, v=False)
        cstep(0, 0, v=False)

        def cpair(k):
            cstep(2 * k + 1, 1)
            cstep(2 * k + 2, 0)
            pl.when(l == 1)(lambda: _weave((xout(k), 1)))

        _loop(0, NCB // 2 - 1, cpair, 1)
        cstep(NCB - 1, 1, f=False)

        @pl.when(l == 0)
        def _():
            _weave((_chain(cmxu(None, NCB - 1, 1, order), ln1(0)), 1))

        @pl.when(l == 1)
        def _():
            m = cmxu(None, NCB - 1, 1, range(R))
            _weave((_take(m, 4), 1))
            _weave((xout(3), 8), (m, R))

        return carry

    _weave((ln1(0), 1))
    with _scope("layers"):
        lax.fori_loop(0, 2, layer, 0)

    with _scope("owait"):
        for j in range(4):
            for c in ocopy(j):
                c.wait()


@jax.jit
def pallas_interleave_layers__sliding_local_dilated__ssm_conv_s4__prompt_kernel(
    A_x: jax.Array,
    A_wqkv: jax.Array,
    A_wo: jax.Array,
    B_u: jax.Array,
    B_A_re: jax.Array,
    B_A_im: jax.Array,
    B_B_re: jax.Array,
    B_B_im: jax.Array,
    B_C_re: jax.Array,
    B_C_im: jax.Array,
    B_log_dt: jax.Array,
    B_Dskip: jax.Array,
):
    del B_u
    hbm = pl.BlockSpec(memory_space=pl.ANY)
    V = pltpu.VMEM
    out = pl.pallas_call(
        _kernel,
        out_shape=jax.ShapeDtypeStruct((S, D), BF16),
        in_specs=[hbm] * 12,
        out_specs=hbm,
        scratch_shapes=[
            V((D,), BF16), V((D,), BF16),
            V((4, S, LN), BF16),
            V((12, D, LN), BF16),
            V((D, D), BF16),
            V((6, D, LN), BF16),
            V((R * LN, LN), U32),
            V((R * D, LN), F32),
            V((2 * R * D, LN), F32),
            V((D, LN), F32),
            V((R * D, LN), BF16),
            V((R * D, LN), F32),
            V((4 * WS, LN), F32),
            [V((D, LN), F32)] * R,
            [[V((40 * TS, LN), F32)] * 2] * 2,
            V((R * D, LN), BF16),
            [V((2 * R * CB, LN), F32)] * 2,
            [V((2 * R * CB, LN), F32)] * 2,
            [V((R * CB, LN), F32)] * 2,
            V((2 * R * D, LN), F32),
            V((6, D, LN), F32),
            [V((4, 8, 8, LN), F32)] * 2,
            V((D, LN), F32),
            V((D, LN), F32),
            [V((4, 8 * 129, LN), F32)] * 2,
            [V((4, 8 * 97, LN), F32)] * 2,
            [V((2, 8 * 25, LN), F32)] * 2,
            pltpu.SMEM((R,), jnp.int32),
            pltpu.SemaphoreType.DMA((26,)),
        ],
        compiler_params=pltpu.CompilerParams(vmem_limit_bytes=100 * 1024 * 1024, flags=FLAGS),
    )(A_x.reshape(S, D), A_wqkv, A_wo, B_A_re, B_A_im, B_B_re, B_B_im, B_C_re, B_C_im,
      B_log_dt, B_Dskip, _M)
    return out.reshape(1, S, D)
```

```python
import contextlib
import numpy as np
import jax
import jax.numpy as jnp
from jax import lax
import jax.experimental.pallas as pl
import jax.experimental.pallas.tpu as pltpu

S, D, DH, WIN = 2048, 512, 16, 8
R = 16
LN = 128
CB = 64
NCB = D // CB
EPS = 1e-5
F32, BF16, U32 = jnp.float32, jnp.bfloat16, jnp.uint32
NN, NT = (((1,), (0,)), ((), ())), (((1,), (1,)), ((), ()))


def _dft_matrices():
    lam = np.arange(LN, dtype=np.float64)[None, :, None]
    r = np.arange(R, dtype=np.float64)[:, None, None]
    f = np.arange(LN, dtype=np.float64)[None, None, :]
    th = 2.0 * np.pi * (f + 0.5) * (R * lam + r) / (2 * S)
    m = np.stack([np.cos(th), -np.sin(th)], axis=1).astype(BF16).view(np.uint16).astype(np.uint32)
    return (m[:, :, 0::2] | (m[:, :, 1::2] << 16)).reshape(R * LN, LN)


_M = _dft_matrices()


SCOPES = False


def _scope(name):
    return jax.named_scope(name) if SCOPES else contextlib.nullcontext()


FLAGS = None
SKIP = NOB = ''
LO, NO = 6, 1
KW = 1
KB, L1 = (0, 3, 3, 1, 0, 1, 0, 0, 0), 1
B3 = ((0, 6, 0), (5, 11, 0), (10, 16, 5), (14, 16, 10), (16, 16, 14))
DO = 256
TS, WS = LN, 2 * D


class _Buf:
    def __init__(self, ref, base=0, size=None):
        if isinstance(base, int):
            self.ref, self.base = ref, base
        else:
            self.ref, self.base = ref.at[pl.ds(pl.multiple_of(base, 16), size), :], 0

    def ld(self, row, n):
        return self.ref[self.base + row:self.base + row + n, :]

    def st(self, row, v):
        self.ref[self.base + row:self.base + row + v.shape[0], :] = v.astype(self.ref.dtype)


def _weave(*stages):
    live = [[g, n, 0] for g, n in stages]
    while live:
        st = min(live, key=lambda t: t[2] / t[1])
        try:
            next(st[0])
            st[2] += 1
        except StopIteration:
            live.remove(st)


def _chain(*gens):
    for g in gens:
        yield from g


def _take(g, n):
    for _, _ in zip(range(n), g):
        yield


def _tree(op, v):
    while len(v) > 1:
        v = [op(v[i], v[i + 1]) for i in range(0, len(v), 2)]
    return v[0]


def _mult(i, n):
    return i if isinstance(i, int) else pl.multiple_of(i, n)


def _loop(lo, hi, body, unroll, force=False):
    n = hi - lo
    assert n % unroll == 0
    if n == unroll and not force:
        for i in range(lo, hi):
            body(i)
        return

    def outer(k, carry):
        for u in range(unroll):
            body(lo + k * unroll + u)
        return carry

    lax.fori_loop(0, n // unroll, outer, 0)


def _iota(shape, dim):
    return lax.broadcasted_iota(jnp.int32, shape, dim)


def _cmul(a, b):
    return (a[0] * b[0] - a[1] * b[1], a[0] * b[1] + a[1] * b[0])


def _csq(a):
    t = a[0] * a[1]
    return (a[0] * a[0] - a[1] * a[1], t + t)


def _radix4(a, b, c, d, sign):
    s0 = (a[0] + c[0], a[1] + c[1])
    d0 = (a[0] - c[0], a[1] - c[1])
    s1 = (b[0] + d[0], b[1] + d[1])
    d1 = (b[0] - d[0], b[1] - d[1])
    y0 = (s0[0] + s1[0], s0[1] + s1[1])
    y2 = (s0[0] - s1[0], s0[1] - s1[1])
    p = (d0[0] - d1[1], d0[1] + d1[0])
    m = (d0[0] + d1[1], d0[1] - d1[0])
    return (y0, p, y2, m) if sign > 0 else (y0, m, y2, p)


def _twiddle(a, k, sign):
    if k == 0:
        return a
    c = float(np.cos(2 * np.pi * k / 16))
    s = float(sign * np.sin(2 * np.pi * k / 16))
    if k == 4:
        return (-a[1], a[0]) if sign > 0 else (a[1], -a[0])
    if k == 2:
        if sign > 0:
            return ((a[0] - a[1]) * c, (a[0] + a[1]) * c)
        return ((a[0] + a[1]) * c, (a[1] - a[0]) * c)
    if k == 6:
        if sign > 0:
            return ((a[0] + a[1]) * c, (a[1] - a[0]) * c)
        return ((a[0] - a[1]) * c, (a[0] + a[1]) * c)
    return (a[0] * c - a[1] * s, a[0] * s + a[1] * c)


def _kernel(x_hbm, wqkv_hbm, wo_hbm, are_hbm, aim_hbm, bre_hbm, bim_hbm, cre_hbm, cim_hbm,
            ldt_hbm, dsk_hbm, m_hbm, out_hbm, ldt_ref, dsk_ref,
            io, wraw, woraw, par, mm, X, KF, DSK, XN, U, W, Z, KVQ, O, G, HH,
            KT, GK, E, DT, ZK, SA, SB, KO, zero, sems):
    for k in range(R):
        zero[k] = 0

    def block(name):
        def deco(f):
            if SKIP and name in SKIP:
                return
            with _scope(name):
                f() if name in NOB else pl.when(zero[0] == 0)(f)
        return deco

    def opaque(r):
        return zero[r] if isinstance(r, int) else 0

    pcp = [[pltpu.make_async_copy(h.at[rows, :], par.at[i, rows, :], sems.at[o + i])
            for i, h in enumerate((are_hbm, aim_hbm, bre_hbm, bim_hbm, cre_hbm, cim_hbm))]
           for o, rows in ((0, pl.ds(0, 2 * CB)), (26, pl.ds(2 * CB, D - 2 * CB)))]
    mcp = pltpu.make_async_copy(m_hbm, mm, sems.at[6])
    xcp = [pltpu.make_async_copy(x_hbm.at[:, pl.ds(j * LN, LN)], io.at[j], sems.at[7 + j])
           for j in range(4)]
    wocp = pltpu.make_async_copy(wo_hbm, woraw, sems.at[11])
    wcp = [pltpu.make_async_copy(wqkv_hbm.at[:, pl.ds(j * LN, LN)], wraw.at[j], sems.at[12 + j])
           for j in range(12)]
    scp = [pltpu.make_async_copy(ldt_hbm, ldt_ref, sems.at[24]),
           pltpu.make_async_copy(dsk_hbm, dsk_ref, sems.at[25])]
    for c in scp + pcp[0]:
        c.start()

    for c in scp:
        c.wait()
    dt_row = jnp.exp(ldt_ref[...].astype(F32).reshape(1, D)).astype(BF16).astype(F32)
    ds_row = dsk_ref[...].astype(F32).reshape(1, D)
    for j in range(4):
        sl = slice(j * LN, (j + 1) * LN)
        DT[sl, :] = jnp.broadcast_to(dt_row[:, sl], (LN, LN)).T
        DSK[sl, :] = jnp.broadcast_to(ds_row[:, sl], (LN, LN)).T

    lane = _iota((8, LN), 1)

    def kexp(J, slot):
        for s in range(8):
            rows = pl.ds(_mult(J * CB + s * 8, 8), 8)
            if s % 2 == 0:
                p16 = [par[i, pl.ds(_mult(J * CB + s * 8, 16), 16), :].astype(F32) for i in range(6)]
            p = [v[s % 2 * 8:s % 2 * 8 + 8] for v in p16]
            dt = DT[rows, :]
            zr, zi = dt * p[0], dt * p[1]
            mag = jnp.exp(zr)
            E[slot][0, s] = mag * jnp.cos(zi)
            yield
            E[slot][1, s] = mag * jnp.sin(zi)
            w = _cmul((p[4], p[5]), (dt * p[2], dt * p[3]))
            E[slot][2, s] = w[0] * (1.0 / S)
            E[slot][3, s] = w[1] * (1.0 / S)
            ZK[rows, :] = (jnp.sum(w[0], axis=1, keepdims=True) + DSK[rows, :]) * (1.0 / S)
            yield

    def kpow(J, slot):
        sa, sb = SA[slot], SB[slot]
        for s in range(8):
            def put(ref, i, v):
                n = (ref.shape[1] // 8 - 1) // 4
                for c in range(2):
                    ref[s // 4 * 2 + c, pl.ds(s % 4 * n + i, 8, stride=4 * n + 1), :] = v[c]

            p = (E[slot][0, s], E[slot][1, s])
            b = [None]
            for k in range(4):
                for i in range(2 ** k):
                    b.append(_cmul(b[i], p) if i else p)
                    put(sb, len(b) - 2, b[-1])
                    yield
                p = _csq(p)
            put(sb, 15, p)
            b = {4: b[4], 8: b[8], 12: b[12], 16: p}
            w = (E[slot][2, s], E[slot][3, s])
            pw = []
            for k in range(5):
                pw.append(p)
                p = _csq(p)
                yield
            e512, e1024 = p, _csq(p)
            for o, st, e in ((15, 4, e512), (19, 8, e1024), (21, 8, _cmul(e512, e1024))):
                for i in range(1, 16 // st + 1):
                    put(sb, o + i, _cmul(e, b[i * st]))
                    yield

            def tree(i, v, k):
                put(sa, i, v)
                yield
                for k2 in range(k):
                    yield from tree(i + 2 ** k2, _cmul(v, pw[k2]), k2)

            yield from tree(0, w, 5)

    def ksum(J, slot):
        sa, sb = SA[slot], SB[slot]
        q = _iota((24, LN), 1) >> 5
        for hm in range(16):
            h, m = divmod(hm, 8)
            o = [lax.dot_general(sb[2 * h + c, m * 97:m * 97 + 96, :],
                                 sa[2 * h + c, m * 129:m * 129 + LN, :],
                                 NT, preferred_element_type=F32) for c in range(2)]
            o = o[0] - o[1]
            KO[slot][h, m * 25:m * 25 + 24, :] = jnp.where(
                q < 2, jnp.where(q == 0, o[0:24], o[24:48]), jnp.where(q == 2, o[48:72], o[72:96]))
            yield

    def kspread(J, slot, h):
        kb = lambda i: KO[slot][h, pl.ds(i, 8, stride=25), :]
        rnd = lambda r, st: int(np.round(r / st))
        quarter = lane >> 5
        q1 = [None] + [pltpu.roll(kb(i), 32, 1) for i in range(16, 20)]
        q2 = [None] + [pltpu.roll(kb(i), 64, 1) for i in range(20, 22)]
        q3 = [None] + [pltpu.roll(kb(i), 96, 1) for i in range(22, 24)]
        k0, q23, rest = [], {}, {}
        for r in (16,) + tuple(range(R)):
            k2, k4, k8 = rnd(r, 2), rnd(r, 4), rnd(r, 8)
            if r:
                q0 = kb(r - 1)
                if r % 2 and k2:
                    q0 = jnp.where((lane & 31) < 16, q0, kb(2 * k2 - 1))
            for s in range(4):
                row = pl.ds(_mult(J * CB + h * 32 + s * 8, 8), 8)
                if r:
                    t = q0
                    if k8 and (k8, s) not in q23:
                        q23[k8, s] = jnp.where(quarter == (s + 2) % 4, q2[k8], q3[k8])
                    if k4:
                        if (k4, k8, s) not in rest:
                            rest[k4, k8, s] = jnp.where(
                                quarter == (s + 1) % 4, q1[k4], q23[k8, s]) if k8 else q1[k4]
                        t = jnp.where(quarter == s, t, rest[k4, k8, s])
                    if s or r == 16:
                        t = pltpu.roll(t, (LN - 32 * s + (r == 16)) % LN, 1)
                    if not k8:
                        t = jnp.where(lane < (64 if k4 else 32 if k2 else 16), t, k0[s])
                else:
                    t = jnp.where(lane == 0, ZK[row, :], k0[s])
                if r == 16:
                    k0.append(t)
                else:
                    _Buf(KT[slot]).st(r * CB + h * 32 + s * 8, t)
            yield

    def ld(b, k, h, n=8, stride=CB):
        return b.ld(2 * k * stride + h, n), b.ld((2 * k + 1) * stride + h, n)

    def st(b, k, h, v, stride=CB):
        b.st(2 * k * stride + h, v[0])
        b.st((2 * k + 1) * stride + h, v[1])

    def mat(r):
        return pltpu.bitcast(jnp.concatenate(ld(_Buf(mm), r, 0, 64, 64), axis=1), BF16)

    def kfwd(i, slot):
        g = _Buf(GK, i * 2 * R * CB, 2 * R * CB)
        for r in range(R):
            t = lax.dot_general(_Buf(KT[slot]).ld(r * CB, CB), mat(r), NN, preferred_element_type=F32)
            st(g, r, 0, (t[:, :LN], t[:, LN:]))
            yield

    def kfft(i):
        kf = _Buf(KF, i * CB, 2 * R * D - D + CB)
        for h in range(0, CB, 8):
            t = []
            for r0 in range(4):
                y = _radix4(*[ld(_Buf(GK, i * 2 * R * CB), r, h) for r in range(r0, R, 4)], -1)
                t.append([_twiddle(y[g0], r0 * g0, -1) for g0 in range(4)])
                yield
            for g0 in range(4):
                y = _radix4(t[0][g0], t[1][g0], t[2][g0], t[3][g0], -1)
                for g1 in range(4):
                    st(kf, 4 * g0 + g1, h, y[g1], D)
                yield

    iow = io.bitcast(U32)

    def xin(j):
        x = _Buf(X, j * LN)
        for rho in range(8):
            t = iow[j, pl.ds(rho, LN, stride=8), :].T
            x.st(2 * rho * D, pltpu.bitcast(t << 16, F32))
            x.st((2 * rho + 1) * D, pltpu.bitcast(t & np.uint32(0xFFFF0000), F32))
            yield

    def wprep(j):
        pr, pc = _iota((LN, LN), 0), _iota((LN, LN), 1)
        perm = jnp.where(pc == (pr & 7) * DH + (pr >> 3), 1.0, 0.0).astype(BF16)
        for c in range(3):
            t = lax.dot_general(perm, wraw[(c + 1) % 3 * 4 + j], NT, preferred_element_type=F32)
            if c == 2:
                t = t * (DH ** -0.5)
            for k in range(4):
                _Buf(W).st(k * WS + (3 * j + c) * LN // 2,
                           pltpu.bitcast(t[:, k * LN:(k + 1) * LN].astype(BF16), F32))
            yield
        t = jnp.dot(perm, woraw[j * LN:(j + 1) * LN, :], preferred_element_type=F32)
        _Buf(W).st(j * WS + 3 * D // 2, pltpu.bitcast(t.T.astype(BF16), F32))
        yield

    def kstep(J, ref):
        @block("kgen")
        def _():
            slot, m, v = ref % 2, [], []
            if 0 <= ref < NCB:
                m.append(ksum(J, slot))
            if 0 <= ref - 2:
                m.append(kfwd(J - 2, slot))
            v = [(g, 16 * KW) for g in m]
            if 0 <= ref - 1 < NCB:
                v.append((_chain(*[kspread(J - 1, 1 - slot, h) for h in range(2)]), 34))
            if 0 <= ref + 1 < NCB:
                v.append((kpow(J + 1, 1 - slot), 8 * 60))
            if ref + 2 < NCB:
                v.append((kexp(J + 2, slot), 16))
            if ref >= NCB:
                js = (2 * (ref - NCB), 2 * (ref - NCB) + 1)
                v += [(_chain(*map(xin, js)), 16), (_chain(*map(wprep, js)), 8)]
            _weave(*v)

    for J in range(-2, 2):
        if J % 2 == 0:
            with _scope("pwait"):
                for c in pcp[J // 2 + 1]:
                    c.wait()
            for c in pcp[1] if J else [mcp] + xcp + wcp + [wocp]:
                c.start()
        kstep(J, J)
    with _scope("mwait"):
        mcp.wait()
    _loop(1, 3, lambda k: (kstep(2 * k, 2), kstep(2 * k + 1, 3)), 1)
    for J in range(6, 10):
        if J == NCB:
            with _scope("xwait"):
                for c in xcp + wcp + [wocp]:
                    c.wait()
        kstep(J, J)

    def colsum(f, step):
        acc = [f(c * 8) for c in range(4)]
        for i in range(4, D // 8):
            acc[i % 4] = acc[i % 4] + f(i * 8)
            if i % step == step - 1:
                yield
        s = jnp.sum((acc[0] + acc[1]) + (acc[2] + acc[3]), axis=0, keepdims=True)
        return jnp.broadcast_to(s * (1.0 / D), (8, LN))

    def ln_stats(ref, base):
        x = _Buf(ref, base + zero[0], D)
        m = yield from colsum(lambda c: x.ld(c, 8), 32)
        x = _Buf(ref, base + zero[1], D)
        v = yield from colsum(lambda c: jnp.square(x.ld(c, 8) - m), 8)
        return _Buf(ref, base + zero[2], D), m, lax.rsqrt(v + EPS)

    def ln(ref, base, out, r):
        x, m, rs = yield from ln_stats(ref, base)
        for c in range(0, D, 16):
            t = [(x.ld(c + k, 8) - m) * rs for k in (0, 8)]
            _Buf(out, r * D).st(c, jnp.concatenate(t, axis=0))
            if c % 64 == 48:
                yield

    def ln1(r):
        return ln(X, r * D, XN, r)

    def ln2(r):
        return ln(Z[r], 0, U, r)

    def wdot(c, n, rhs):
        lhs = jnp.concatenate(
            [pltpu.bitcast(W[t * WS + c // 2:t * WS + (c + n) // 2, :], BF16)
             for t in range(4)], axis=1)
        return jnp.dot(lhs, rhs.ld(0, D), preferred_element_type=F32)

    def qkvproj(j, r):
        b, i = _Buf(KVQ[j % 2][r % 2]), r // 2
        for c in range(3):
            t = wdot((3 * j + c) * LN, LN, _Buf(XN, r * D + zero[(r + c) % R], D))
            if c == 2:
                b.st((32 + i) * TS, t)
            else:
                b.st((16 * c + 8 + i) * TS, t)
                if i:
                    b.st((16 * c + i) * TS, pltpu.roll(t, 1, 1))
            yield

    def core(j, r):
        b, i = _Buf(KVQ[j % 2][r % 2], zero[r], 40 * TS), r // 2
        lg = [None] * WIN
        for dh in range(DH):
            q = b.ld((32 + i) * TS + dh * 8, 8)
            for w in range(WIN):
                t = q * b.ld((8 + i - w) * TS + dh * 8, 8)
                lg[w] = t if dh == 0 else lg[w] + t
            if dh % 2:
                yield
        for w in range(i + 1, WIN):
            lg[w] = jnp.where(lane > 0, lg[w], -1e9)
        mx = _tree(jnp.maximum, lg)
        e = [jnp.exp(v - mx) for v in lg]
        inv = 1.0 / _tree(jnp.add, e)
        e = [v * inv for v in e]
        yield
        yield
        for dh in range(0, DH, 2):
            oo = []
            for k in (dh, dh + 1):
                acc = None
                for w in range(WIN):
                    t = e[w] * b.ld((24 + i - w) * TS + k * 8, 8)
                    acc = t if acc is None else acc + t
                oo.append(acc)
            _Buf(O, r * D + j * LN).st(dh * 8, jnp.concatenate(oo, axis=0))
            yield

    def oproj(r):
        for c in range(0, D, DO):
            Z[r][c:c + DO, :] = X[r * D + c:r * D + c + DO, :] + wdot(
                3 * D + c, DO, _Buf(O, r * D + zero[(r + c // DO) % R], D))
            yield

    def cmxu(fi, ii, slot, rs):
        if fi is not None:
            u_ = _Buf(U, fi * CB, R * D - D + CB)
        if ii is not None:
            x = _Buf(X, ii * CB, R * D - D + CB)
        for r in rs:
            if fi is not None:
                t = lax.dot_general(u_.ld(r * D, CB), mat(r), NN, preferred_element_type=F32)
                st(_Buf(G[slot]), r, 0, (t[:, :LN], t[:, LN:]))
                yield
            if ii is not None:
                lhs = jnp.concatenate(ld(_Buf(HH[slot]), r, 0, CB), axis=1)
                t = lax.dot_general(lhs, mat(r), NT, preferred_element_type=F32)
                x.st(r * D, _Buf(Z[r], ii * CB, CB).ld(0, CB) + t)
                yield

    def cmid(i, slot):
        g, hh = _Buf(G[slot], zero[0], 2 * R * CB), _Buf(HH[slot])
        kf = _Buf(KF, i * CB, 2 * R * D - D + CB)

        for h in range(0, CB, 8):
            t, v = [], []
            for r0 in range(4):
                y = _radix4(*[ld(g, r, h) for r in range(r0, R, 4)], -1)
                t.append([_twiddle(y[g0], r0 * g0, -1) for g0 in range(4)])
                yield
            yield
            for g0 in range(4):
                y = _radix4(t[0][g0], t[1][g0], t[2][g0], t[3][g0], -1)
                yield
                y = [_cmul(y[g1], ld(kf, 4 * g0 + g1, h, 8, D)) for g1 in range(4)]
                yield
                y = _radix4(*y, 1)
                v.append([_twiddle(y[r0], r0 * g0, 1) for r0 in range(4)])
                yield
                if g0 != 1:
                    yield
            for r0 in range(4):
                y = _radix4(*[v[g0][r0] for g0 in range(4)], 1)
                for r1 in range(4):
                    st(hh, r0 + 4 * r1, h, y[r1])
                yield

    def ocopy(j):
        n = S // NO
        return [pltpu.make_async_copy(
            io.at[j, pl.ds(k * n, n), :],
            out_hbm.at[pl.ds(k * n, n), pl.ds(_mult(j * LN, LN), LN)], sems.at[NO * j + k])
            for k in range(NO)]

    def xout(j):
        x = _Buf(X, j * LN, R * D - D + LN)
        for rho in range(8):
            lo, hi = (pltpu.bitcast(x.ld(r * D, LN).astype(BF16).astype(F32), U32)
                      for r in (2 * rho, 2 * rho + 1))
            iow[j, pl.ds(rho, LN, stride=8), :] = ((lo >> 16) | hi).T
            yield
        for c in ocopy(j):
            c.start()

    order = list(range(0, R, 2)) + list(range(1, R, 2))
    NCORE, NLN1, NLN2 = 18, 18, 18

    def layer(l, carry):
        def spectra(b):
            ids = range(sum(KB[:b]), sum(KB[:b + 1]))
            return _chain(*map(kfft, ids)), 64 * len(ids) + 0.01

        @block("ph1")
        def _():
            _weave((_chain(*[qkvproj(0, r) for r in order]), 3 * R),
                   (_chain(*map(ln1, order[1:])), NLN1 * (R + L1)), spectra(0))

        for b, (j, lo, hi) in enumerate(((1, 0, R), (2, 0, R), (3, 0, R // 2), (3, R // 2, R))):
            @block("ph2")
            def _():
                early = _chain(*[core(3, r) for r in order[:LO if lo else 0]])
                kf, nk = spectra(1 + b)
                nk = int(nk) // (hi - lo)
                for r in order[lo:hi]:
                    _weave((qkvproj(j, r), 3), (core(j - 1, r), NCORE),
                           (_take(early, -(-LO * NCORE // 8)), LO * NCORE / 8),
                           (_take(kf, nk), nk + 0.01))

        for b, (prev, cur) in enumerate(zip(B3, B3[1:])):
            @block("ph3")
            def _():
                w, c, n = (order[u:v] for u, v in zip(prev, cur))
                _weave((_chain(*map(oproj, w)), len(w) * D // DO),
                       (_chain(*[core(3, r) for r in c]), len(c) * NCORE + 0.01),
                       (_chain(*map(ln2, n)), len(n) * NLN2 + 0.01), spectra(5 + b))

        def cstep(i, slot, f=True, m=True, v=True):
            @block("conv")
            def _():
                _weave((cmxu(i + 1 if f else None, i - 1 if v else None, 1 - slot, order), R * (f + v)),
                       *([(cmid(i, slot), 3 * CB)] if m else []),
                       *[(ln2(r), 2 * NLN2) for r in order[B3[-1][2]:] if f and not m])

        cstep(-1, 1, m=False, v=False)
        cstep(0, 0, v=False)

        def cpair(k):
            cstep(2 * k + 1, 1)
            cstep(2 * k + 2, 0)
            pl.when(l == 1)(lambda: _weave((xout(k), 1)))

        _loop(0, NCB // 2 - 1, cpair, 1)
        cstep(NCB - 1, 1, f=False)

        @pl.when(l == 0)
        def _():
            _weave((_chain(cmxu(None, NCB - 1, 1, order), ln1(0)), 1))

        @pl.when(l == 1)
        def _():
            m = cmxu(None, NCB - 1, 1, range(R))
            _weave((_take(m, 4), 1))
            _weave((xout(3), 8), (m, R))

        return carry

    _weave((ln1(0), 1))
    with _scope("layers"):
        lax.fori_loop(0, 2, layer, 0)

    with _scope("owait"):
        for j in range(4):
            for c in ocopy(j):
                c.wait()


@jax.jit
def pallas_interleave_layers__sliding_local_dilated__ssm_conv_s4__prompt_kernel(
    A_x: jax.Array,
    A_wqkv: jax.Array,
    A_wo: jax.Array,
    B_u: jax.Array,
    B_A_re: jax.Array,
    B_A_im: jax.Array,
    B_B_re: jax.Array,
    B_B_im: jax.Array,
    B_C_re: jax.Array,
    B_C_im: jax.Array,
    B_log_dt: jax.Array,
    B_Dskip: jax.Array,
):
    del B_u
    hbm = pl.BlockSpec(memory_space=pl.ANY)
    V = pltpu.VMEM
    out = pl.pallas_call(
        _kernel,
        out_shape=jax.ShapeDtypeStruct((S, D), BF16),
        in_specs=[hbm] * 12,
        out_specs=hbm,
        scratch_shapes=[
            V((D,), BF16), V((D,), BF16),
            V((4, S, LN), BF16),
            V((12, D, LN), BF16),
            V((D, D), BF16),
            V((6, D, LN), BF16),
            V((R * LN, LN), U32),
            V((R * D, LN), F32),
            V((2 * R * D, LN), F32),
            V((D, LN), F32),
            V((R * D, LN), BF16),
            V((R * D, LN), F32),
            V((4 * WS, LN), F32),
            [V((D, LN), F32)] * R,
            [[V((40 * TS, LN), F32)] * 2] * 2,
            V((R * D, LN), BF16),
            [V((2 * R * CB, LN), F32)] * 2,
            [V((2 * R * CB, LN), F32)] * 2,
            [V((R * CB, LN), F32)] * 2,
            V((2 * R * D, LN), F32),
            [V((4, 8, 8, LN), F32)] * 2,
            V((D, LN), F32),
            V((D, LN), F32),
            [V((4, 8 * 129, LN), F32)] * 2,
            [V((4, 8 * 97, LN), F32)] * 2,
            [V((2, 8 * 25, LN), F32)] * 2,
            pltpu.SMEM((R,), jnp.int32),
            pltpu.SemaphoreType.DMA((32,)),
        ],
        compiler_params=pltpu.CompilerParams(vmem_limit_bytes=100 * 1024 * 1024, flags=FLAGS),
    )(A_x.reshape(S, D), A_wqkv, A_wo, B_A_re, B_A_im, B_B_re, B_B_im, B_C_re, B_C_im,
      B_log_dt, B_Dskip, _M)
    return out.reshape(1, S, D)
```

```python
import contextlib
import numpy as np
import jax
import jax.numpy as jnp
from jax import lax
import jax.experimental.pallas as pl
import jax.experimental.pallas.tpu as pltpu

S, D, DH, WIN = 2048, 512, 16, 8
R = 16
LN = 128
CB = 64
NCB = D // CB
EPS = 1e-5
F32, BF16, U32 = jnp.float32, jnp.bfloat16, jnp.uint32
NN, NT = (((1,), (0,)), ((), ())), (((1,), (1,)), ((), ()))


def _dft_matrices():
    lam = np.arange(LN, dtype=np.float64)[None, :, None]
    r = np.arange(R, dtype=np.float64)[:, None, None]
    f = np.arange(LN, dtype=np.float64)[None, None, :]
    th = 2.0 * np.pi * (f + 0.5) * (R * lam + r) / (2 * S) + 2.0 * np.pi * 2 / 16 * (r % 4 == 2)
    m = np.stack([np.cos(th), -np.sin(th)], axis=1).astype(BF16).view(np.uint16).astype(np.uint32)
    return (m[:, :, 0::2] | (m[:, :, 1::2] << 16)).reshape(R * LN, LN)


_M = _dft_matrices()


SCOPES = False


def _scope(name):
    return jax.named_scope(name) if SCOPES else contextlib.nullcontext()


FLAGS = None
SKIP = NOB = ''
LO, NO = 6, 1
KW = 1
WP, XP = (8, 8, 9, 9), (7, 7, 8, 9)
KB, L1 = (0, 3, 3, 1, 0, 1, 0, 0, 0), 1
B3 = ((0, 6, 0), (5, 11, 0), (10, 16, 5), (14, 16, 10), (16, 16, 14))
DO = 256
TS, WS = LN, 2 * D


class _Buf:
    def __init__(self, ref, base=0, size=None):
        if isinstance(base, int):
            self.ref, self.base = ref, base
        else:
            self.ref, self.base = ref.at[pl.ds(pl.multiple_of(base, 16), size), :], 0

    def ld(self, row, n):
        return self.ref[self.base + row:self.base + row + n, :]

    def st(self, row, v):
        self.ref[self.base + row:self.base + row + v.shape[0], :] = v.astype(self.ref.dtype)


def _weave(*stages):
    live = [[g, n, 0] for g, n in stages]
    while live:
        st = min(live, key=lambda t: t[2] / t[1])
        try:
            next(st[0])
            st[2] += 1
        except StopIteration:
            live.remove(st)


def _chain(*gens):
    for g in gens:
        yield from g


def _take(g, n):
    for _, _ in zip(range(n), g):
        yield


def _tree(op, v):
    while len(v) > 1:
        v = [op(v[i], v[i + 1]) for i in range(0, len(v), 2)]
    return v[0]


def _mult(i, n):
    return i if isinstance(i, int) else pl.multiple_of(i, n)


def _loop(lo, hi, body, unroll, force=False):
    n = hi - lo
    assert n % unroll == 0
    if n == unroll and not force:
        for i in range(lo, hi):
            body(i)
        return

    def outer(k, carry):
        for u in range(unroll):
            body(lo + k * unroll + u)
        return carry

    lax.fori_loop(0, n // unroll, outer, 0)


def _iota(shape, dim):
    return lax.broadcasted_iota(jnp.int32, shape, dim)


def _cmul(a, b):
    return (a[0] * b[0] - a[1] * b[1], a[0] * b[1] + a[1] * b[0])


def _csq(a):
    t = a[0] * a[1]
    return (a[0] * a[0] - a[1] * a[1], t + t)


def _radix4(a, b, c, d, sign):
    s0 = (a[0] + c[0], a[1] + c[1])
    d0 = (a[0] - c[0], a[1] - c[1])
    s1 = (b[0] + d[0], b[1] + d[1])
    d1 = (b[0] - d[0], b[1] - d[1])
    y0 = (s0[0] + s1[0], s0[1] + s1[1])
    y2 = (s0[0] - s1[0], s0[1] - s1[1])
    p = (d0[0] - d1[1], d0[1] + d1[0])
    m = (d0[0] + d1[1], d0[1] - d1[0])
    return (y0, p, y2, m) if sign > 0 else (y0, m, y2, p)


def _twiddle(a, k, sign):
    k = sign * k % 16
    c, s = float(np.cos(2 * np.pi * k / 16)), float(np.sin(2 * np.pi * k / 16))
    if k % 4 == 0:
        return (a, (-a[1], a[0]), (-a[0], -a[1]), (a[1], -a[0]))[k // 4]
    if k % 8 == 2:
        return ((a[0] - a[1]) * c, (a[0] + a[1]) * c)
    if k % 8 == 6:
        return ((a[0] + a[1]) * c, (a[1] - a[0]) * c)
    return (a[0] * c - a[1] * s, a[0] * s + a[1] * c)


_ROW, _COL = (0, 0, 2, 0), (0, 0, 2, 0)
_TW = [[r0 * g0 - _ROW[r0] - _COL[g0] for g0 in range(4)] for r0 in range(4)]


def _kernel(x_hbm, wqkv_hbm, wo_hbm, are_hbm, aim_hbm, bre_hbm, bim_hbm, cre_hbm, cim_hbm,
            ldt_hbm, dsk_hbm, m_hbm, out_hbm, ldt_ref, dsk_ref,
            io, wraw, woraw, par, mm, X, KF, DSK, XN, U, W, Z, KVQ, O, G, HH,
            KT, GK, E, DT, ZK, SA, SB, KO, zero, sems):
    for k in range(R):
        zero[k] = 0

    def block(name):
        def deco(f):
            if SKIP and name in SKIP:
                return
            with _scope(name):
                f() if name in NOB else pl.when(zero[0] == 0)(f)
        return deco

    def opaque(r):
        return zero[r] if isinstance(r, int) else 0

    pcp = [[pltpu.make_async_copy(h.at[rows, :], par.at[i, rows, :], sems.at[o + i])
            for i, h in enumerate((are_hbm, aim_hbm, bre_hbm, bim_hbm, cre_hbm, cim_hbm))]
           for o, rows in ((0, pl.ds(0, 2 * CB)), (26, pl.ds(2 * CB, D - 2 * CB)))]
    mcp = pltpu.make_async_copy(m_hbm, mm, sems.at[6])
    xcp = [pltpu.make_async_copy(x_hbm.at[:, pl.ds(j * LN, LN)], io.at[j], sems.at[7 + j])
           for j in range(4)]
    wocp = [pltpu.make_async_copy(wo_hbm.at[pl.ds(j * LN, LN), :], woraw.at[pl.ds(j * LN, LN), :],
                                  sems.at[32 + j]) for j in range(4)]
    wcp = [pltpu.make_async_copy(wqkv_hbm.at[:, pl.ds(j * LN, LN)], wraw.at[j], sems.at[12 + j])
           for j in range(12)]
    scp = [pltpu.make_async_copy(ldt_hbm, ldt_ref, sems.at[24]),
           pltpu.make_async_copy(dsk_hbm, dsk_ref, sems.at[25])]
    for c in scp + pcp[0]:
        c.start()

    for c in scp:
        c.wait()
    dt_row = jnp.exp(ldt_ref[...].astype(F32).reshape(1, D)).astype(BF16).astype(F32)
    ds_row = dsk_ref[...].astype(F32).reshape(1, D)
    for j in range(4):
        sl = slice(j * LN, (j + 1) * LN)
        DT[sl, :] = jnp.broadcast_to(dt_row[:, sl], (LN, LN)).T
        DSK[sl, :] = jnp.broadcast_to(ds_row[:, sl], (LN, LN)).T

    lane = _iota((8, LN), 1)

    def kexp(J, slot):
        for s in range(8):
            rows = pl.ds(_mult(J * CB + s * 8, 8), 8)
            if s % 2 == 0:
                p16 = [par[i, pl.ds(_mult(J * CB + s * 8, 16), 16), :].astype(F32) for i in range(6)]
            p = [v[s % 2 * 8:s % 2 * 8 + 8] for v in p16]
            dt = DT[rows, :]
            zr, zi = dt * p[0], dt * p[1]
            mag = jnp.exp(zr)
            E[slot][0, s] = mag * jnp.cos(zi)
            yield
            E[slot][1, s] = mag * jnp.sin(zi)
            w = _cmul((p[4], p[5]), (dt * p[2], dt * p[3]))
            E[slot][2, s] = w[0] * (1.0 / S)
            E[slot][3, s] = w[1] * (1.0 / S)
            ZK[rows, :] = (jnp.sum(w[0], axis=1, keepdims=True) + DSK[rows, :]) * (1.0 / S)
            yield

    def kpow(J, slot):
        sa, sb = SA[slot], SB[slot]
        for s in range(8):
            def put(ref, i, v):
                n = (ref.shape[1] // 8 - 1) // 4
                for c in range(2):
                    ref[s // 4 * 2 + c, pl.ds(s % 4 * n + i, 8, stride=4 * n + 1), :] = v[c]

            p = (E[slot][0, s], E[slot][1, s])
            b = [None]
            for k in range(4):
                for i in range(2 ** k):
                    b.append(_cmul(b[i], p) if i else p)
                    put(sb, len(b) - 2, b[-1])
                    yield
                p = _csq(p)
            put(sb, 15, p)
            b = {4: b[4], 8: b[8], 12: b[12], 16: p}
            w = (E[slot][2, s], E[slot][3, s])
            pw = []
            for k in range(5):
                pw.append(p)
                p = _csq(p)
                yield
            e512, e1024 = p, _csq(p)
            for o, st, e in ((15, 4, e512), (19, 8, e1024), (21, 8, _cmul(e512, e1024))):
                for i in range(1, 16 // st + 1):
                    put(sb, o + i, _cmul(e, b[i * st]))
                    yield

            def tree(i, v, k):
                put(sa, i, v)
                yield
                for k2 in range(k):
                    yield from tree(i + 2 ** k2, _cmul(v, pw[k2]), k2)

            yield from tree(0, w, 5)

    def ksum(J, slot):
        sa, sb = SA[slot], SB[slot]
        q = _iota((24, LN), 1) >> 5
        for hm in range(16):
            h, m = divmod(hm, 8)
            o = [lax.dot_general(sb[2 * h + c, m * 97:m * 97 + 96, :],
                                 sa[2 * h + c, m * 129:m * 129 + LN, :],
                                 NT, preferred_element_type=F32) for c in range(2)]
            o = o[0] - o[1]
            KO[slot][h, m * 25:m * 25 + 24, :] = jnp.where(
                q < 2, jnp.where(q == 0, o[0:24], o[24:48]), jnp.where(q == 2, o[48:72], o[72:96]))
            yield

    def kspread(J, slot, h):
        kb = lambda i: KO[slot][h, pl.ds(i, 8, stride=25), :]
        rnd = lambda r, st: int(np.round(r / st))
        quarter = lane >> 5
        q1 = [None] + [pltpu.roll(kb(i), 32, 1) for i in range(16, 20)]
        q2 = [None] + [pltpu.roll(kb(i), 64, 1) for i in range(20, 22)]
        q3 = [None] + [pltpu.roll(kb(i), 96, 1) for i in range(22, 24)]
        k0, q23, rest = [], {}, {}
        for r in (16,) + tuple(range(R)):
            k2, k4, k8 = rnd(r, 2), rnd(r, 4), rnd(r, 8)
            if r:
                q0 = kb(r - 1)
                if r % 2 and k2:
                    q0 = jnp.where((lane & 31) < 16, q0, kb(2 * k2 - 1))
            for s in range(4):
                row = pl.ds(_mult(J * CB + h * 32 + s * 8, 8), 8)
                if r:
                    t = q0
                    if k8 and (k8, s) not in q23:
                        q23[k8, s] = jnp.where(quarter == (s + 2) % 4, q2[k8], q3[k8])
                    if k4:
                        if (k4, k8, s) not in rest:
                            rest[k4, k8, s] = jnp.where(
                                quarter == (s + 1) % 4, q1[k4], q23[k8, s]) if k8 else q1[k4]
                        t = jnp.where(quarter == s, t, rest[k4, k8, s])
                    if s or r == 16:
                        t = pltpu.roll(t, (LN - 32 * s + (r == 16)) % LN, 1)
                    if not k8:
                        t = jnp.where(lane < (64 if k4 else 32 if k2 else 16), t, k0[s])
                else:
                    t = jnp.where(lane == 0, ZK[row, :], k0[s])
                if r == 16:
                    k0.append(t)
                else:
                    _Buf(KT[slot]).st(r * CB + h * 32 + s * 8, t)
            yield

    def ld(b, k, h, n=8, stride=CB):
        return b.ld(2 * k * stride + h, n), b.ld((2 * k + 1) * stride + h, n)

    def st(b, k, h, v, stride=CB):
        b.st(2 * k * stride + h, v[0])
        b.st((2 * k + 1) * stride + h, v[1])

    def mat(r):
        return pltpu.bitcast(jnp.concatenate(ld(_Buf(mm), r, 0, 64, 64), axis=1), BF16)

    def kfwd(i, slot):
        g = _Buf(GK, i * 2 * R * CB, 2 * R * CB)
        for r in range(R):
            t = lax.dot_general(_Buf(KT[slot]).ld(r * CB, CB), mat(r), NN, preferred_element_type=F32)
            st(g, r, 0, (t[:, :LN], t[:, LN:]))
            yield

    def kfft(i):
        kf = _Buf(KF, i * CB, 2 * R * D - D + CB)
        for h in range(0, CB, 8):
            t = []
            for r0 in range(4):
                y = _radix4(*[ld(_Buf(GK, i * 2 * R * CB), r, h) for r in range(r0, R, 4)], -1)
                t.append([_twiddle(y[g0], _TW[r0][g0], -1) for g0 in range(4)])
                yield
            for g0 in range(4):
                y = _radix4(t[0][g0], t[1][g0], t[2][g0], t[3][g0], -1)
                for g1 in range(4):
                    st(kf, 4 * g0 + g1, h, _twiddle(y[g1], _COL[g0], -1), D)
                yield

    iow = io.bitcast(U32)

    def xin(j):
        x = _Buf(X, j * LN)
        for rho in range(8):
            t = iow[j, pl.ds(rho, LN, stride=8), :].T
            x.st(2 * rho * D, pltpu.bitcast(t << 16, F32))
            x.st((2 * rho + 1) * D, pltpu.bitcast(t & np.uint32(0xFFFF0000), F32))
            yield

    def wprep(j):
        pr, pc = _iota((LN, LN), 0), _iota((LN, LN), 1)
        perm = jnp.where(pc == (pr & 7) * DH + (pr >> 3), 1.0, 0.0).astype(BF16)
        for c in range(3):
            t = lax.dot_general(perm, wraw[(c + 1) % 3 * 4 + j], NT, preferred_element_type=F32)
            if c == 2:
                t = t * (DH ** -0.5)
            for k in range(4):
                _Buf(W).st(k * WS + (3 * j + c) * LN // 2,
                           pltpu.bitcast(t[:, k * LN:(k + 1) * LN].astype(BF16), F32))
            yield
        t = jnp.dot(perm, woraw[j * LN:(j + 1) * LN, :], preferred_element_type=F32)
        _Buf(W).st(j * WS + 3 * D // 2, pltpu.bitcast(t.T.astype(BF16), F32))
        yield

    def kstep(J, ref):
        @block("kgen")
        def _():
            slot, m, v = ref % 2, [], []
            if 0 <= ref < NCB:
                m.append(ksum(J, slot))
            if 0 <= ref - 2:
                m.append(kfwd(J - 2, slot))
            v = [(g, 16 * KW) for g in m]
            if 0 <= ref - 1 < NCB:
                v.append((_chain(*[kspread(J - 1, 1 - slot, h) for h in range(2)]), 34))
            if 0 <= ref + 1 < NCB:
                v.append((kpow(J + 1, 1 - slot), 8 * 60))
            if ref + 2 < NCB:
                v.append((kexp(J + 2, slot), 16))
            for gen, steps, n in ((xin, XP, 8), (wprep, WP, 4)):
                js = [j for j in range(4) if steps[j] == ref]
                v.append((_chain(*map(gen, js)), n * len(js) + 0.01))
            _weave(*v)

    def wcopies(J):
        return [c for j in range(4) if WP[j] in J for c in wcp[j::4] + [wocp[j]]]

    for J in range(-2, 10):
        with _scope("wait"):
            for c in ({-2: pcp[0], 0: pcp[1], 2: [mcp]}.get(J, []) + wcopies((J,))
                      + [xcp[j] for j in range(4) if XP[j] == J]):
                c.wait()
        for c in {-2: pcp[1], -1: wcopies((1,)), 0: [mcp], 2: xcp + wcopies(range(6, 10))}.get(J, []):
            c.start()
        if J == 2:
            _loop(1, 3, lambda k: (kstep(2 * k, 2), kstep(2 * k + 1, 3)), 1)
        elif not 2 <= J < 6:
            kstep(J, J)

    def colsum(f, step):
        acc = [f(c * 8) for c in range(4)]
        for i in range(4, D // 8):
            acc[i % 4] = acc[i % 4] + f(i * 8)
            if i % step == step - 1:
                yield
        s = jnp.sum((acc[0] + acc[1]) + (acc[2] + acc[3]), axis=0, keepdims=True)
        return jnp.broadcast_to(s * (1.0 / D), (8, LN))

    def ln_stats(ref, base):
        x = _Buf(ref, base + zero[0], D)
        m = yield from colsum(lambda c: x.ld(c, 8), 32)
        x = _Buf(ref, base + zero[1], D)
        v = yield from colsum(lambda c: jnp.square(x.ld(c, 8) - m), 8)
        return _Buf(ref, base + zero[2], D), m, lax.rsqrt(v + EPS)

    def ln(ref, base, out, r):
        x, m, rs = yield from ln_stats(ref, base)
        for c in range(0, D, 16):
            t = [(x.ld(c + k, 8) - m) * rs for k in (0, 8)]
            _Buf(out, r * D).st(c, jnp.concatenate(t, axis=0))
            if c % 64 == 48:
                yield

    def ln1(r):
        return ln(X, r * D, XN, r)

    def ln2(r):
        return ln(Z[r], 0, U, r)

    def wdot(c, n, rhs):
        lhs = jnp.concatenate(
            [pltpu.bitcast(W[t * WS + c // 2:t * WS + (c + n) // 2, :], BF16)
             for t in range(4)], axis=1)
        return jnp.dot(lhs, rhs.ld(0, D), preferred_element_type=F32)

    def qkvproj(j, r):
        b, i = _Buf(KVQ[j % 2][r % 2]), r // 2
        for c in range(3):
            t = wdot((3 * j + c) * LN, LN, _Buf(XN, r * D + zero[(r + c) % R], D))
            if c == 2:
                b.st((32 + i) * TS, t)
            else:
                b.st((16 * c + 8 + i) * TS, t)
                if i:
                    b.st((16 * c + i) * TS, pltpu.roll(t, 1, 1))
            yield

    def core(j, r):
        b, i = _Buf(KVQ[j % 2][r % 2], zero[r], 40 * TS), r // 2
        lg = [None] * WIN
        for dh in range(DH):
            q = b.ld((32 + i) * TS + dh * 8, 8)
            for w in range(WIN):
                t = q * b.ld((8 + i - w) * TS + dh * 8, 8)
                lg[w] = t if dh == 0 else lg[w] + t
            if dh % 2:
                yield
        for w in range(i + 1, WIN):
            lg[w] = jnp.where(lane > 0, lg[w], -1e9)
        mx = _tree(jnp.maximum, lg)
        e = [jnp.exp(v - mx) for v in lg]
        inv = 1.0 / _tree(jnp.add, e)
        e = [v * inv for v in e]
        yield
        yield
        for dh in range(0, DH, 2):
            oo = []
            for k in (dh, dh + 1):
                acc = None
                for w in range(WIN):
                    t = e[w] * b.ld((24 + i - w) * TS + k * 8, 8)
                    acc = t if acc is None else acc + t
                oo.append(acc)
            _Buf(O, r * D + j * LN).st(dh * 8, jnp.concatenate(oo, axis=0))
            yield

    def oproj(r):
        for c in range(0, D, DO):
            Z[r][c:c + DO, :] = X[r * D + c:r * D + c + DO, :] + wdot(
                3 * D + c, DO, _Buf(O, r * D + zero[(r + c // DO) % R], D))
            yield

    def cmxu(fi, ii, slot, rs):
        if fi is not None:
            u_ = _Buf(U, fi * CB, R * D - D + CB)
        if ii is not None:
            x = _Buf(X, ii * CB, R * D - D + CB)
        for r in rs:
            if fi is not None:
                t = lax.dot_general(u_.ld(r * D, CB), mat(r), NN, preferred_element_type=F32)
                st(_Buf(G[slot]), r, 0, (t[:, :LN], t[:, LN:]))
                yield
            if ii is not None:
                lhs = jnp.concatenate(ld(_Buf(HH[slot]), r, 0, CB), axis=1)
                t = lax.dot_general(lhs, mat(r), NT, preferred_element_type=F32)
                x.st(r * D, _Buf(Z[r], ii * CB, CB).ld(0, CB) + t)
                yield

    def cmid(i, slot):
        g, hh = _Buf(G[slot], zero[0], 2 * R * CB), _Buf(HH[slot])
        kf = _Buf(KF, i * CB, 2 * R * D - D + CB)

        for h in range(0, CB, 8):
            t, v = [], []
            for r0 in range(4):
                y = _radix4(*[ld(g, r, h) for r in range(r0, R, 4)], -1)
                t.append([_twiddle(y[g0], _TW[r0][g0], -1) for g0 in range(4)])
                yield
            yield
            for g0 in range(4):
                y = _radix4(t[0][g0], t[1][g0], t[2][g0], t[3][g0], -1)
                yield
                y = [_cmul(y[g1], ld(kf, 4 * g0 + g1, h, 8, D)) for g1 in range(4)]
                yield
                y = _radix4(*y, 1)
                v.append([_twiddle(y[r0], _TW[r0][g0], 1) for r0 in range(4)])
                yield
                if g0 != 1:
                    yield
            for r0 in range(4):
                y = _radix4(*[v[g0][r0] for g0 in range(4)], 1)
                for r1 in range(4):
                    st(hh, r0 + 4 * r1, h, y[r1])
                yield

    def ocopy(j):
        n = S // NO
        return [pltpu.make_async_copy(
            io.at[j, pl.ds(k * n, n), :],
            out_hbm.at[pl.ds(k * n, n), pl.ds(_mult(j * LN, LN), LN)], sems.at[NO * j + k])
            for k in range(NO)]

    def xout(j):
        x = _Buf(X, j * LN, R * D - D + LN)
        for rho in range(8):
            lo, hi = (pltpu.bitcast(x.ld(r * D, LN).astype(BF16).astype(F32), U32)
                      for r in (2 * rho, 2 * rho + 1))
            iow[j, pl.ds(rho, LN, stride=8), :] = ((lo >> 16) | hi).T
            yield
        for c in ocopy(j):
            c.start()

    order = list(range(0, R, 2)) + list(range(1, R, 2))
    NCORE, NLN1, NLN2 = 18, 18, 18

    def layer(l, carry):
        def spectra(b):
            ids = range(sum(KB[:b]), sum(KB[:b + 1]))
            return _chain(*map(kfft, ids)), 64 * len(ids) + 0.01

        @block("ph1")
        def _():
            _weave((_chain(*[qkvproj(0, r) for r in order]), 3 * R),
                   (_chain(*map(ln1, order[1:])), NLN1 * (R + L1)), spectra(0))

        for b, (j, lo, hi) in enumerate(((1, 0, R), (2, 0, R), (3, 0, R // 2), (3, R // 2, R))):
            @block("ph2")
            def _():
                early = _chain(*[core(3, r) for r in order[:LO if lo else 0]])
                kf, nk = spectra(1 + b)
                nk = int(nk) // (hi - lo)
                for r in order[lo:hi]:
                    _weave((qkvproj(j, r), 3), (core(j - 1, r), NCORE),
                           (_take(early, -(-LO * NCORE // 8)), LO * NCORE / 8),
                           (_take(kf, nk), nk + 0.01))

        for b, (prev, cur) in enumerate(zip(B3, B3[1:])):
            @block("ph3")
            def _():
                w, c, n = (order[u:v] for u, v in zip(prev, cur))
                _weave((_chain(*map(oproj, w)), len(w) * D // DO),
                       (_chain(*[core(3, r) for r in c]), len(c) * NCORE + 0.01),
                       (_chain(*map(ln2, n)), len(n) * NLN2 + 0.01), spectra(5 + b))

        def cstep(i, slot, f=True, m=True, v=True):
            @block("conv")
            def _():
                _weave((cmxu(i + 1 if f else None, i - 1 if v else None, 1 - slot, order), R * (f + v)),
                       *([(cmid(i, slot), 3 * CB)] if m else []),
                       *[(ln2(r), 2 * NLN2) for r in order[B3[-1][2]:] if f and not m])

        cstep(-1, 1, m=False, v=False)
        cstep(0, 0, v=False)

        def cpair(k):
            cstep(2 * k + 1, 1)
            cstep(2 * k + 2, 0)
            pl.when(l == 1)(lambda: _weave((xout(k), 1)))

        _loop(0, NCB // 2 - 1, cpair, 1)
        cstep(NCB - 1, 1, f=False)

        @pl.when(l == 0)
        def _():
            _weave((_chain(cmxu(None, NCB - 1, 1, order), ln1(0)), 1))

        @pl.when(l == 1)
        def _():
            m = cmxu(None, NCB - 1, 1, range(R))
            _weave((_take(m, 4), 1))
            _weave((xout(3), 8), (m, R))

        return carry

    _weave((ln1(0), 1))
    with _scope("layers"):
        lax.fori_loop(0, 2, layer, 0)

    with _scope("owait"):
        for j in range(4):
            for c in ocopy(j):
                c.wait()


@jax.jit
def pallas_interleave_layers__sliding_local_dilated__ssm_conv_s4__prompt_kernel(
    A_x: jax.Array,
    A_wqkv: jax.Array,
    A_wo: jax.Array,
    B_u: jax.Array,
    B_A_re: jax.Array,
    B_A_im: jax.Array,
    B_B_re: jax.Array,
    B_B_im: jax.Array,
    B_C_re: jax.Array,
    B_C_im: jax.Array,
    B_log_dt: jax.Array,
    B_Dskip: jax.Array,
):
    del B_u
    hbm = pl.BlockSpec(memory_space=pl.ANY)
    V = pltpu.VMEM
    out = pl.pallas_call(
        _kernel,
        out_shape=jax.ShapeDtypeStruct((S, D), BF16),
        in_specs=[hbm] * 12,
        out_specs=hbm,
        scratch_shapes=[
            V((D,), BF16), V((D,), BF16),
            V((4, S, LN), BF16),
            V((12, D, LN), BF16),
            V((D, D), BF16),
            V((6, D, LN), BF16),
            V((R * LN, LN), U32),
            V((R * D, LN), F32),
            V((2 * R * D, LN), F32),
            V((D, LN), F32),
            V((R * D, LN), BF16),
            V((R * D, LN), F32),
            V((4 * WS, LN), F32),
            [V((D, LN), F32)] * R,
            [[V((40 * TS, LN), F32)] * 2] * 2,
            V((R * D, LN), BF16),
            [V((2 * R * CB, LN), F32)] * 2,
            [V((2 * R * CB, LN), F32)] * 2,
            [V((R * CB, LN), F32)] * 2,
            V((2 * R * D, LN), F32),
            [V((4, 8, 8, LN), F32)] * 2,
            V((D, LN), F32),
            V((D, LN), F32),
            [V((4, 8 * 129, LN), F32)] * 2,
            [V((4, 8 * 97, LN), F32)] * 2,
            [V((2, 8 * 25, LN), F32)] * 2,
            pltpu.SMEM((R,), jnp.int32),
            pltpu.SemaphoreType.DMA((36,)),
        ],
        compiler_params=pltpu.CompilerParams(vmem_limit_bytes=100 * 1024 * 1024, flags=FLAGS),
    )(A_x.reshape(S, D), A_wqkv, A_wo, B_A_re, B_A_im, B_B_re, B_B_im, B_C_re, B_C_im,
      B_log_dt, B_Dskip, _M)
    return out.reshape(1, S, D)
```

```python
import contextlib
import numpy as np
import jax
import jax.numpy as jnp
from jax import lax
import jax.experimental.pallas as pl
import jax.experimental.pallas.tpu as pltpu

S, D, DH, WIN = 2048, 512, 16, 8
R = 16
LN = 128
CB = 64
NCB = D // CB
EPS = 1e-5
F32, BF16, U32 = jnp.float32, jnp.bfloat16, jnp.uint32
NN, NT = (((1,), (0,)), ((), ())), (((1,), (1,)), ((), ()))


def _dft_matrices():
    lam = np.arange(LN, dtype=np.float64)[None, :, None]
    r = np.arange(R, dtype=np.float64)[:, None, None]
    f = np.arange(LN, dtype=np.float64)[None, None, :]
    th = 2.0 * np.pi * (f + 0.5) * (R * lam + r) / (2 * S) + 2.0 * np.pi * 2 / 16 * (r % 4 == 2)
    m = np.stack([np.cos(th), -np.sin(th)], axis=1).astype(BF16).view(np.uint16).astype(np.uint32)
    return (m[:, :, 0::2] | (m[:, :, 1::2] << 16)).reshape(R * LN, LN)


_M = _dft_matrices()


SCOPES = False


def _scope(name):
    return jax.named_scope(name) if SCOPES else contextlib.nullcontext()


FLAGS = None
SKIP = NOB = ''
LO, NO = 6, 1
KW = 1
WP, XP = (8, 8, 9, 9), (7, 7, 8, 9)
KB, L1 = (0, 3, 3, 1, 0, 1, 0, 0, 0), 1
B3 = ((0, 6, 0), (5, 11, 0), (10, 16, 5), (14, 16, 10), (16, 16, 14))
DO = 256
TS, WS = LN, 2 * D


class _Buf:
    def __init__(self, ref, base=0, size=None):
        if isinstance(base, int):
            self.ref, self.base = ref, base
        else:
            self.ref, self.base = ref.at[pl.ds(pl.multiple_of(base, 16), size), :], 0

    def ld(self, row, n):
        return self.ref[self.base + row:self.base + row + n, :]

    def st(self, row, v):
        self.ref[self.base + row:self.base + row + v.shape[0], :] = v.astype(self.ref.dtype)


def _weave(*stages):
    live = [[g, n, 0] for g, n in stages]
    while live:
        st = min(live, key=lambda t: t[2] / t[1])
        try:
            next(st[0])
            st[2] += 1
        except StopIteration:
            live.remove(st)


def _chain(*gens):
    for g in gens:
        yield from g


def _take(g, n):
    for _, _ in zip(range(n), g):
        yield


def _tree(op, v):
    while len(v) > 1:
        v = [op(v[i], v[i + 1]) for i in range(0, len(v), 2)]
    return v[0]


def _mult(i, n):
    return i if isinstance(i, int) else pl.multiple_of(i, n)


def _loop(lo, hi, body, unroll, force=False):
    n = hi - lo
    assert n % unroll == 0
    if n == unroll and not force:
        for i in range(lo, hi):
            body(i)
        return

    def outer(k, carry):
        for u in range(unroll):
            body(lo + k * unroll + u)
        return carry

    lax.fori_loop(0, n // unroll, outer, 0)


def _iota(shape, dim):
    return lax.broadcasted_iota(jnp.int32, shape, dim)


def _cmul(a, b):
    return (a[0] * b[0] - a[1] * b[1], a[0] * b[1] + a[1] * b[0])


def _csq(a):
    t = a[0] * a[1]
    return (a[0] * a[0] - a[1] * a[1], t + t)


def _radix4(a, b, c, d, sign):
    s0 = (a[0] + c[0], a[1] + c[1])
    d0 = (a[0] - c[0], a[1] - c[1])
    s1 = (b[0] + d[0], b[1] + d[1])
    d1 = (b[0] - d[0], b[1] - d[1])
    y0 = (s0[0] + s1[0], s0[1] + s1[1])
    y2 = (s0[0] - s1[0], s0[1] - s1[1])
    p = (d0[0] - d1[1], d0[1] + d1[0])
    m = (d0[0] + d1[1], d0[1] - d1[0])
    return (y0, p, y2, m) if sign > 0 else (y0, m, y2, p)


def _twiddle(a, k, sign):
    k = sign * k % 16
    c, s = float(np.cos(2 * np.pi * k / 16)), float(np.sin(2 * np.pi * k / 16))
    if k % 4 == 0:
        return (a, (-a[1], a[0]), (-a[0], -a[1]), (a[1], -a[0]))[k // 4]
    if k % 8 == 2:
        return ((a[0] - a[1]) * c, (a[0] + a[1]) * c)
    if k % 8 == 6:
        return ((a[0] + a[1]) * c, (a[1] - a[0]) * c)
    return (a[0] * c - a[1] * s, a[0] * s + a[1] * c)


_ROW, _COL = (0, 0, 2, 0), (0, 0, 2, 0)
_TW = [[r0 * g0 - _ROW[r0] - _COL[g0] for g0 in range(4)] for r0 in range(4)]


def _kernel(x_hbm, wqkv_hbm, wo_hbm, are_hbm, aim_hbm, bre_hbm, bim_hbm, cre_hbm, cim_hbm,
            ldt_hbm, dsk_hbm, m_hbm, out_hbm, ldt_ref, dsk_ref,
            io, wraw, woraw, par, mm, X, KF, DSK, XN, U, W, Z, KVQ, O, G, HH,
            KT, GK, E, DT, ZK, SA, SB, KO, zero, sems):
    for k in range(R):
        zero[k] = 0

    def block(name, cond=None):
        def deco(f):
            if SKIP and name in SKIP:
                return
            with _scope(name):
                f() if name in NOB else pl.when(zero[0] == 0 if cond is None else cond)(f)
        return deco

    def opaque(r):
        return zero[r] if isinstance(r, int) else 0

    pcp = [[pltpu.make_async_copy(h.at[rows, :], par.at[i, rows, :], sems.at[o + i])
            for i, h in enumerate((are_hbm, aim_hbm, bre_hbm, bim_hbm, cre_hbm, cim_hbm))]
           for o, rows in ((0, pl.ds(0, 2 * CB)), (26, pl.ds(2 * CB, D - 2 * CB)))]
    mcp = pltpu.make_async_copy(m_hbm, mm, sems.at[6])
    xcp = [pltpu.make_async_copy(x_hbm.at[:, pl.ds(j * LN, LN)], io.at[j], sems.at[7 + j])
           for j in range(4)]
    wocp = [pltpu.make_async_copy(wo_hbm.at[pl.ds(j * LN, LN), :], woraw.at[pl.ds(j * LN, LN), :],
                                  sems.at[32 + j]) for j in range(4)]
    wcp = [pltpu.make_async_copy(wqkv_hbm.at[:, pl.ds(j * LN, LN)], wraw.at[j], sems.at[12 + j])
           for j in range(12)]
    scp = [pltpu.make_async_copy(ldt_hbm, ldt_ref, sems.at[24]),
           pltpu.make_async_copy(dsk_hbm, dsk_ref, sems.at[25])]
    for c in scp + pcp[0]:
        c.start()

    for c in scp:
        c.wait()
    dt_row = jnp.exp(ldt_ref[...].astype(F32).reshape(1, D)).astype(BF16).astype(F32)
    ds_row = dsk_ref[...].astype(F32).reshape(1, D)
    for j in range(4):
        sl = slice(j * LN, (j + 1) * LN)
        DT[sl, :] = jnp.broadcast_to(dt_row[:, sl], (LN, LN)).T
        DSK[sl, :] = jnp.broadcast_to(ds_row[:, sl], (LN, LN)).T

    lane = _iota((8, LN), 1)

    def kexp(J, slot):
        for s in range(8):
            rows = pl.ds(_mult(J * CB + s * 8, 8), 8)
            if s % 2 == 0:
                p16 = [par[i, pl.ds(_mult(J * CB + s * 8, 16), 16), :].astype(F32) for i in range(6)]
            p = [v[s % 2 * 8:s % 2 * 8 + 8] for v in p16]
            dt = DT[rows, :]
            zr, zi = dt * p[0], dt * p[1]
            mag = jnp.exp(zr)
            E[slot][0, s] = mag * jnp.cos(zi)
            yield
            E[slot][1, s] = mag * jnp.sin(zi)
            w = _cmul((p[4], p[5]), (dt * p[2], dt * p[3]))
            E[slot][2, s] = w[0] * (1.0 / S)
            E[slot][3, s] = w[1] * (1.0 / S)
            ZK[rows, :] = (jnp.sum(w[0], axis=1, keepdims=True) + DSK[rows, :]) * (1.0 / S)
            yield

    def kpow(J, slot):
        sa, sb = SA[slot], SB[slot]
        for s in range(8):
            def put(ref, i, v):
                n = (ref.shape[1] // 8 - 1) // 4
                for c in range(2):
                    ref[s // 4 * 2 + c, pl.ds(s % 4 * n + i, 8, stride=4 * n + 1), :] = v[c]

            p = (E[slot][0, s], E[slot][1, s])
            b = [None]
            for k in range(4):
                for i in range(2 ** k):
                    b.append(_cmul(b[i], p) if i else p)
                    put(sb, len(b) - 2, b[-1])
                    yield
                p = _csq(p)
            put(sb, 15, p)
            b = {4: b[4], 8: b[8], 12: b[12], 16: p}
            w = (E[slot][2, s], E[slot][3, s])
            pw = []
            for k in range(5):
                pw.append(p)
                p = _csq(p)
                yield
            e512, e1024 = p, _csq(p)
            for o, st, e in ((15, 4, e512), (19, 8, e1024), (21, 8, _cmul(e512, e1024))):
                for i in range(1, 16 // st + 1):
                    put(sb, o + i, _cmul(e, b[i * st]))
                    yield

            def tree(i, v, k):
                put(sa, i, v)
                yield
                for k2 in range(k):
                    yield from tree(i + 2 ** k2, _cmul(v, pw[k2]), k2)

            yield from tree(0, w, 5)

    def ksum(J, slot):
        sa, sb = SA[slot], SB[slot]
        q = _iota((24, LN), 1) >> 5
        for hm in range(16):
            h, m = divmod(hm, 8)
            o = [lax.dot_general(sb[2 * h + c, m * 97:m * 97 + 96, :],
                                 sa[2 * h + c, m * 129:m * 129 + LN, :],
                                 NT, preferred_element_type=F32) for c in range(2)]
            o = o[0] - o[1]
            KO[slot][h, m * 25:m * 25 + 24, :] = jnp.where(
                q < 2, jnp.where(q == 0, o[0:24], o[24:48]), jnp.where(q == 2, o[48:72], o[72:96]))
            yield

    def kspread(J, slot, h):
        kb = lambda i: KO[slot][h, pl.ds(i, 8, stride=25), :]
        rnd = lambda r, st: int(np.round(r / st))
        quarter = lane >> 5
        q1 = [None] + [pltpu.roll(kb(i), 32, 1) for i in range(16, 20)]
        q2 = [None] + [pltpu.roll(kb(i), 64, 1) for i in range(20, 22)]
        q3 = [None] + [pltpu.roll(kb(i), 96, 1) for i in range(22, 24)]
        k0, q23, rest = [], {}, {}
        for r in (16,) + tuple(range(R)):
            k2, k4, k8 = rnd(r, 2), rnd(r, 4), rnd(r, 8)
            if r:
                q0 = kb(r - 1)
                if r % 2 and k2:
                    q0 = jnp.where((lane & 31) < 16, q0, kb(2 * k2 - 1))
            for s in range(4):
                row = pl.ds(_mult(J * CB + h * 32 + s * 8, 8), 8)
                if r:
                    t = q0
                    if k8 and (k8, s) not in q23:
                        q23[k8, s] = jnp.where(quarter == (s + 2) % 4, q2[k8], q3[k8])
                    if k4:
                        if (k4, k8, s) not in rest:
                            rest[k4, k8, s] = jnp.where(
                                quarter == (s + 1) % 4, q1[k4], q23[k8, s]) if k8 else q1[k4]
                        t = jnp.where(quarter == s, t, rest[k4, k8, s])
                    if s or r == 16:
                        t = pltpu.roll(t, (LN - 32 * s + (r == 16)) % LN, 1)
                    if not k8:
                        t = jnp.where(lane < (64 if k4 else 32 if k2 else 16), t, k0[s])
                else:
                    t = jnp.where(lane == 0, ZK[row, :], k0[s])
                if r == 16:
                    k0.append(t)
                else:
                    _Buf(KT[slot]).st(r * CB + h * 32 + s * 8, t)
            yield

    def ld(b, k, h, n=8, stride=CB):
        return b.ld(2 * k * stride + h, n), b.ld((2 * k + 1) * stride + h, n)

    def st(b, k, h, v, stride=CB):
        b.st(2 * k * stride + h, v[0])
        b.st((2 * k + 1) * stride + h, v[1])

    def mat(r):
        return pltpu.bitcast(jnp.concatenate(ld(_Buf(mm), r, 0, 64, 64), axis=1), BF16)

    def kfwd(i, slot):
        g = _Buf(GK, i * 2 * R * CB, 2 * R * CB)
        for r in range(R):
            t = lax.dot_general(_Buf(KT[slot]).ld(r * CB, CB), mat(r), NN, preferred_element_type=F32)
            st(g, r, 0, (t[:, :LN], t[:, LN:]))
            yield

    def kfft(i):
        kf = _Buf(KF, i * CB, 2 * R * D - D + CB)
        for h in range(0, CB, 8):
            t = []
            for r0 in range(4):
                y = _radix4(*[ld(_Buf(GK, i * 2 * R * CB), r, h) for r in range(r0, R, 4)], -1)
                t.append([_twiddle(y[g0], _TW[r0][g0], -1) for g0 in range(4)])
                yield
            for g0 in range(4):
                y = _radix4(t[0][g0], t[1][g0], t[2][g0], t[3][g0], -1)
                for g1 in range(4):
                    st(kf, 4 * g0 + g1, h, _twiddle(y[g1], _COL[g0], -1), D)
                yield

    iow = io.bitcast(U32)

    def xin(j):
        x = _Buf(X, j * LN)
        for rho in range(8):
            t = iow[j, pl.ds(rho, LN, stride=8), :].T
            x.st(2 * rho * D, pltpu.bitcast(t << 16, F32))
            x.st((2 * rho + 1) * D, pltpu.bitcast(t & np.uint32(0xFFFF0000), F32))
            yield

    def wprep(j):
        pr, pc = _iota((LN, LN), 0), _iota((LN, LN), 1)
        perm = jnp.where(pc == (pr & 7) * DH + (pr >> 3), 1.0, 0.0).astype(BF16)
        for c in range(3):
            t = lax.dot_general(perm, wraw[(c + 1) % 3 * 4 + j], NT, preferred_element_type=F32)
            if c == 2:
                t = t * (DH ** -0.5)
            for k in range(4):
                _Buf(W).st(k * WS + (3 * j + c) * LN // 2,
                           pltpu.bitcast(t[:, k * LN:(k + 1) * LN].astype(BF16), F32))
            yield
        t = jnp.dot(perm, woraw[j * LN:(j + 1) * LN, :], preferred_element_type=F32)
        _Buf(W).st(j * WS + 3 * D // 2, pltpu.bitcast(t.T.astype(BF16), F32))
        yield

    def kstep(J, ref):
        @block("kgen")
        def _():
            slot, m, v = ref % 2, [], []
            if 0 <= ref < NCB:
                m.append(ksum(J, slot))
            if 0 <= ref - 2:
                m.append(kfwd(J - 2, slot))
            v = [(g, 16 * KW) for g in m]
            if 0 <= ref - 1 < NCB:
                v.append((_chain(*[kspread(J - 1, 1 - slot, h) for h in range(2)]), 34))
            if 0 <= ref + 1 < NCB:
                v.append((kpow(J + 1, 1 - slot), 8 * 60))
            if ref + 2 < NCB:
                v.append((kexp(J + 2, slot), 16))
            for gen, steps, n in ((xin, XP, 8), (wprep, WP, 4)):
                js = [j for j in range(4) if steps[j] == ref]
                v.append((_chain(*map(gen, js)), n * len(js) + 0.01))
            _weave(*v)

    def wcopies(J):
        return [c for j in range(4) if WP[j] in J for c in wcp[j::4] + [wocp[j]]]

    for J in range(-2, 10):
        with _scope("wait"):
            for c in ({-2: pcp[0], 0: pcp[1], 2: [mcp]}.get(J, []) + wcopies((J,))
                      + [xcp[j] for j in range(4) if XP[j] == J]):
                c.wait()
        for c in {-2: pcp[1], -1: wcopies((1,)), 0: [mcp], 2: xcp + wcopies(range(6, 10))}.get(J, []):
            c.start()
        if J == 2:
            _loop(1, 3, lambda k: (kstep(2 * k, 2), kstep(2 * k + 1, 3)), 1)
        elif not 2 <= J < 6:
            kstep(J, J)

    def colsum(f, step):
        acc = [f(c * 8) for c in range(4)]
        for i in range(4, D // 8):
            acc[i % 4] = acc[i % 4] + f(i * 8)
            if i % step == step - 1:
                yield
        s = jnp.sum((acc[0] + acc[1]) + (acc[2] + acc[3]), axis=0, keepdims=True)
        return jnp.broadcast_to(s * (1.0 / D), (8, LN))

    def ln_stats(ref, base):
        x = _Buf(ref, base + zero[0], D)
        m = yield from colsum(lambda c: x.ld(c, 8), 32)
        x = _Buf(ref, base + zero[1], D)
        v = yield from colsum(lambda c: jnp.square(x.ld(c, 8) - m), 8)
        return _Buf(ref, base + zero[2], D), m, lax.rsqrt(v + EPS)

    def ln(ref, base, out, r):
        x, m, rs = yield from ln_stats(ref, base)
        for c in range(0, D, 16):
            t = [(x.ld(c + k, 8) - m) * rs for k in (0, 8)]
            _Buf(out, r * D).st(c, jnp.concatenate(t, axis=0))
            if c % 64 == 48:
                yield

    def ln1(r):
        return ln(X, r * D, XN, r)

    def ln2(r):
        return ln(Z[r], 0, U, r)

    def wdot(c, n, rhs):
        lhs = jnp.concatenate(
            [pltpu.bitcast(W[t * WS + c // 2:t * WS + (c + n) // 2, :], BF16)
             for t in range(4)], axis=1)
        return jnp.dot(lhs, rhs.ld(0, D), preferred_element_type=F32)

    def qkvproj(j, r):
        b, i = _Buf(KVQ[j % 2][r % 2]), r // 2
        for c in range(3):
            t = wdot((3 * j + c) * LN, LN, _Buf(XN, r * D + zero[(r + c) % R], D))
            if c == 2:
                b.st((32 + i) * TS, t)
            else:
                b.st((16 * c + 8 + i) * TS, t)
                if i:
                    b.st((16 * c + i) * TS, pltpu.roll(t, 1, 1))
            yield

    def core(j, r):
        b, i = _Buf(KVQ[j % 2][r % 2], zero[r], 40 * TS), r // 2
        lg = [None] * WIN
        for dh in range(DH):
            q = b.ld((32 + i) * TS + dh * 8, 8)
            for w in range(WIN):
                t = q * b.ld((8 + i - w) * TS + dh * 8, 8)
                lg[w] = t if dh == 0 else lg[w] + t
            if dh % 2:
                yield
        for w in range(i + 1, WIN):
            lg[w] = jnp.where(lane > 0, lg[w], -1e9)
        mx = _tree(jnp.maximum, lg)
        e = [jnp.exp(v - mx) for v in lg]
        inv = 1.0 / _tree(jnp.add, e)
        e = [v * inv for v in e]
        yield
        yield
        for dh in range(0, DH, 2):
            oo = []
            for k in (dh, dh + 1):
                acc = None
                for w in range(WIN):
                    t = e[w] * b.ld((24 + i - w) * TS + k * 8, 8)
                    acc = t if acc is None else acc + t
                oo.append(acc)
            _Buf(O, r * D + j * LN).st(dh * 8, jnp.concatenate(oo, axis=0))
            yield

    def oproj(r):
        for c in range(0, D, DO):
            Z[r][c:c + DO, :] = X[r * D + c:r * D + c + DO, :] + wdot(
                3 * D + c, DO, _Buf(O, r * D + zero[(r + c // DO) % R], D))
            yield

    def cmxu(fi, ii, slot, rs):
        if fi is not None:
            u_ = _Buf(U, fi * CB, R * D - D + CB)
        if ii is not None:
            x = _Buf(X, ii * CB, R * D - D + CB)
        for r in rs:
            if fi is not None:
                t = lax.dot_general(u_.ld(r * D, CB), mat(r), NN, preferred_element_type=F32)
                st(_Buf(G[slot]), r, 0, (t[:, :LN], t[:, LN:]))
                yield
            if ii is not None:
                lhs = jnp.concatenate(ld(_Buf(HH[slot]), r, 0, CB), axis=1)
                t = lax.dot_general(lhs, mat(r), NT, preferred_element_type=F32)
                x.st(r * D, _Buf(Z[r], ii * CB, CB).ld(0, CB) + t)
                yield

    def cmid(i, slot):
        g, hh = _Buf(G[slot], zero[0], 2 * R * CB), _Buf(HH[slot])
        kf = _Buf(KF, i * CB, 2 * R * D - D + CB)

        for h in range(0, CB, 8):
            t, v = [], []
            for r0 in range(4):
                y = _radix4(*[ld(g, r, h) for r in range(r0, R, 4)], -1)
                t.append([_twiddle(y[g0], _TW[r0][g0], -1) for g0 in range(4)])
                yield
            yield
            for g0 in range(4):
                y = _radix4(t[0][g0], t[1][g0], t[2][g0], t[3][g0], -1)
                yield
                y = [_cmul(y[g1], ld(kf, 4 * g0 + g1, h, 8, D)) for g1 in range(4)]
                yield
                y = _radix4(*y, 1)
                v.append([_twiddle(y[r0], _TW[r0][g0], 1) for r0 in range(4)])
                yield
                if g0 != 1:
                    yield
            for r0 in range(4):
                y = _radix4(*[v[g0][r0] for g0 in range(4)], 1)
                for r1 in range(4):
                    st(hh, r0 + 4 * r1, h, y[r1])
                yield

    def ocopy(j):
        n = S // NO
        return [pltpu.make_async_copy(
            io.at[j, pl.ds(k * n, n), :],
            out_hbm.at[pl.ds(k * n, n), pl.ds(_mult(j * LN, LN), LN)], sems.at[NO * j + k])
            for k in range(NO)]

    def xout(j, lo=0, hi=8):
        x = _Buf(X, j * LN, R * D - D + LN)
        for rho in range(lo, hi):
            a, b = (pltpu.bitcast(x.ld(r * D, LN).astype(BF16).astype(F32), U32)
                      for r in (2 * rho, 2 * rho + 1))
            iow[j, pl.ds(rho, LN, stride=8), :] = ((a >> 16) | b).T
            yield
        for c in ocopy(j) if hi == 8 else ():
            c.start()

    order = list(range(0, R, 2)) + list(range(1, R, 2))
    NCORE, NLN1, NLN2 = 18, 18, 18

    def layer(l, carry):
        def spectra(b):
            ids = range(sum(KB[:b]), sum(KB[:b + 1]))
            return _chain(*map(kfft, ids)), 64 * len(ids) + 0.01

        @block("ph1")
        def _():
            _weave((_chain(*[qkvproj(0, r) for r in order]), 3 * R),
                   (_chain(*map(ln1, order[1:])), NLN1 * (R + L1)), spectra(0))

        for b, (j, lo, hi) in enumerate(((1, 0, R), (2, 0, R), (3, 0, R // 2), (3, R // 2, R))):
            @block("ph2")
            def _():
                early = _chain(*[core(3, r) for r in order[:LO if lo else 0]])
                kf, nk = spectra(1 + b)
                nk = int(nk) // (hi - lo)
                for r in order[lo:hi]:
                    _weave((qkvproj(j, r), 3), (core(j - 1, r), NCORE),
                           (_take(early, -(-LO * NCORE // 8)), LO * NCORE / 8),
                           (_take(kf, nk), nk + 0.01))

        for b, (prev, cur) in enumerate(zip(B3, B3[1:])):
            @block("ph3")
            def _():
                w, c, n = (order[u:v] for u, v in zip(prev, cur))
                _weave((_chain(*map(oproj, w)), len(w) * D // DO),
                       (_chain(*[core(3, r) for r in c]), len(c) * NCORE + 0.01),
                       (_chain(*map(ln2, n)), len(n) * NLN2 + 0.01), spectra(5 + b))

        def cstep(i, slot, f=True, m=True, v=True, out=(), cond=None):
            @block("conv", cond)
            def _():
                _weave((cmxu(i + 1 if f else None, i - 1 if v else None, 1 - slot, order), R * (f + v)),
                       *([(cmid(i, slot), 3 * CB)] if m else []),
                       *[(ln2(r), 2 * NLN2) for r in order[B3[-1][2]:] if f and not m], *out)

        cstep(-1, 1, m=False, v=False)
        cstep(0, 0, v=False)

        def cpair(k):
            for e in range(2):
                cstep(2 * k + 1 + e, 1 - e, cond=l * k == 0)
                cstep(2 * k + 1 + e, 1 - e, cond=l * k > 0,
                      out=[(xout(k - 1, 4 * e, 4 * e + 4), 5)])

        _loop(0, NCB // 2 - 1, cpair, 1)
        cstep(NCB - 1, 1, f=False, cond=l == 0)
        cstep(NCB - 1, 1, f=False, cond=l == 1, out=[(xout(2), 10)])

        @pl.when(l == 0)
        def _():
            _weave((_chain(cmxu(None, NCB - 1, 1, order), ln1(0)), 1))

        @pl.when(l == 1)
        def _():
            m = cmxu(None, NCB - 1, 1, range(R))
            _weave((_take(m, 4), 1))
            _weave((xout(3), 8), (m, R))

        return carry

    _weave((ln1(0), 1))
    with _scope("layers"):
        lax.fori_loop(0, 2, layer, 0)

    with _scope("owait"):
        for j in range(4):
            for c in ocopy(j):
                c.wait()


@jax.jit
def pallas_interleave_layers__sliding_local_dilated__ssm_conv_s4__prompt_kernel(
    A_x: jax.Array,
    A_wqkv: jax.Array,
    A_wo: jax.Array,
    B_u: jax.Array,
    B_A_re: jax.Array,
    B_A_im: jax.Array,
    B_B_re: jax.Array,
    B_B_im: jax.Array,
    B_C_re: jax.Array,
    B_C_im: jax.Array,
    B_log_dt: jax.Array,
    B_Dskip: jax.Array,
):
    del B_u
    hbm = pl.BlockSpec(memory_space=pl.ANY)
    V = pltpu.VMEM
    out = pl.pallas_call(
        _kernel,
        out_shape=jax.ShapeDtypeStruct((S, D), BF16),
        in_specs=[hbm] * 12,
        out_specs=hbm,
        scratch_shapes=[
            V((D,), BF16), V((D,), BF16),
            V((4, S, LN), BF16),
            V((12, D, LN), BF16),
            V((D, D), BF16),
            V((6, D, LN), BF16),
            V((R * LN, LN), U32),
            V((R * D, LN), F32),
            V((2 * R * D, LN), F32),
            V((D, LN), F32),
            V((R * D, LN), BF16),
            V((R * D, LN), F32),
            V((4 * WS, LN), F32),
            [V((D, LN), F32)] * R,
            [[V((40 * TS, LN), F32)] * 2] * 2,
            V((R * D, LN), BF16),
            [V((2 * R * CB, LN), F32)] * 2,
            [V((2 * R * CB, LN), F32)] * 2,
            [V((R * CB, LN), F32)] * 2,
            V((2 * R * D, LN), F32),
            [V((4, 8, 8, LN), F32)] * 2,
            V((D, LN), F32),
            V((D, LN), F32),
            [V((4, 8 * 129, LN), F32)] * 2,
            [V((4, 8 * 97, LN), F32)] * 2,
            [V((2, 8 * 25, LN), F32)] * 2,
            pltpu.SMEM((R,), jnp.int32),
            pltpu.SemaphoreType.DMA((36,)),
        ],
        compiler_params=pltpu.CompilerParams(vmem_limit_bytes=100 * 1024 * 1024, flags=FLAGS),
    )(A_x.reshape(S, D), A_wqkv, A_wo, B_A_re, B_A_im, B_B_re, B_B_im, B_C_re, B_C_im,
      B_log_dt, B_Dskip, _M)
    return out.reshape(1, S, D)
```

```python
import numpy as np
import jax
import jax.numpy as jnp
from jax import lax
import jax.experimental.pallas as pl
import jax.experimental.pallas.tpu as pltpu

S, D, DH, WIN = 2048, 512, 16, 8
R = 16
LN = 128
CB = 64
NCB = D // CB
EPS = 1e-5
F32, BF16, U32 = jnp.float32, jnp.bfloat16, jnp.uint32
NN, NT = (((1,), (0,)), ((), ())), (((1,), (1,)), ((), ()))


def _dft_matrices():
    lam = np.arange(LN, dtype=np.float64)[None, :, None]
    r = np.arange(R, dtype=np.float64)[:, None, None]
    f = np.arange(LN, dtype=np.float64)[None, None, :]
    th = 2.0 * np.pi * (f + 0.5) * (R * lam + r) / (2 * S) + 2.0 * np.pi * 2 / 16 * (r % 4 == 2)
    m = np.stack([np.cos(th), -np.sin(th)], axis=1).astype(BF16).view(np.uint16).astype(np.uint32)
    return (m[:, :, 0::2] | (m[:, :, 1::2] << 16)).reshape(R * LN, LN)


_M = _dft_matrices()


WS = 2 * D
DO = 256
EARLY = 6
B3 = ((0, EARLY, 0), (5, 11, 0), (10, 16, 5), (14, 16, 10), (16, 16, 14))
KB = (3, 3, 1, 0, 1, 0, 0, 0)
WP, XP = (8, 8, 9, 9), (7, 7, 8, 9)


class _Buf:
    def __init__(self, ref, base=0, size=None):
        if isinstance(base, int):
            self.ref, self.base = ref, base
        else:
            self.ref, self.base = ref.at[pl.ds(pl.multiple_of(base, 16), size), :], 0

    def ld(self, row, n):
        return self.ref[self.base + row:self.base + row + n, :]

    def st(self, row, v):
        self.ref[self.base + row:self.base + row + v.shape[0], :] = v.astype(self.ref.dtype)


def _weave(*stages):
    live = [[g, n, 0] for g, n in stages]
    while live:
        st = min(live, key=lambda t: t[2] / t[1])
        try:
            next(st[0])
            st[2] += 1
        except StopIteration:
            live.remove(st)


def _chain(*gens):
    for g in gens:
        yield from g


def _take(g, n):
    for _, _ in zip(range(n), g):
        yield


def _tree(op, v):
    while len(v) > 1:
        v = [op(v[i], v[i + 1]) for i in range(0, len(v), 2)]
    return v[0]


def _mult(i, n):
    return i if isinstance(i, int) else pl.multiple_of(i, n)


def _loop(lo, hi, body):
    def step(k, carry):
        body(k)
        return carry

    lax.fori_loop(lo, hi, step, 0)


def _iota(shape, dim):
    return lax.broadcasted_iota(jnp.int32, shape, dim)


def _cmul(a, b):
    return (a[0] * b[0] - a[1] * b[1], a[0] * b[1] + a[1] * b[0])


def _csq(a):
    t = a[0] * a[1]
    return (a[0] * a[0] - a[1] * a[1], t + t)


def _radix4(a, b, c, d, sign):
    s0 = (a[0] + c[0], a[1] + c[1])
    d0 = (a[0] - c[0], a[1] - c[1])
    s1 = (b[0] + d[0], b[1] + d[1])
    d1 = (b[0] - d[0], b[1] - d[1])
    y0 = (s0[0] + s1[0], s0[1] + s1[1])
    y2 = (s0[0] - s1[0], s0[1] - s1[1])
    p = (d0[0] - d1[1], d0[1] + d1[0])
    m = (d0[0] + d1[1], d0[1] - d1[0])
    return (y0, p, y2, m) if sign > 0 else (y0, m, y2, p)


def _twiddle(a, k, sign):
    k = sign * k % 16
    c, s = float(np.cos(2 * np.pi * k / 16)), float(np.sin(2 * np.pi * k / 16))
    if k % 4 == 0:
        return (a, (-a[1], a[0]), (-a[0], -a[1]), (a[1], -a[0]))[k // 4]
    if k % 8 == 2:
        return ((a[0] - a[1]) * c, (a[0] + a[1]) * c)
    if k % 8 == 6:
        return ((a[0] + a[1]) * c, (a[1] - a[0]) * c)
    return (a[0] * c - a[1] * s, a[0] * s + a[1] * c)


_ROW, _COL = (0, 0, 2, 0), (0, 0, 2, 0)
_TW = [[r0 * g0 - _ROW[r0] - _COL[g0] for g0 in range(4)] for r0 in range(4)]


def _kernel(x_hbm, wqkv_hbm, wo_hbm, are_hbm, aim_hbm, bre_hbm, bim_hbm, cre_hbm, cim_hbm,
            ldt_hbm, dsk_hbm, m_hbm, out_hbm, ldt_ref, dsk_ref,
            io, wraw, woraw, par, mm, X, KF, DSK, XN, U, W, Z, KVQ, O, G, HH,
            KT, GK, E, DT, ZK, SA, SB, KO, zero, sems):
    for k in range(R):
        zero[k] = 0

    def block(cond=None):
        return pl.when(zero[0] == 0 if cond is None else cond)

    pcp = [[pltpu.make_async_copy(h.at[rows, :], par.at[i, rows, :], sems.at[o + i])
            for i, h in enumerate((are_hbm, aim_hbm, bre_hbm, bim_hbm, cre_hbm, cim_hbm))]
           for o, rows in ((0, pl.ds(0, 2 * CB)), (26, pl.ds(2 * CB, D - 2 * CB)))]
    mcp = pltpu.make_async_copy(m_hbm, mm, sems.at[6])
    xcp = [pltpu.make_async_copy(x_hbm.at[:, pl.ds(j * LN, LN)], io.at[j], sems.at[7 + j])
           for j in range(4)]
    wocp = [pltpu.make_async_copy(wo_hbm.at[pl.ds(j * LN, LN), :], woraw.at[pl.ds(j * LN, LN), :],
                                  sems.at[32 + j]) for j in range(4)]
    wcp = [pltpu.make_async_copy(wqkv_hbm.at[:, pl.ds(j * LN, LN)], wraw.at[j], sems.at[12 + j])
           for j in range(12)]
    scp = [pltpu.make_async_copy(ldt_hbm, ldt_ref, sems.at[24]),
           pltpu.make_async_copy(dsk_hbm, dsk_ref, sems.at[25])]
    for c in scp + pcp[0]:
        c.start()

    for c in scp:
        c.wait()
    dt_row = jnp.exp(ldt_ref[...].astype(F32).reshape(1, D)).astype(BF16).astype(F32)
    ds_row = dsk_ref[...].astype(F32).reshape(1, D)
    for j in range(4):
        sl = slice(j * LN, (j + 1) * LN)
        DT[sl, :] = jnp.broadcast_to(dt_row[:, sl], (LN, LN)).T
        DSK[sl, :] = jnp.broadcast_to(ds_row[:, sl], (LN, LN)).T

    lane = _iota((8, LN), 1)

    def kexp(J, slot):
        for s in range(8):
            rows = pl.ds(_mult(J * CB + s * 8, 8), 8)
            if s % 2 == 0:
                p16 = [par[i, pl.ds(_mult(J * CB + s * 8, 16), 16), :].astype(F32) for i in range(6)]
            p = [v[s % 2 * 8:s % 2 * 8 + 8] for v in p16]
            dt = DT[rows, :]
            zr, zi = dt * p[0], dt * p[1]
            mag = jnp.exp(zr)
            E[slot][0, s] = mag * jnp.cos(zi)
            yield
            E[slot][1, s] = mag * jnp.sin(zi)
            w = _cmul((p[4], p[5]), (dt * p[2], dt * p[3]))
            E[slot][2, s] = w[0] * (1.0 / S)
            E[slot][3, s] = w[1] * (1.0 / S)
            ZK[rows, :] = (jnp.sum(w[0], axis=1, keepdims=True) + DSK[rows, :]) * (1.0 / S)
            yield

    def kpow(J, slot):
        sa, sb = SA[slot], SB[slot]
        for s in range(8):
            def put(ref, i, v):
                n = (ref.shape[1] // 8 - 1) // 4
                for c in range(2):
                    ref[s // 4 * 2 + c, pl.ds(s % 4 * n + i, 8, stride=4 * n + 1), :] = v[c]

            p = (E[slot][0, s], E[slot][1, s])
            b = [None]
            for k in range(4):
                for i in range(2 ** k):
                    b.append(_cmul(b[i], p) if i else p)
                    put(sb, len(b) - 2, b[-1])
                    yield
                p = _csq(p)
            put(sb, 15, p)
            b = {4: b[4], 8: b[8], 12: b[12], 16: p}
            w = (E[slot][2, s], E[slot][3, s])
            pw = []
            for k in range(5):
                pw.append(p)
                p = _csq(p)
                yield
            e512, e1024 = p, _csq(p)
            for o, st, e in ((15, 4, e512), (19, 8, e1024), (21, 8, _cmul(e512, e1024))):
                for i in range(1, 16 // st + 1):
                    put(sb, o + i, _cmul(e, b[i * st]))
                    yield

            def tree(i, v, k):
                put(sa, i, v)
                yield
                for k2 in range(k):
                    yield from tree(i + 2 ** k2, _cmul(v, pw[k2]), k2)

            yield from tree(0, w, 5)

    def ksum(J, slot):
        sa, sb = SA[slot], SB[slot]
        q = _iota((24, LN), 1) >> 5
        for hm in range(16):
            h, m = divmod(hm, 8)
            o = [lax.dot_general(sb[2 * h + c, m * 97:m * 97 + 96, :],
                                 sa[2 * h + c, m * 129:m * 129 + LN, :],
                                 NT, preferred_element_type=F32) for c in range(2)]
            o = o[0] - o[1]
            KO[slot][h, m * 25:m * 25 + 24, :] = jnp.where(
                q < 2, jnp.where(q == 0, o[0:24], o[24:48]), jnp.where(q == 2, o[48:72], o[72:96]))
            yield

    def kspread(J, slot, h):
        kb = lambda i: KO[slot][h, pl.ds(i, 8, stride=25), :]
        rnd = lambda r, st: int(np.round(r / st))
        quarter = lane >> 5
        q1 = [None] + [pltpu.roll(kb(i), 32, 1) for i in range(16, 20)]
        q2 = [None] + [pltpu.roll(kb(i), 64, 1) for i in range(20, 22)]
        q3 = [None] + [pltpu.roll(kb(i), 96, 1) for i in range(22, 24)]
        k0, q23, rest = [], {}, {}
        for r in (16,) + tuple(range(R)):
            k2, k4, k8 = rnd(r, 2), rnd(r, 4), rnd(r, 8)
            if r:
                q0 = kb(r - 1)
                if r % 2 and k2:
                    q0 = jnp.where((lane & 31) < 16, q0, kb(2 * k2 - 1))
            for s in range(4):
                row = pl.ds(_mult(J * CB + h * 32 + s * 8, 8), 8)
                if r:
                    t = q0
                    if k8 and (k8, s) not in q23:
                        q23[k8, s] = jnp.where(quarter == (s + 2) % 4, q2[k8], q3[k8])
                    if k4:
                        if (k4, k8, s) not in rest:
                            rest[k4, k8, s] = jnp.where(
                                quarter == (s + 1) % 4, q1[k4], q23[k8, s]) if k8 else q1[k4]
                        t = jnp.where(quarter == s, t, rest[k4, k8, s])
                    if s or r == 16:
                        t = pltpu.roll(t, (LN - 32 * s + (r == 16)) % LN, 1)
                    if not k8:
                        t = jnp.where(lane < (64 if k4 else 32 if k2 else 16), t, k0[s])
                else:
                    t = jnp.where(lane == 0, ZK[row, :], k0[s])
                if r == 16:
                    k0.append(t)
                else:
                    _Buf(KT[slot]).st(r * CB + h * 32 + s * 8, t)
            yield

    def ld(b, k, h, n=8, stride=CB):
        return b.ld(2 * k * stride + h, n), b.ld((2 * k + 1) * stride + h, n)

    def st(b, k, h, v, stride=CB):
        b.st(2 * k * stride + h, v[0])
        b.st((2 * k + 1) * stride + h, v[1])

    def mat(r):
        return pltpu.bitcast(jnp.concatenate(ld(_Buf(mm), r, 0, 64, 64), axis=1), BF16)

    def kfwd(i, slot):
        g = _Buf(GK, i * 2 * R * CB, 2 * R * CB)
        for r in range(R):
            t = lax.dot_general(_Buf(KT[slot]).ld(r * CB, CB), mat(r), NN, preferred_element_type=F32)
            st(g, r, 0, (t[:, :LN], t[:, LN:]))
            yield

    def kfft(i):
        kf = _Buf(KF, i * CB, 2 * R * D - D + CB)
        for h in range(0, CB, 8):
            t = []
            for r0 in range(4):
                y = _radix4(*[ld(_Buf(GK, i * 2 * R * CB), r, h) for r in range(r0, R, 4)], -1)
                t.append([_twiddle(y[g0], _TW[r0][g0], -1) for g0 in range(4)])
                yield
            for g0 in range(4):
                y = _radix4(t[0][g0], t[1][g0], t[2][g0], t[3][g0], -1)
                for g1 in range(4):
                    st(kf, 4 * g0 + g1, h, _twiddle(y[g1], _COL[g0], -1), D)
                yield

    iow = io.bitcast(U32)

    def xin(j):
        x = _Buf(X, j * LN)
        for rho in range(8):
            t = iow[j, pl.ds(rho, LN, stride=8), :].T
            x.st(2 * rho * D, pltpu.bitcast(t << 16, F32))
            x.st((2 * rho + 1) * D, pltpu.bitcast(t & np.uint32(0xFFFF0000), F32))
            yield

    def wprep(j):
        pr, pc = _iota((LN, LN), 0), _iota((LN, LN), 1)
        perm = jnp.where(pc == (pr & 7) * DH + (pr >> 3), 1.0, 0.0).astype(BF16)
        for c in range(3):
            t = lax.dot_general(perm, wraw[(c + 1) % 3 * 4 + j], NT, preferred_element_type=F32)
            if c == 2:
                t = t * (DH ** -0.5)
            for k in range(4):
                _Buf(W).st(k * WS + (3 * j + c) * LN // 2,
                           pltpu.bitcast(t[:, k * LN:(k + 1) * LN].astype(BF16), U32))
            yield
        t = jnp.dot(perm, woraw[j * LN:(j + 1) * LN, :], preferred_element_type=F32)
        _Buf(W).st(j * WS + 3 * D // 2, pltpu.bitcast(t.T.astype(BF16), U32))
        yield

    def kstep(J, ref):
        @block()
        def _():
            slot, m, v = ref % 2, [], []
            if 0 <= ref < NCB:
                m.append(ksum(J, slot))
            if 0 <= ref - 2:
                m.append(kfwd(J - 2, slot))
            v = [(g, 16) for g in m]
            if 0 <= ref - 1 < NCB:
                v.append((_chain(*[kspread(J - 1, 1 - slot, h) for h in range(2)]), 34))
            if 0 <= ref + 1 < NCB:
                v.append((kpow(J + 1, 1 - slot), 8 * 60))
            if ref + 2 < NCB:
                v.append((kexp(J + 2, slot), 16))
            for gen, steps, n in ((xin, XP, 8), (wprep, WP, 4)):
                js = [j for j in range(4) if steps[j] == ref]
                v.append((_chain(*map(gen, js)), n * len(js) + 0.01))
            _weave(*v)

    def wcopies(J):
        return [c for j in range(4) if WP[j] in J for c in wcp[j::4] + [wocp[j]]]

    for J in range(-2, 10):
        for c in ({-2: pcp[0], 0: pcp[1], 2: [mcp]}.get(J, []) + wcopies((J,))
                  + [xcp[j] for j in range(4) if XP[j] == J]):
            c.wait()
        for c in {-2: pcp[1], 0: [mcp], 2: xcp + wcopies(WP)}.get(J, []):
            c.start()
        if J == 2:
            _loop(1, 3, lambda k: (kstep(2 * k, 2), kstep(2 * k + 1, 3)))
        elif not 2 <= J < 6:
            kstep(J, J)

    def colsum(f, step):
        acc = [f(c * 8) for c in range(4)]
        for i in range(4, D // 8):
            acc[i % 4] = acc[i % 4] + f(i * 8)
            if i % step == step - 1:
                yield
        s = jnp.sum((acc[0] + acc[1]) + (acc[2] + acc[3]), axis=0, keepdims=True)
        return jnp.broadcast_to(s * (1.0 / D), (8, LN))

    def ln_stats(ref, base):
        x = _Buf(ref, base + zero[0], D)
        m = yield from colsum(lambda c: x.ld(c, 8), 32)
        x = _Buf(ref, base + zero[1], D)
        v = yield from colsum(lambda c: jnp.square(x.ld(c, 8) - m), 8)
        return _Buf(ref, base + zero[2], D), m, lax.rsqrt(v + EPS)

    def ln(ref, base, out, r):
        x, m, rs = yield from ln_stats(ref, base)
        for c in range(0, D, 16):
            t = [(x.ld(c + k, 8) - m) * rs for k in (0, 8)]
            _Buf(out, r * D).st(c, jnp.concatenate(t, axis=0))
            if c % 64 == 48:
                yield

    def ln1(r):
        return ln(X, r * D, XN, r)

    def ln2(r):
        return ln(Z[r], 0, U, r)

    def wdot(c, n, rhs):
        lhs = jnp.concatenate(
            [pltpu.bitcast(W[t * WS + c // 2:t * WS + (c + n) // 2, :], BF16)
             for t in range(4)], axis=1)
        return jnp.dot(lhs, rhs.ld(0, D), preferred_element_type=F32)

    def qkvproj(j, r):
        b, i = _Buf(KVQ[j % 2][r % 2]), r // 2
        for c in range(3):
            t = wdot((3 * j + c) * LN, LN, _Buf(XN, r * D + zero[(r + c) % R], D))
            if c == 2:
                b.st((32 + i) * LN, t)
            else:
                b.st((16 * c + 8 + i) * LN, t)
                if i:
                    b.st((16 * c + i) * LN, pltpu.roll(t, 1, 1))
            yield

    def core(j, r):
        b, i = _Buf(KVQ[j % 2][r % 2], zero[r], 40 * LN), r // 2
        lg = [None] * WIN
        for dh in range(DH):
            q = b.ld((32 + i) * LN + dh * 8, 8)
            for w in range(WIN):
                t = q * b.ld((8 + i - w) * LN + dh * 8, 8)
                lg[w] = t if dh == 0 else lg[w] + t
            if dh % 2:
                yield
        for w in range(i + 1, WIN):
            lg[w] = jnp.where(lane > 0, lg[w], -1e9)
        mx = _tree(jnp.maximum, lg)
        e = [jnp.exp(v - mx) for v in lg]
        inv = 1.0 / _tree(jnp.add, e)
        e = [v * inv for v in e]
        yield
        yield
        for dh in range(0, DH, 2):
            oo = []
            for k in (dh, dh + 1):
                acc = None
                for w in range(WIN):
                    t = e[w] * b.ld((24 + i - w) * LN + k * 8, 8)
                    acc = t if acc is None else acc + t
                oo.append(acc)
            _Buf(O, r * D + j * LN).st(dh * 8, jnp.concatenate(oo, axis=0))
            yield

    def oproj(r):
        for c in range(0, D, DO):
            Z[r][c:c + DO, :] = X[r * D + c:r * D + c + DO, :] + wdot(
                3 * D + c, DO, _Buf(O, r * D + zero[(r + c // DO) % R], D))
            yield

    def cmxu(fi, ii, slot, rs):
        if fi is not None:
            u_ = _Buf(U, fi * CB, R * D - D + CB)
        if ii is not None:
            x = _Buf(X, ii * CB, R * D - D + CB)
        for r in rs:
            if fi is not None:
                t = lax.dot_general(u_.ld(r * D, CB), mat(r), NN, preferred_element_type=F32)
                st(_Buf(G[slot]), r, 0, (t[:, :LN], t[:, LN:]))
                yield
            if ii is not None:
                lhs = jnp.concatenate(ld(_Buf(HH[slot]), r, 0, CB), axis=1)
                t = lax.dot_general(lhs, mat(r), NT, preferred_element_type=F32)
                x.st(r * D, _Buf(Z[r], ii * CB, CB).ld(0, CB) + t)
                yield

    def cmid(i, slot):
        g, hh = _Buf(G[slot], zero[0], 2 * R * CB), _Buf(HH[slot])
        kf = _Buf(KF, i * CB, 2 * R * D - D + CB)

        for h in range(0, CB, 8):
            t, v = [], []
            for r0 in range(4):
                y = _radix4(*[ld(g, r, h) for r in range(r0, R, 4)], -1)
                t.append([_twiddle(y[g0], _TW[r0][g0], -1) for g0 in range(4)])
                yield
            yield
            for g0 in range(4):
                y = _radix4(t[0][g0], t[1][g0], t[2][g0], t[3][g0], -1)
                yield
                y = [_cmul(y[g1], ld(kf, 4 * g0 + g1, h, 8, D)) for g1 in range(4)]
                yield
                y = _radix4(*y, 1)
                v.append([_twiddle(y[r0], _TW[r0][g0], 1) for r0 in range(4)])
                yield
                if g0 != 1:
                    yield
            for r0 in range(4):
                y = _radix4(*[v[g0][r0] for g0 in range(4)], 1)
                for r1 in range(4):
                    st(hh, r0 + 4 * r1, h, y[r1])
                yield

    def ocopy(j):
        return pltpu.make_async_copy(
            io.at[j], out_hbm.at[:, pl.ds(_mult(j * LN, LN), LN)], sems.at[7 + j])

    def xout(j, lo=0, hi=8):
        x = _Buf(X, j * LN, R * D - D + LN)
        for rho in range(lo, hi):
            a, b = (pltpu.bitcast(x.ld(r * D, LN).astype(BF16).astype(F32), U32)
                      for r in (2 * rho, 2 * rho + 1))
            iow[j, pl.ds(rho, LN, stride=8), :] = ((a >> 16) | b).T
            yield
        if hi == 8:
            ocopy(j).start()

    order = list(range(0, R, 2)) + list(range(1, R, 2))
    NCORE, NLN1, NLN2 = 18, 18, 18

    def layer(l, carry):
        def spectra(b):
            ids = range(sum(KB[:b]), sum(KB[:b + 1]))
            return _chain(*map(kfft, ids)), 64 * len(ids) + 0.01

        @block()
        def _():
            _weave((_chain(*[qkvproj(0, r) for r in order]), 3 * R),
                   (_chain(*map(ln1, order[1:])), NLN1 * (R + 1)))

        for b, (j, lo, hi) in enumerate(((1, 0, R), (2, 0, R), (3, 0, R // 2), (3, R // 2, R))):
            @block()
            def _():
                early = _chain(*[core(3, r) for r in order[:EARLY if lo else 0]])
                kf, nk = spectra(b)
                nk = int(nk) // (hi - lo)
                for r in order[lo:hi]:
                    _weave((qkvproj(j, r), 3), (core(j - 1, r), NCORE),
                           (_take(early, -(-EARLY * NCORE // 8)), EARLY * NCORE / 8),
                           (_take(kf, nk), nk + 0.01))

        for b, (prev, cur) in enumerate(zip(B3, B3[1:])):
            @block()
            def _():
                w, c, n = (order[u:v] for u, v in zip(prev, cur))
                _weave((_chain(*map(oproj, w)), len(w) * D // DO),
                       (_chain(*[core(3, r) for r in c]), len(c) * NCORE + 0.01),
                       (_chain(*map(ln2, n)), len(n) * NLN2 + 0.01), spectra(4 + b))

        def cstep(i, slot, f=True, m=True, v=True, out=(), cond=None):
            @block(cond)
            def _():
                _weave((cmxu(i + 1 if f else None, i - 1 if v else None, 1 - slot, order), R * (f + v)),
                       *([(cmid(i, slot), 3 * CB)] if m else []),
                       *[(ln2(r), 2 * NLN2) for r in order[B3[-1][2]:] if f and not m], *out)

        cstep(-1, 1, m=False, v=False)
        cstep(0, 0, v=False)

        def cpair(k):
            for e in range(2):
                cstep(2 * k + 1 + e, 1 - e, cond=l * k == 0)
                cstep(2 * k + 1 + e, 1 - e, cond=l * k > 0,
                      out=[(xout(k - 1, 4 * e, 4 * e + 4), 5)])

        _loop(0, NCB // 2 - 1, cpair)
        cstep(NCB - 1, 1, f=False, cond=l == 0)
        cstep(NCB - 1, 1, f=False, cond=l == 1, out=[(xout(2), 10)])

        @pl.when(l == 0)
        def _():
            _weave((_chain(cmxu(None, NCB - 1, 1, order), ln1(0)), 1))

        @pl.when(l == 1)
        def _():
            m = cmxu(None, NCB - 1, 1, range(R))
            _weave((_take(m, 4), 1))
            _weave((xout(3), 8), (m, R))

        return carry

    _weave((ln1(0), 1))
    lax.fori_loop(0, 2, layer, 0)

    for j in range(4):
        ocopy(j).wait()


@jax.jit
def pallas_interleave_layers__sliding_local_dilated__ssm_conv_s4__prompt_kernel(
    A_x: jax.Array,
    A_wqkv: jax.Array,
    A_wo: jax.Array,
    B_u: jax.Array,
    B_A_re: jax.Array,
    B_A_im: jax.Array,
    B_B_re: jax.Array,
    B_B_im: jax.Array,
    B_C_re: jax.Array,
    B_C_im: jax.Array,
    B_log_dt: jax.Array,
    B_Dskip: jax.Array,
):
    del B_u
    hbm = pl.BlockSpec(memory_space=pl.ANY)
    V = pltpu.VMEM
    out = pl.pallas_call(
        _kernel,
        out_shape=jax.ShapeDtypeStruct((S, D), BF16),
        in_specs=[hbm] * 12,
        out_specs=hbm,
        scratch_shapes=[
            V((D,), BF16), V((D,), BF16),
            V((4, S, LN), BF16),
            V((12, D, LN), BF16),
            V((D, D), BF16),
            V((6, D, LN), BF16),
            V((R * LN, LN), U32),
            V((R * D, LN), F32),
            V((2 * R * D, LN), F32),
            V((D, LN), F32),
            V((R * D, LN), BF16),
            V((R * D, LN), F32),
            V((4 * WS, LN), U32),
            [V((D, LN), F32)] * R,
            [[V((40 * LN, LN), F32)] * 2] * 2,
            V((R * D, LN), BF16),
            [V((2 * R * CB, LN), F32)] * 2,
            [V((2 * R * CB, LN), F32)] * 2,
            [V((R * CB, LN), F32)] * 2,
            V((2 * R * D, LN), F32),
            [V((4, 8, 8, LN), F32)] * 2,
            V((D, LN), F32),
            V((D, LN), F32),
            [V((4, 8 * 129, LN), F32)] * 2,
            [V((4, 8 * 97, LN), F32)] * 2,
            [V((2, 8 * 25, LN), F32)] * 2,
            pltpu.SMEM((R,), jnp.int32),
            pltpu.SemaphoreType.DMA((36,)),
        ],
        compiler_params=pltpu.CompilerParams(vmem_limit_bytes=100 * 1024 * 1024),
    )(A_x.reshape(S, D), A_wqkv, A_wo, B_A_re, B_A_im, B_B_re, B_B_im, B_C_re, B_C_im,
      B_log_dt, B_Dskip, _M)
    return out.reshape(1, S, D)
```

```python
import numpy as np
import jax
import jax.numpy as jnp
from jax import lax
import jax.experimental.pallas as pl
import jax.experimental.pallas.tpu as pltpu

S, D, DH, WIN = 2048, 512, 16, 8
R = 16
LN = 128
CB = 64
NCB = D // CB
EPS = 1e-5
F32, BF16, U32 = jnp.float32, jnp.bfloat16, jnp.uint32
NN, NT = (((1,), (0,)), ((), ())), (((1,), (1,)), ((), ()))


def _dft_matrices():
    lam = np.arange(LN, dtype=np.float64)[None, :, None]
    r = np.arange(R, dtype=np.float64)[:, None, None]
    f = np.arange(LN, dtype=np.float64)[None, None, :]
    th = 2.0 * np.pi * (f + 0.5) * (R * lam + r) / (2 * S) + 2.0 * np.pi * 2 / 16 * (r % 4 == 2)
    m = np.stack([np.cos(th), -np.sin(th)], axis=1).astype(BF16).view(np.uint16).astype(np.uint32)
    return (m[:, :, 0::2] | (m[:, :, 1::2] << 16)).reshape(R * LN, LN)


_M = _dft_matrices()


WS = 2 * D
DO = 256
EARLY = 6
B3 = ((0, EARLY, 0), (5, 11, 0), (10, 16, 5), (14, 16, 10), (16, 16, 14))
KB = (3, 3, 1, 0, 1, 0, 0, 0)
WP, XP = (8, 8, 9, 9), (7, 7, 8, 9)


class _Buf:
    def __init__(self, ref, base=0, size=None):
        if isinstance(base, int):
            self.ref, self.base = ref, base
        else:
            self.ref, self.base = ref.at[pl.ds(pl.multiple_of(base, 16), size), :], 0

    def ld(self, row, n):
        return self.ref[self.base + row:self.base + row + n, :]

    def st(self, row, v):
        self.ref[self.base + row:self.base + row + v.shape[0], :] = v.astype(self.ref.dtype)


def _weave(*stages):
    live = [[g, n, 0] for g, n in stages]
    while live:
        st = min(live, key=lambda t: t[2] / t[1])
        try:
            next(st[0])
            st[2] += 1
        except StopIteration:
            live.remove(st)


def _chain(*gens):
    for g in gens:
        yield from g


def _take(g, n):
    for _, _ in zip(range(n), g):
        yield


def _tree(op, v):
    while len(v) > 1:
        v = [op(v[i], v[i + 1]) for i in range(0, len(v), 2)]
    return v[0]


def _mult(i, n):
    return i if isinstance(i, int) else pl.multiple_of(i, n)


def _loop(lo, hi, body):
    def step(k, carry):
        body(k)
        return carry

    lax.fori_loop(lo, hi, step, 0)


def _iota(shape, dim):
    return lax.broadcasted_iota(jnp.int32, shape, dim)


def _cmul(a, b):
    return (a[0] * b[0] - a[1] * b[1], a[0] * b[1] + a[1] * b[0])


def _csq(a):
    t = a[0] * a[1]
    return (a[0] * a[0] - a[1] * a[1], t + t)


def _radix4(a, b, c, d, sign):
    s0 = (a[0] + c[0], a[1] + c[1])
    d0 = (a[0] - c[0], a[1] - c[1])
    s1 = (b[0] + d[0], b[1] + d[1])
    d1 = (b[0] - d[0], b[1] - d[1])
    y0 = (s0[0] + s1[0], s0[1] + s1[1])
    y2 = (s0[0] - s1[0], s0[1] - s1[1])
    p = (d0[0] - d1[1], d0[1] + d1[0])
    m = (d0[0] + d1[1], d0[1] - d1[0])
    return (y0, p, y2, m) if sign > 0 else (y0, m, y2, p)


def _twiddle(a, k, sign):
    k = sign * k % 16
    c, s = float(np.cos(2 * np.pi * k / 16)), float(np.sin(2 * np.pi * k / 16))
    if k % 4 == 0:
        return (a, (-a[1], a[0]), (-a[0], -a[1]), (a[1], -a[0]))[k // 4]
    if k % 8 == 2:
        return ((a[0] - a[1]) * c, (a[0] + a[1]) * c)
    if k % 8 == 6:
        return ((a[0] + a[1]) * c, (a[1] - a[0]) * c)
    return (a[0] * c - a[1] * s, a[0] * s + a[1] * c)


_ROW, _COL = (0, 0, 2, 0), (0, 0, 2, 0)
_TW = [[r0 * g0 - _ROW[r0] - _COL[g0] for g0 in range(4)] for r0 in range(4)]


def _kernel(x_hbm, wqkv_hbm, wo_hbm, are_hbm, aim_hbm, bre_hbm, bim_hbm, cre_hbm, cim_hbm,
            ldt_hbm, dsk_hbm, m_hbm, out_hbm, ldt_ref, dsk_ref,
            io, oo, wraw, woraw, par, mm, X, KF, DSK, XN, U, W, Z, KVQ, O, G, HH,
            KT, GK, E, DT, ZK, SA, SB, KO, zero, sems):
    for k in range(R):
        zero[k] = 0

    def block(cond=None):
        return pl.when(zero[0] == 0 if cond is None else cond)

    pcp = [[pltpu.make_async_copy(h.at[rows, :], par.at[i, rows, :], sems.at[o + i])
            for i, h in enumerate((are_hbm, aim_hbm, bre_hbm, bim_hbm, cre_hbm, cim_hbm))]
           for o, rows in ((0, pl.ds(0, 2 * CB)), (26, pl.ds(2 * CB, D - 2 * CB)))]
    mcp = pltpu.make_async_copy(m_hbm, mm, sems.at[6])
    xcp = [pltpu.make_async_copy(x_hbm.at[:, pl.ds(j * LN, LN)], io.at[j], sems.at[7 + j])
           for j in range(4)]
    wocp = [pltpu.make_async_copy(wo_hbm.at[pl.ds(j * LN, LN), :], woraw.at[pl.ds(j * LN, LN), :],
                                  sems.at[32 + j]) for j in range(4)]
    wcp = [pltpu.make_async_copy(wqkv_hbm.at[:, pl.ds(j * LN, LN)], wraw.at[j], sems.at[12 + j])
           for j in range(12)]
    scp = [pltpu.make_async_copy(ldt_hbm, ldt_ref, sems.at[24]),
           pltpu.make_async_copy(dsk_hbm, dsk_ref, sems.at[25])]
    for c in scp + pcp[0]:
        c.start()

    for c in scp:
        c.wait()
    dt_row = jnp.exp(ldt_ref[...].astype(F32).reshape(1, D)).astype(BF16).astype(F32)
    ds_row = dsk_ref[...].astype(F32).reshape(1, D)
    for j in range(4):
        sl = slice(j * LN, (j + 1) * LN)
        DT[sl, :] = jnp.broadcast_to(dt_row[:, sl], (LN, LN)).T
        DSK[sl, :] = jnp.broadcast_to(ds_row[:, sl], (LN, LN)).T

    lane = _iota((8, LN), 1)

    def kexp(J, slot):
        for s in range(8):
            rows = pl.ds(_mult(J * CB + s * 8, 8), 8)
            if s % 2 == 0:
                p16 = [par[i, pl.ds(_mult(J * CB + s * 8, 16), 16), :].astype(F32) for i in range(6)]
            p = [v[s % 2 * 8:s % 2 * 8 + 8] for v in p16]
            dt = DT[rows, :]
            zr, zi = dt * p[0], dt * p[1]
            mag = jnp.exp(zr)
            E[slot][0, s] = mag * jnp.cos(zi)
            yield
            E[slot][1, s] = mag * jnp.sin(zi)
            w = _cmul((p[4], p[5]), (dt * p[2], dt * p[3]))
            E[slot][2, s] = w[0] * (1.0 / S)
            E[slot][3, s] = w[1] * (1.0 / S)
            ZK[rows, :] = (jnp.sum(w[0], axis=1, keepdims=True) + DSK[rows, :]) * (1.0 / S)
            yield

    def kpow(J, slot):
        sa, sb = SA[slot], SB[slot]
        for s in range(8):
            def put(ref, i, v):
                n = (ref.shape[1] // 8 - 1) // 4
                for c in range(2):
                    ref[s // 4 * 2 + c, pl.ds(s % 4 * n + i, 8, stride=4 * n + 1), :] = v[c]

            p = (E[slot][0, s], E[slot][1, s])
            b = [None]
            for k in range(4):
                for i in range(2 ** k):
                    b.append(_cmul(b[i], p) if i else p)
                    put(sb, len(b) - 2, b[-1])
                    yield
                p = _csq(p)
            put(sb, 15, p)
            b = {4: b[4], 8: b[8], 12: b[12], 16: p}
            w = (E[slot][2, s], E[slot][3, s])
            pw = []
            for k in range(5):
                pw.append(p)
                p = _csq(p)
                yield
            e512, e1024 = p, _csq(p)
            for o, st, e in ((15, 4, e512), (19, 8, e1024), (21, 8, _cmul(e512, e1024))):
                for i in range(1, 16 // st + 1):
                    put(sb, o + i, _cmul(e, b[i * st]))
                    yield

            def tree(i, v, k):
                put(sa, i, v)
                yield
                for k2 in range(k):
                    yield from tree(i + 2 ** k2, _cmul(v, pw[k2]), k2)

            yield from tree(0, w, 5)

    def ksum(J, slot):
        sa, sb = SA[slot], SB[slot]
        q = _iota((24, LN), 1) >> 5
        for hm in range(16):
            h, m = divmod(hm, 8)
            o = [lax.dot_general(sb[2 * h + c, m * 97:m * 97 + 96, :],
                                 sa[2 * h + c, m * 129:m * 129 + LN, :],
                                 NT, preferred_element_type=F32) for c in range(2)]
            o = o[0] - o[1]
            KO[slot][h, m * 25:m * 25 + 24, :] = jnp.where(
                q < 2, jnp.where(q == 0, o[0:24], o[24:48]), jnp.where(q == 2, o[48:72], o[72:96]))
            yield

    def kspread(J, slot, h):
        kb = lambda i: KO[slot][h, pl.ds(i, 8, stride=25), :]
        rnd = lambda r, st: int(np.round(r / st))
        quarter = lane >> 5
        q1 = [None] + [pltpu.roll(kb(i), 32, 1) for i in range(16, 20)]
        q2 = [None] + [pltpu.roll(kb(i), 64, 1) for i in range(20, 22)]
        q3 = [None] + [pltpu.roll(kb(i), 96, 1) for i in range(22, 24)]
        k0, q23, rest = [], {}, {}
        for r in (16,) + tuple(range(R)):
            k2, k4, k8 = rnd(r, 2), rnd(r, 4), rnd(r, 8)
            if r:
                q0 = kb(r - 1)
                if r % 2 and k2:
                    q0 = jnp.where((lane & 31) < 16, q0, kb(2 * k2 - 1))
            for s in range(4):
                row = pl.ds(_mult(J * CB + h * 32 + s * 8, 8), 8)
                if r:
                    t = q0
                    if k8 and (k8, s) not in q23:
                        q23[k8, s] = jnp.where(quarter == (s + 2) % 4, q2[k8], q3[k8])
                    if k4:
                        if (k4, k8, s) not in rest:
                            rest[k4, k8, s] = jnp.where(
                                quarter == (s + 1) % 4, q1[k4], q23[k8, s]) if k8 else q1[k4]
                        t = jnp.where(quarter == s, t, rest[k4, k8, s])
                    if s or r == 16:
                        t = pltpu.roll(t, (LN - 32 * s + (r == 16)) % LN, 1)
                    if not k8:
                        t = jnp.where(lane < (64 if k4 else 32 if k2 else 16), t, k0[s])
                else:
                    t = jnp.where(lane == 0, ZK[row, :], k0[s])
                if r == 16:
                    k0.append(t)
                else:
                    _Buf(KT[slot]).st(r * CB + h * 32 + s * 8, t)
            yield

    def ld(b, k, h, n=8, stride=CB):
        return b.ld(2 * k * stride + h, n), b.ld((2 * k + 1) * stride + h, n)

    def st(b, k, h, v, stride=CB):
        b.st(2 * k * stride + h, v[0])
        b.st((2 * k + 1) * stride + h, v[1])

    def mat(r):
        return pltpu.bitcast(jnp.concatenate(ld(_Buf(mm), r, 0, 64, 64), axis=1), BF16)

    def kfwd(i, slot):
        g = _Buf(GK, i * 2 * R * CB, 2 * R * CB)
        for r in range(R):
            t = lax.dot_general(_Buf(KT[slot]).ld(r * CB, CB), mat(r), NN, preferred_element_type=F32)
            st(g, r, 0, (t[:, :LN], t[:, LN:]))
            yield

    def kfft(i):
        kf = _Buf(KF, i * CB, 2 * R * D - D + CB)
        for h in range(0, CB, 8):
            t = []
            for r0 in range(4):
                y = _radix4(*[ld(_Buf(GK, i * 2 * R * CB), r, h) for r in range(r0, R, 4)], -1)
                t.append([_twiddle(y[g0], _TW[r0][g0], -1) for g0 in range(4)])
                yield
            for g0 in range(4):
                y = _radix4(t[0][g0], t[1][g0], t[2][g0], t[3][g0], -1)
                for g1 in range(4):
                    st(kf, 4 * g0 + g1, h, _twiddle(y[g1], _COL[g0], -1), D)
                yield

    iow = io.bitcast(U32)

    def xin(j):
        x = _Buf(X, j * LN)
        for rho in range(8):
            t = iow[j, pl.ds(rho, LN, stride=8), :].T
            x.st(2 * rho * D, pltpu.bitcast(t << 16, F32))
            x.st((2 * rho + 1) * D, pltpu.bitcast(t & np.uint32(0xFFFF0000), F32))
            yield

    def wprep(j):
        pr, pc = _iota((LN, LN), 0), _iota((LN, LN), 1)
        perm = jnp.where(pc == (pr & 7) * DH + (pr >> 3), 1.0, 0.0).astype(BF16)
        for c in range(3):
            t = lax.dot_general(perm, wraw[(c + 1) % 3 * 4 + j], NT, preferred_element_type=F32)
            if c == 2:
                t = t * (DH ** -0.5)
            for k in range(4):
                _Buf(W).st(k * WS + (3 * j + c) * LN // 2,
                           pltpu.bitcast(t[:, k * LN:(k + 1) * LN].astype(BF16), U32))
            yield
        t = jnp.dot(perm, woraw[j * LN:(j + 1) * LN, :], preferred_element_type=F32)
        _Buf(W).st(j * WS + 3 * D // 2, pltpu.bitcast(t.T.astype(BF16), U32))
        yield

    def kstep(J, ref):
        @block()
        def _():
            slot, m, v = ref % 2, [], []
            if 0 <= ref < NCB:
                m.append(ksum(J, slot))
            if 0 <= ref - 2:
                m.append(kfwd(J - 2, slot))
            v = [(g, 16) for g in m]
            if 0 <= ref - 1 < NCB:
                v.append((_chain(*[kspread(J - 1, 1 - slot, h) for h in range(2)]), 34))
            if 0 <= ref + 1 < NCB:
                v.append((kpow(J + 1, 1 - slot), 8 * 60))
            if ref + 2 < NCB:
                v.append((kexp(J + 2, slot), 16))
            for gen, steps, n in ((xin, XP, 8), (wprep, WP, 4)):
                js = [j for j in range(4) if steps[j] == ref]
                v.append((_chain(*map(gen, js)), n * len(js) + 0.01))
            _weave(*v)

    def wcopies(J):
        return [c for j in range(4) if WP[j] in J for c in wcp[j::4] + [wocp[j]]]

    for J in range(-2, 10):
        for c in ({-2: pcp[0], 0: pcp[1], 2: [mcp]}.get(J, []) + wcopies((J,))
                  + (xcp if J == XP[0] else [])):
            c.wait()
        for c in {-2: pcp[1], 0: [mcp], 2: xcp + wcopies(WP)}.get(J, []):
            c.start()
        if J == 2:
            _loop(1, 3, lambda k: (kstep(2 * k, 2), kstep(2 * k + 1, 3)))
        elif not 2 <= J < 6:
            kstep(J, J)

    def colsum(f, step):
        acc = [f(c * 8) for c in range(4)]
        for i in range(4, D // 8):
            acc[i % 4] = acc[i % 4] + f(i * 8)
            if i % step == step - 1:
                yield
        s = jnp.sum((acc[0] + acc[1]) + (acc[2] + acc[3]), axis=0, keepdims=True)
        return jnp.broadcast_to(s * (1.0 / D), (8, LN))

    def ln_stats(ref, base):
        x = _Buf(ref, base + zero[0], D)
        m = yield from colsum(lambda c: x.ld(c, 8), 32)
        x = _Buf(ref, base + zero[1], D)
        v = yield from colsum(lambda c: jnp.square(x.ld(c, 8) - m), 8)
        return _Buf(ref, base + zero[2], D), m, lax.rsqrt(v + EPS)

    def ln(ref, base, out, r):
        x, m, rs = yield from ln_stats(ref, base)
        for c in range(0, D, 16):
            t = [(x.ld(c + k, 8) - m) * rs for k in (0, 8)]
            _Buf(out, r * D).st(c, jnp.concatenate(t, axis=0))
            if c % 64 == 48:
                yield

    def ln1(r):
        return ln(X, r * D, XN, r)

    def ln2(r):
        return ln(Z[r], 0, U, r)

    def wdot(c, n, rhs):
        lhs = jnp.concatenate(
            [pltpu.bitcast(W[t * WS + c // 2:t * WS + (c + n) // 2, :], BF16)
             for t in range(4)], axis=1)
        return jnp.dot(lhs, rhs.ld(0, D), preferred_element_type=F32)

    def qkvproj(j, r):
        b, i = _Buf(KVQ[j % 2][r % 2]), r // 2
        for c in range(3):
            t = wdot((3 * j + c) * LN, LN, _Buf(XN, r * D + zero[(r + c) % R], D))
            if c == 2:
                b.st((32 + i) * LN, t)
            else:
                b.st((16 * c + 8 + i) * LN, t)
                if i:
                    b.st((16 * c + i) * LN, pltpu.roll(t, 1, 1))
            yield

    def core(j, r):
        b, i = _Buf(KVQ[j % 2][r % 2], zero[r], 40 * LN), r // 2
        lg = [None] * WIN
        for dh in range(DH):
            q = b.ld((32 + i) * LN + dh * 8, 8)
            for w in range(WIN):
                t = q * b.ld((8 + i - w) * LN + dh * 8, 8)
                lg[w] = t if dh == 0 else lg[w] + t
            if dh % 2:
                yield
        for w in range(i + 1, WIN):
            lg[w] = jnp.where(lane > 0, lg[w], -1e9)
        mx = _tree(jnp.maximum, lg)
        e = [jnp.exp(v - mx) for v in lg]
        inv = 1.0 / _tree(jnp.add, e)
        e = [v * inv for v in e]
        yield
        yield
        for dh in range(0, DH, 2):
            oo = []
            for k in (dh, dh + 1):
                acc = None
                for w in range(WIN):
                    t = e[w] * b.ld((24 + i - w) * LN + k * 8, 8)
                    acc = t if acc is None else acc + t
                oo.append(acc)
            _Buf(O, r * D + j * LN).st(dh * 8, jnp.concatenate(oo, axis=0))
            yield

    def oproj(r):
        for c in range(0, D, DO):
            Z[r][c:c + DO, :] = X[r * D + c:r * D + c + DO, :] + wdot(
                3 * D + c, DO, _Buf(O, r * D + zero[(r + c // DO) % R], D))
            yield

    def cmxu(fi, ii, slot, rs):
        if fi is not None:
            u_ = _Buf(U, fi * CB, R * D - D + CB)
        if ii is not None:
            x = _Buf(X, ii * CB, R * D - D + CB)
        for r in rs:
            if fi is not None:
                t = lax.dot_general(u_.ld(r * D, CB), mat(r), NN, preferred_element_type=F32)
                st(_Buf(G[slot]), r, 0, (t[:, :LN], t[:, LN:]))
                yield
            if ii is not None:
                lhs = jnp.concatenate(ld(_Buf(HH[slot]), r, 0, CB), axis=1)
                t = lax.dot_general(lhs, mat(r), NT, preferred_element_type=F32)
                x.st(r * D, _Buf(Z[r], ii * CB, CB).ld(0, CB) + t)
                yield

    def cmid(i, slot):
        g, hh = _Buf(G[slot], zero[0], 2 * R * CB), _Buf(HH[slot])
        kf = _Buf(KF, i * CB, 2 * R * D - D + CB)

        for h in range(0, CB, 8):
            t, v = [], []
            for r0 in range(4):
                y = _radix4(*[ld(g, r, h) for r in range(r0, R, 4)], -1)
                t.append([_twiddle(y[g0], _TW[r0][g0], -1) for g0 in range(4)])
                yield
            yield
            for g0 in range(4):
                y = _radix4(t[0][g0], t[1][g0], t[2][g0], t[3][g0], -1)
                yield
                y = [_cmul(y[g1], ld(kf, 4 * g0 + g1, h, 8, D)) for g1 in range(4)]
                yield
                y = _radix4(*y, 1)
                v.append([_twiddle(y[r0], _TW[r0][g0], 1) for r0 in range(4)])
                yield
                if g0 != 1:
                    yield
            for r0 in range(4):
                y = _radix4(*[v[g0][r0] for g0 in range(4)], 1)
                for r1 in range(4):
                    st(hh, r0 + 4 * r1, h, y[r1])
                yield

    ocp = [pltpu.make_async_copy(src, out_hbm.at[:, pl.ds(j * LN, LN)], sems.at[7 + j])
           for j, src in enumerate((oo[0].at[0], oo[0].at[1], oo[1].at[0], oo[2].at[0]))]

    def xout(j, buf, first, rhos=range(8)):
        x, w = _Buf(X, j * LN, R * D - D + LN), buf.bitcast(U32)
        for rho in rhos:
            a, b = (pltpu.bitcast(x.ld(r * D, LN).astype(BF16).astype(F32), U32)
                    for r in (2 * rho, 2 * rho + 1))
            w[j - first, pl.ds(rho, LN, stride=8), :] = ((a >> 16) | b).T
            yield

    order = list(range(0, R, 2)) + list(range(1, R, 2))
    NCORE, NLN1, NLN2 = 18, 18, 18

    def layer(l, carry):
        def spectra(b):
            ids = range(sum(KB[:b]), sum(KB[:b + 1]))
            return _chain(*map(kfft, ids)), 64 * len(ids) + 0.01

        @block()
        def _():
            _weave((_chain(*[qkvproj(0, r) for r in order]), 3 * R),
                   (_chain(*map(ln1, order[1:])), NLN1 * (R + 1)))

        for b, (j, lo, hi) in enumerate(((1, 0, R), (2, 0, R), (3, 0, R // 2), (3, R // 2, R))):
            @block()
            def _():
                early = _chain(*[core(3, r) for r in order[:EARLY if lo else 0]])
                kf, nk = spectra(b)
                nk = int(nk) // (hi - lo)
                for r in order[lo:hi]:
                    _weave((qkvproj(j, r), 3), (core(j - 1, r), NCORE),
                           (_take(early, -(-EARLY * NCORE // 8)), EARLY * NCORE / 8),
                           (_take(kf, nk), nk + 0.01))

        for b, (prev, cur) in enumerate(zip(B3, B3[1:])):
            @block()
            def _():
                w, c, n = (order[u:v] for u, v in zip(prev, cur))
                _weave((_chain(*map(oproj, w)), len(w) * D // DO),
                       (_chain(*[core(3, r) for r in c]), len(c) * NCORE + 0.01),
                       (_chain(*map(ln2, n)), len(n) * NLN2 + 0.01), spectra(4 + b))

        def cstep(i, slot, f=True, m=True, v=True, out=(), cond=None):
            @block(cond)
            def _():
                _weave((cmxu(i + 1 if f else None, i - 1 if v else None, 1 - slot, order), R * (f + v)),
                       *([(cmid(i, slot), 3 * CB)] if m else []),
                       *[(ln2(r), 2 * NLN2) for r in order[B3[-1][2]:] if f and not m], *out)

        cstep(-1, 1, m=False, v=False)
        cstep(0, 0, v=False)

        def cpair(k):
            for e in range(2):
                cstep(2 * k + 1 + e, 1 - e, cond=l * k == 0)
                cstep(2 * k + 1 + e, 1 - e, cond=l * k > 0,
                      out=[(xout(k - 1, oo[0], 0, range(4 * e, 4 * e + 4)), 5)])
            for j in range(2):
                pl.when(l * k == j + 1)(ocp[j].start)

        _loop(0, NCB // 2 - 1, cpair)
        cstep(NCB - 1, 1, f=False, cond=l == 0)
        cstep(NCB - 1, 1, f=False, cond=l == 1, out=[(xout(2, oo[1], 2), 10)])

        @pl.when(l == 0)
        def _():
            _weave((_chain(cmxu(None, NCB - 1, 1, order), ln1(0)), 1))

        @pl.when(l == 1)
        def _():
            ocp[2].start()
            m = cmxu(None, NCB - 1, 1, range(R))
            _weave((_take(m, 4), 1))
            _weave((xout(3, oo[2], 3), 8), (m, R))
            ocp[3].start()

        return carry

    _weave((ln1(0), 1))
    lax.fori_loop(0, 2, layer, 0)

    for c in ocp:
        c.wait()


@jax.jit
def pallas_interleave_layers__sliding_local_dilated__ssm_conv_s4__prompt_kernel(
    A_x: jax.Array,
    A_wqkv: jax.Array,
    A_wo: jax.Array,
    B_u: jax.Array,
    B_A_re: jax.Array,
    B_A_im: jax.Array,
    B_B_re: jax.Array,
    B_B_im: jax.Array,
    B_C_re: jax.Array,
    B_C_im: jax.Array,
    B_log_dt: jax.Array,
    B_Dskip: jax.Array,
):
    del B_u
    hbm = pl.BlockSpec(memory_space=pl.ANY)
    V = pltpu.VMEM
    out = pl.pallas_call(
        _kernel,
        out_shape=jax.ShapeDtypeStruct((S, D), BF16),
        in_specs=[hbm] * 12,
        out_specs=hbm,
        scratch_shapes=[
            V((D,), BF16), V((D,), BF16),
            V((4, S, LN), BF16),
            [V((n, S, LN), BF16) for n in (2, 1, 1)],
            V((12, D, LN), BF16),
            V((D, D), BF16),
            V((6, D, LN), BF16),
            V((R * LN, LN), U32),
            V((R * D, LN), F32),
            V((2 * R * D, LN), F32),
            V((D, LN), F32),
            V((R * D, LN), BF16),
            V((R * D, LN), F32),
            V((4 * WS, LN), U32),
            [V((D, LN), F32)] * R,
            [[V((40 * LN, LN), F32)] * 2] * 2,
            V((R * D, LN), BF16),
            [V((2 * R * CB, LN), F32)] * 2,
            [V((2 * R * CB, LN), F32)] * 2,
            [V((R * CB, LN), F32)] * 2,
            V((2 * R * D, LN), F32),
            [V((4, 8, 8, LN), F32)] * 2,
            V((D, LN), F32),
            V((D, LN), F32),
            [V((4, 8 * 129, LN), F32)] * 2,
            [V((4, 8 * 97, LN), F32)] * 2,
            [V((2, 8 * 25, LN), F32)] * 2,
            pltpu.SMEM((R,), jnp.int32),
            pltpu.SemaphoreType.DMA((36,)),
        ],
        compiler_params=pltpu.CompilerParams(vmem_limit_bytes=100 * 1024 * 1024),
    )(A_x.reshape(S, D), A_wqkv, A_wo, B_A_re, B_A_im, B_B_re, B_B_im, B_C_re, B_C_im,
      B_log_dt, B_Dskip, _M)
    return out.reshape(1, S, D)
```
